```python
import jax
import jax.numpy as jnp

def _softmax(x, axis=-1):
    return jax.nn.softmax(x, axis=axis)

def _gelu(x):
    return jax.nn.gelu(x, approximate=True)

def _silu(x):
    return jax.nn.silu(x)

def _sigmoid(x):
    return jax.nn.sigmoid(x)

def _layernorm(x, axis=-1, eps=1e-05):
    m = jnp.mean(x, axis=axis, keepdims=True)
    v = jnp.var(x, axis=axis, keepdims=True)
    return (x - m) / jnp.sqrt(v + eps)

def _scatter_add(tgt, idx, src, axis=0):
    return tgt.at[idx].add(src)

def _segment_sum(src, seg, n):
    return jax.ops.segment_sum(src, seg, n)

class _Rng:

    def __init__(self, key):
        self._k = key

    def _next(self):
        self._k, sub = jax.random.split(self._k)
        return sub

    def normal(self, shape):
        return jax.random.normal(self._next(), shape, dtype=jnp.bfloat16)

    def randint(self, lo, hi, shape):
        return jax.random.randint(self._next(), shape, lo, hi, dtype=jnp.int32)

    def uniform(self, shape, lo=0.0, hi=1.0):
        return jax.random.uniform(self._next(), shape, jnp.bfloat16, lo, hi)

    def permutation(self, n):
        return jax.random.permutation(self._next(), n)
kernel_name = 'adaLN_cond__ssm_conv_h3__glu_gated_reglu__prompt'

def setup_inputs():
    _rng = _Rng(jax.random.key(int.from_bytes(__import__("os").urandom(4), "little")))
    _w = lambda a: (lambda t: t.astype(jnp.bfloat16) if jnp.issubdtype(t.dtype, jnp.floating) else t)(jnp.asarray(a))

    def _A_setup():
        B, S, D = (1, 2048, 640)
        ks = 4
        return {'q': _w((lambda *s: _rng.normal(s) * 0.05)(B, S, D)), 'k': _w((lambda *s: _rng.normal(s) * 0.05)(B, S, D)), 'v': _w((lambda *s: _rng.normal(s) * 0.05)(B, S, D)), 'shift_k': _w((lambda *s: _rng.normal(s) * 0.05)(D, ks) * 0.5), 'ssm_k': _w((lambda *s: _rng.normal(s) * 0.05)(D, S) * (1.0 / S ** 0.5)), 'ssm_D': _w((lambda *s: _rng.normal(s) * 0.05)(D))}
    _A_in = _A_setup()

    def _B_setup():
        B, S, D, F = (1, 2048, 640, 1536)
        return {'x': _w((lambda *s: _rng.normal(s) * 0.05)(B, S, D)), 'W_gate': _w((lambda *s: _rng.normal(s) * 0.05)(D, F) * (2.0 / D) ** 0.5), 'W_up': _w((lambda *s: _rng.normal(s) * 0.05)(D, F) * (2.0 / D) ** 0.5), 'W_down': _w((lambda *s: _rng.normal(s) * 0.05)(F, D) * (1.0 / F) ** 0.5)}
    _B_in = _B_setup()
    return {'A_q': _A_in['q'], 'A_k': _A_in['k'], 'A_v': _A_in['v'], 'A_shift_k': _A_in['shift_k'], 'A_ssm_k': _A_in['ssm_k'], 'A_ssm_D': _A_in['ssm_D'], 'B_x': _B_in['x'], 'B_W_gate': _B_in['W_gate'], 'B_W_up': _B_in['W_up'], 'B_W_down': _B_in['W_down'], 'c': _w((lambda *s: _rng.normal(s) * 0.05)(1, 640)), 'w_mod': _w((lambda *s: _rng.normal(s) * 0.05)(640, 6 * 640) * 640 ** (-0.5))}

def reference(A_q, A_k, A_v, A_shift_k, A_ssm_k, A_ssm_D, B_x, B_W_gate, B_W_up, B_W_down, c, w_mod):

    def _A_ref(q, k, v, shift_k, ssm_k, ssm_D):
        B, S, D = q.shape
        ks = shift_k.shape[-1]
        k_pad = jnp.pad(k, ((0, 0), (ks - 1, 0), (0, 0)))
        k_shift = jnp.zeros_like(k)
        for t in range(ks):
            k_shift = k_shift + k_pad[:, t:t + S, :] * shift_k[:, ks - 1 - t][None, None, :]
        kv = k_shift * v
        L = 2 * S
        kv_pad = jnp.pad(kv, ((0, 0), (0, S), (0, 0)))
        kf_pad = jnp.pad(ssm_k, ((0, 0), (0, S)))
        kv_f = (lambda x, axes=(-2, -1): jnp.fft.rfft2(x.astype(jnp.float32), axes=axes))(kv_pad[:, None, :, :], axes=(1, 2))
        kf_f = (lambda x, axes=(-2, -1): jnp.fft.rfft2(x.astype(jnp.float32), axes=axes))(kf_pad[:, None, :], axes=(1, 2))
        kf_f = (lambda x, *d: x.transpose(*d))(kf_f, 1, 2, 0)
        y_f = kv_f * kf_f[None, :, :, :]
        y = (lambda x, s, axes=(-2, -1): jnp.fft.irfft2(x, s=s, axes=axes).astype(jnp.bfloat16))(y_f, (1, L), axes=(1, 2))[:, 0, :S, :]
        y = y + kv * ssm_D[None, None, :]
        return q * y

    def _B_ref(x, W_gate, W_up, W_down):
        gate = jnp.einsum('bsd,df->bsf', x, W_gate)
        up = jnp.einsum('bsd,df->bsf', x, W_up)
        gate = gate * (lambda x, dt: x.astype(dt))(gate > 0, gate.dtype)
        h = gate * up
        return jnp.einsum('bsf,fd->bsd', h, W_down)
    x = A_q
    mod = (_silu(c) @ w_mod).reshape(c.shape[0], 6, 1, -1)
    sa, ca, ga, sb, cb, gb = (mod[:, 0].copy(), mod[:, 1].copy(), mod[:, 2].copy(), mod[:, 3].copy(), mod[:, 4].copy(), mod[:, 5].copy())
    h = _layernorm(x, axis=-1) * (1 + ca) + sa
    x = x + ga * _A_ref(h, A_k, A_v, A_shift_k, A_ssm_k, A_ssm_D)
    h = _layernorm(x, axis=-1) * (1 + cb) + sb
    x = x + gb * _B_ref(h, B_W_gate, B_W_up, B_W_down)
    return x
```

```python
import contextlib
import functools
import numpy as np
import jax
import jax.numpy as jnp
from jax import lax
from jax.experimental import pallas as pl
from jax.experimental.pallas import tpu as pltpu

S, D, F = 2048, 640, 1536
NB = 128
T = 256
NS = S // T
NBLK = S // NB
FC = 512
NC = F // FC
NL = D // 128
EPS = 1e-5
f32 = jnp.float32
bf16 = jnp.bfloat16
i32 = jnp.int32

CFG = dict(only=None, pad=8, sc_lanes=2, lnlag=1, lnent=4, k4=0.0, k4f=0.0, tree=(2, 5), treef=(1,), scpos='start', scopes=False)

MNAMES = ['sa', 'ca', 'ga', 'sb', 'cb', 'gb']
NW = 3 * (NS + 1)
NG = NB // 8
HT = T // 2


def _dft_mats():
    f = np.concatenate([np.arange(0, NB, 2), np.arange(1, NB, 2)])
    j = np.arange(NB)
    idx = ((2 * f[:, None] + 1) * j[None, :]) % (4 * NB)
    ang = 2.0 * np.pi * idx / (4 * NB)
    fwd = np.stack([np.cos(ang).reshape(NB // 8, 8, NB), np.sin(ang).reshape(NB // 8, 8, NB)], axis=1)
    fwd = fwd.reshape(2 * NB, NB)
    inv = fwd.T / NB
    return fwd.astype(np.float32), inv.astype(np.float32)


def kernel(q_hbm, k_hbm, v_hbm, sh_hbm, ssm_hbm, dd_hbm, wg_hbm, wu_hbm, wd_hbm, c_hbm, wm_hbm,
           fw_hbm, iv_hbm, o_hbm,
           q_v, k_v, v_v, ssm_v, wg_v, wu_v, wd_v, wm_v, fw_v, iv_v, o_v,
           uv, ap, zb, kvb, mv, yb, x1b, hn_v, hf, hn1, sh_v, dd_v, c_v,
           sems, osem):
    pid = pl.program_id(0)

    def rows(s):
        return pl.ds(s * T, T) if isinstance(s, int) else pl.ds(pl.multiple_of(s * T, T), T)

    small = {
        'sh': (sh_hbm, sh_v), 'dd': (dd_hbm, dd_v), 'c': (c_hbm, c_v), 'fw': (fw_hbm, fw_v), 'iv': (iv_hbm, iv_v),
    }
    misc = list(small) + [('wm', nm) for nm in MNAMES] + [(w, c) for c in range(NC) for w in ('wg', 'wu', 'wd')]

    NM = len(misc)

    def cp(name):
        if isinstance(name, str):
            src, dst = small[name]
            return pltpu.make_async_copy(src, dst, sems.at[misc.index(name)])
        kind, j = name
        if kind == 'k':
            return pltpu.make_async_copy(k_hbm.at[0, rows(j), :], k_v.at[j], sems.at[NM + j])
        if kind == 'v':
            return pltpu.make_async_copy(v_hbm.at[0, rows(j), :], v_v.at[j], sems.at[NM + NS + j])
        if kind == 'q':
            return pltpu.make_async_copy(q_hbm.at[0, rows(j), :], q_v.at[j], sems.at[NM + 2 * NS + j])
        if kind == 'o':
            return pltpu.make_async_copy(o_v.at[j], o_hbm.at[0, rows(j), :], osem.at[j])
        if kind == 's':
            c0 = j * NB if isinstance(j, int) else pl.multiple_of(j * NB, NB)
            return pltpu.make_async_copy(ssm_hbm.at[:, pl.ds(c0, NB)], ssm_v.at[j], sems.at[NM + 3 * NS + j])
        sem = sems.at[misc.index(name)]
        if kind == 'wm':
            r = pl.ds(MNAMES.index(j) * D, D)
            return pltpu.make_async_copy(wm_hbm.at[:, r], wm_v.at[:, r], sem)
        r = pl.ds(j * FC, FC)
        if kind == 'wg':
            return pltpu.make_async_copy(wg_hbm.at[:, r], wg_v.at[:, r], sem)
        if kind == 'wu':
            return pltpu.make_async_copy(wu_hbm.at[:, r], wu_v.at[:, r], sem)
        return pltpu.make_async_copy(wd_hbm.at[r, :], wd_v.at[r, :], sem)

    def wait(*names):
        for nm in names:
            cp(nm).wait()

    def ss2(s):
        return [('s', 2 * s), ('s', 2 * s + 1)]

    def kvs(s):
        return [('k', s), ('v', s)] + ss2(s)

    H = NB // 2

    class Reg:
        def __init__(self):
            z0 = lax.shift_right_logical(pid, 8)
            self.z0 = z0
            self.row = lax.broadcasted_iota(i32, (8, 128), 0)
            self.st = {}

        def off(self, s, n):
            return s * n if isinstance(s, int) else pl.multiple_of(s * n, n)

        def modpart(self, nm):
            p = MNAMES.index(nm)
            c32 = c_v[...].astype(f32)
            sc8 = jnp.broadcast_to((c32 * jax.nn.sigmoid(c32)).astype(bf16), (8, D))
            return jnp.dot(sc8, wm_v[:, p * D:(p + 1) * D], preferred_element_type=f32)

        def sconv(self, s, lanes, lcs=None):
            row = self.row
            taps = sh_v[...].astype(f32)
            if lcs is None or lcs[0] == 0:
                self.sctoks = [None] * lanes if lanes else None
            toks = self.sctoks
            gi = 0
            for lc in (range(NL) if lcs is None else lcs):
                ls = pl.ds(lc * 128, 128)
                w = [jnp.broadcast_to(taps[j:j + 1, lc * 128:(lc + 1) * 128], (8, 128)) for j in range(4)]
                if isinstance(s, int) and s == 0:
                    pk = jnp.zeros((8, 128), f32); pt = jnp.zeros((8, 128), f32)
                else:
                    kp = k_v[s - 1, T - 16:T, ls].astype(f32)[8:16]
                    pk = pltpu.roll(kp, 1, 0)
                    pt = pltpu.roll(w[2] * kp + w[3] * pk, 2, 0)
                for rg in range(T // 16):
                    kk = k_v[s, rg * 16:rg * 16 + 16, ls].astype(f32)
                    vv = v_v[s, rg * 16:rg * 16 + 16, ls].astype(f32)
                    outs = []
                    for h in range(2):
                        kc = kk[8 * h:8 * h + 8]
                        if h == 0 and lanes and toks[gi % lanes] is not None:
                            kc = kc + toks[gi % lanes]
                        rk = pltpu.roll(kc, 1, 0)
                        sk = jnp.where(row < 1, pk, rk)
                        t = w[2] * kc + w[3] * sk
                        rt = pltpu.roll(t, 2, 0)
                        stt = jnp.where(row < 2, pt, rt)
                        outs.append(((w[0] * kc + w[1] * sk) + stt) * vv[8 * h:8 * h + 8])
                        pk, pt = rk, rt
                    kvp = pltpu.bitcast(jnp.concatenate(outs, axis=0).astype(bf16), f32)
                    kvb.at[self.z0][rg * 8:rg * 8 + 8, ls] = kvp
                    if lanes:
                        toks[gi % lanes] = kvb[0, HT:HT + 8, ls]
                    gi += 1

        def fwd_x(self, s, lc):
            ou = self.z0 + 3 * s
            ls = pl.ds(lc * 128, 128)
            kv = pltpu.bitcast(jnp.concatenate([kvb[0, 0:64, ls], kvb[0, 64:128, ls]], axis=1), bf16)
            xx = jnp.dot(fw_v[...], kv, preferred_element_type=f32)
            x0 = xx[:, 0:128]; x1 = xx[:, 128:256]
            if isinstance(s, int) and s == 0:
                u1 = -x0
            else:
                pu = 3 * (s - 1)
                u1 = (uv[pu + 2, :, 16:32, ls] + uv[pu, :, 16:32, ls]).reshape(2 * NB, 128) - x0
            uv[ou, :, 16:32, ls] = x0.reshape(NG, 16, 128)
            uv[ou + 1, :, 16:32, ls] = u1.reshape(NG, 16, 128)
            uv[ou + 2, :, 16:32, ls] = (x1 - x0).reshape(NG, 16, 128)

        def fwd_h(self, s, lc, src=None):
            src = s if src is None else src
            ov = self.z0 + 3 * s
            ls = pl.ds(lc * 128, 128)

            def fold(a, p):
                parts = []
                for g in range(NB // 8):
                    ar, ai = a[16 * g:16 * g + 8], a[16 * g + 8:16 * g + 16]
                    pr, pi = p[16 * g:16 * g + 8], p[16 * g + 8:16 * g + 16]
                    parts += [ar + pi, ai - pr] if g < NB // 16 else [ar - pi, ai + pr]
                return jnp.concatenate(parts, axis=0)

            w = jnp.concatenate([ssm_v[2 * src, ls, :], ssm_v[2 * src + 1, ls, :]], axis=0)
            aa = lax.dot_general(fw_v[...], w, (((1,), (1,)), ((), ())), preferred_element_type=f32)
            a0 = aa[:, 0:128]; a1 = aa[:, 128:256]
            if isinstance(s, int) and s == 0:
                dd = dd_v[...].astype(f32).reshape(1, D)[:, lc * 128:(lc + 1) * 128]
                h0 = jnp.concatenate([a0[8 * g:8 * g + 8] + dd if g % 2 == 0 else a0[8 * g:8 * g + 8]
                                      for g in range(NB // 4)], axis=0)
            else:
                h0 = fold(a0, ap[0, :, ls])
            h1 = fold(a1, a0)
            uv[ov, :, 0:16, ls] = (h0 + h1).reshape(NG, 16, 128)
            uv[ov + 1, :, 0:16, ls] = h1.reshape(NG, 16, 128)
            uv[ov + 2, :, 0:16, ls] = h0.reshape(NG, 16, 128)
            ap[self.z0, :, ls] = a1

        def fwd(self, s):
            for lc in range(NL):
                self.fwd_h(s, lc)
            for lc in range(NL):
                self.fwd_x(s, lc)

        def mac(self, s, k4frac, tree=()):
            static = isinstance(s, int)
            ng = s + 1 if static else NS
            toks = [None] * 2
            acc4 = 0.0
            ub = [3 * (s - g) if static else 3 * jnp.maximum(s - g, 0) for g in range(ng)]
            for fc in range(NB // 8):
                for lc in range(NL):
                    fr = pl.ds(fc * 16, 8); fi = pl.ds(fc * 16 + 8, 8); ls = pl.ds(lc * 128, 128)
                    dense = k4frac is None
                    if not dense:
                        acc4 += k4frac
                        if acc4 >= 1.0:
                            acc4 -= 1.0
                            dense = True

                    def chain(j, ar, ai):
                        for g in range(ng):
                            hr = uv[3 * g + j, fc, 0:8, ls]; hi = uv[3 * g + j, fc, 8:16, ls]
                            xr = uv[ub[g] + j, fc, 16:24, ls]; xi = uv[ub[g] + j, fc, 24:32, ls]
                            if ar is not None and (k4frac is None or g in tree):
                                ar = ar + (hr * xr - hi * xi)
                                ai = ai + (hr * xi + hi * xr)
                            else:
                                ar = (hr * xr if ar is None else ar + hr * xr) - hi * xi
                                ai = (hr * xi if ai is None else ai + hr * xi) + hi * xr
                        return ar, ai

                    def tk(v, zmask):
                        return pltpu.bitcast(pltpu.bitcast(v, i32) & zmask, f32)

                    a1 = chain(0, toks[0], toks[1])
                    z0 = chain(1, *a1)
                    if k4frac is not None:
                        zmask = pltpu.bitcast(zb[0, T:T + 8, ls], i32)
                    if dense:
                        z1 = chain(2, *a1)
                    else:
                        z1 = chain(2, a1[0] + tk(z0[0], zmask), a1[1] + tk(z0[1], zmask))
                    for b, z in enumerate((z0, z1)):
                        zp = pltpu.bitcast(jnp.concatenate(z, axis=0).astype(bf16), f32)
                        zb.at[self.z0][b * HT + fc * 8:b * HT + fc * 8 + 8, ls] = zp
                    if k4frac is not None:
                        for p in range(2):
                            if dense:
                                bits = pltpu.bitcast(z0[p], i32) | pltpu.bitcast(z1[p], i32)
                                toks[p] = pltpu.bitcast(bits & zmask, f32)
                            else:
                                toks[p] = tk(z1[p], zmask)

        def inv(self, slot=0):
            for b in range(2):
                yb[self.z0, slot * T + b * NB:slot * T + (b + 1) * NB, :] = jnp.dot(
                    iv_v[...], pltpu.bitcast(zb[0, b * HT:(b + 1) * HT, :], bf16), preferred_element_type=f32)

        def rep(self, tk, n):
            return tk if n == 8 else jnp.concatenate([tk] * (n // 8), axis=0)

        def rowsum(self, x, tk=None):
            ps = x[:, 0:128]
            if tk is not None:
                ps = ps + self.rep(tk, x.shape[0])
            for lc in range(1, NL):
                ps = ps + x[:, lc * 128:(lc + 1) * 128]
            return jnp.sum(ps, axis=-1, keepdims=True)

        def ln1(self, s):
            RG = 16
            for g in range(T // RG):
                x = q_v[s, g * RG:(g + 1) * RG, :].astype(f32)
                xc = x - self.rowsum(x) * (1.0 / D)
                var = self.rowsum(xc * xc) * (1.0 / D) + EPS
                hn1[self.z0 + s, g * RG:(g + 1) * RG, :] = xc * lax.rsqrt(var)

        def lnf(self, s, lag, dst, dofs, slot=0, pre=False):
            a1 = mv[0:1, :]; a0 = mv[8:9, :]; b1 = mv[16:17, :]; b0 = mv[24:25, :]
            RG = 16
            ent = CFG['lnent']
            toks = {}
            for g in range(T // RG):
                tk = toks.get(g) if lag else None
                gr = slice(g * RG, (g + 1) * RG)
                x = q_v[s, gr, :].astype(f32)
                if pre:
                    hn = hn1[s, gr, :]
                else:
                    xc = x - self.rowsum(x) * (1.0 / D)
                    var = self.rowsum(xc * xc) * (1.0 / D) + EPS
                    hn = xc * lax.rsqrt(var)
                y = yb[0, slot * T + g * RG:slot * T + (g + 1) * RG, :]
                x1 = x + (hn * a1 + a0) * y
                x1b[self.z0 + s, gr, :] = x1
                m2 = self.rowsum(x1, tk if ent == 3 else None) * (1.0 / D)
                xc2 = x1 - m2
                var2 = self.rowsum(xc2 * xc2, tk if ent == 4 else None) * (1.0 / D) + EPS
                h2 = ((xc2 * lax.rsqrt(var2)) * b1 + b0).astype(bf16)
                dst.at[self.z0][dofs + g * (RG // 2):dofs + (g + 1) * (RG // 2), :] = pltpu.bitcast(h2, f32)
                if lag:
                    toks[g + lag] = dst[0, HT:HT + 8, 0:128]

        def g_(self, x, c):
            self.st['g'] = jnp.dot(x(), wg_v[:, c * FC:(c + 1) * FC], preferred_element_type=f32)

        def u_(self, x, c):
            u = jnp.dot(x(), wu_v[:, c * FC:(c + 1) * FC], preferred_element_type=f32)
            self.st['a'] = (jnp.maximum(self.st.pop('g'), 0.0) * u).astype(bf16)

        def d_(self, c):
            d = jnp.dot(self.st.pop('a'), wd_v[c * FC:(c + 1) * FC, :], preferred_element_type=f32)
            self.st['acc'] = d if c == 0 else self.st['acc'] + d

        def tail(self, x, s, n, fs, src, lanes):
            c = NC - 1
            gs, acts_ = [], []
            nq = FC // 128
            hq = 0
            for j in range(nq):
                c0 = c * FC + j * 128
                gs.append(jnp.dot(x(), wg_v[:, c0:c0 + 128], preferred_element_type=f32))
                self.fwd_h(fs, hq, src); hq += 1
            for j in range(nq):
                c0 = c * FC + j * 128
                u = jnp.dot(x(), wu_v[:, c0:c0 + 128], preferred_element_type=f32)
                acts_.append((jnp.maximum(gs[j], 0.0) * u).astype(bf16))
                if hq < NL:
                    self.fwd_h(fs, hq, src); hq += 1
            a = jnp.concatenate(acts_, axis=1)
            acc = self.st.pop('acc')
            for lc in range(NL):
                ls = pl.ds(lc * 128, 128)
                d = jnp.dot(a, wd_v[c * FC:(c + 1) * FC, ls], preferred_element_type=f32)
                tot = acc[:, lc * 128:(lc + 1) * 128] + d
                for j in range(n):
                    o_v[s + j, :, ls] = (x1b[s + j, :, ls] + mv[32:33, ls] * tot[j * T:(j + 1) * T]).astype(bf16)
                self.sconv(src, lanes, [lc])
                self.fwd_x(fs, lc)

        def fin(self, s, n):
            acc = self.st.pop('acc')
            for j in range(n):
                o_v[s + j] = (x1b[s + j] + mv[32:33, :] * acc[j * T:(j + 1) * T]).astype(bf16)

    SCL, LAG = CFG['sc_lanes'], CFG['lnlag']

    def scope(name):
        return jax.named_scope(name) if CFG['scopes'] else contextlib.nullcontext()

    def first():
        R = Reg()
        order = ['sh', 'dd', 'c', 'fw', 'iv'] + kvs(0) + kvs(1) + [('q', 0), ('q', 1)]
        order += [('wm', nm) for nm in ['ca', 'sa', 'ga', 'cb', 'sb']]
        for c in range(NC):
            order += [('wg', c), ('wu', c), ('wd', c)]
        order += [('wm', 'gb')] + kvs(2) + [('q', 2)] + kvs(3)
        for s in range(3, NS):
            order += [('q', s)]
            if s + 1 < NS:
                order += kvs(s + 1)
        for name in order:
            cp(name).start()
        z = jnp.zeros((8, D), f32)
        kvb[0, HT:HT + 8, :] = z
        hn_v[0, HT:HT + 8, :] = z
        zb[0, T:T + 8, :] = z
        def zero_blk(j, _):
            uv[j, :, 0:16, :] = jnp.zeros((NG, 16, D), f32)
            return 0
        lax.fori_loop(12, 3 * NS, zero_blk, 0)
        with scope("p_w0"):
            wait('sh', 'dd', 'c', 'fw', 'iv', *kvs(0))
        with scope("p_c0"):
            R.sconv(0, 0); R.fwd(0); R.mac(0, None); R.inv(0)
        with scope("p_w1"):
            wait(*kvs(1))
        with scope("p_c1"):
            R.sconv(1, 0); R.fwd(1); R.mac(1, None); R.inv(1)
        with scope("p_ln1"):
            wait(('q', 0), ('q', 1))
            R.ln1(0); R.ln1(1)
        md = {}
        with scope("p_mod"):
            for nm in ['ca', 'sa', 'ga', 'cb', 'sb']:
                wait(('wm', nm))
                md[nm] = R.modpart(nm)
            mv[0:8, :] = md['ga'] * (1.0 + md['ca'])
            mv[8:16, :] = md['ga'] * md['sa']
            mv[16:24, :] = 1.0 + md['cb']
            mv[24:32, :] = md['sb']
        with scope("p_ln"):
            R.lnf(0, 0, hf, 0, 0, True); R.lnf(1, 0, hf, HT, 1, True)
        x = lambda: pltpu.bitcast(hf[0], bf16)
        with scope("f_w0"):
            wait(('wg', 0), ('wu', 0))
        with scope("f_a"):
            R.g_(x, 0); R.u_(x, 0)
        with scope("f_w1"):
            wait(('wd', 0), ('wg', 1), ('wu', 1), ('wd', 1))
        with scope("f_b"):
            R.d_(0); R.g_(x, 1); R.u_(x, 1); R.d_(1)
        with scope("f_w2"):
            wait(('wg', 2), ('wu', 2), ('wd', 2), ('wm', 'gb'), *kvs(2), ('q', 2), *kvs(3))
        with scope("f_c"):
            mv[32:40, :] = R.modpart('gb')
            R.sconv(2, 2)
            R.g_(x, 2)
            R.fwd(2)
            R.mac(2, CFG['k4f'], CFG['treef'])
            R.u_(x, 2)
            R.inv()
            R.lnf(2, LAG, hn_v, 0)
            R.sconv(3, 2)
            R.d_(2)
            R.fin(0, 2)
            R.fwd(3)
            cp(('o', 0)).start(); cp(('o', 1)).start()

    def steady():
        R = Reg()
        s = pid + 1
        nxt = jnp.minimum(s + 2, NS - 1)
        with scope("s_w"):
            wait(('q', s + 1))
            @pl.when(s + 2 < NS)
            def _():
                wait(*kvs(s + 2))
        with scope("s"):
            xv = pltpu.bitcast(hn_v[0, 0:HT, :], bf16)
            x = lambda: xv
            R.mac(s + 1, CFG['k4'], CFG['tree'])
            R.g_(x, 0); R.u_(x, 0); R.d_(0); R.g_(x, 1); R.u_(x, 1); R.d_(1)
            R.inv()
            R.lnf(s + 1, LAG, hn_v, 0)
            R.tail(x, s, 1, s + 2, nxt, CFG['sc_lanes'])
            cp(('o', s)).start()

    def last():
        R = Reg()
        with scope("l"):
            x = lambda: pltpu.bitcast(hn_v[0, 0:HT, :], bf16)
            for c in range(NC):
                R.g_(x, c); R.u_(x, c); R.d_(c)
            R.fin(NS - 1, 1)
            cp(('o', NS - 1)).start()
        with scope("e_w"):
            for t in range(NS):
                cp(('o', t)).wait()

    only = CFG['only']
    if only is None or 0 in only:
        pl.when(pid == 0)(first)
    if only is None or 1 in only:
        pl.when(jnp.logical_and(pid >= 1, pid <= NS - 3))(steady)
    if only is None or 2 in only:
        pl.when(pid == NS - 2)(last)


@jax.jit
def pallas_adaLN_cond__ssm_conv_h3__glu_gated_reglu__prompt_kernel(A_q, A_k, A_v, A_shift_k, A_ssm_k, A_ssm_D, B_x, B_W_gate, B_W_up, B_W_down, c, w_mod):
    fwd, inv = _dft_mats()
    fw = jnp.asarray(fwd, bf16)
    iv = jnp.asarray(inv, bf16)
    any_spec = pl.BlockSpec(memory_space=pl.ANY)
    dma = pltpu.SemaphoreType.DMA
    return pl.pallas_call(
        kernel,
        grid=(NS - 1,),
        in_specs=[any_spec] * 13,
        out_specs=any_spec,
        out_shape=jax.ShapeDtypeStruct((1, S, D), bf16),
        scratch_shapes=[
            pltpu.VMEM((NS, T, D), bf16), pltpu.VMEM((NS, T, D), bf16), pltpu.VMEM((NS, T, D), bf16),
            pltpu.VMEM((NBLK, D, NB), bf16),
            pltpu.VMEM((D, F), bf16), pltpu.VMEM((D, F), bf16), pltpu.VMEM((F, D), bf16),
            pltpu.VMEM((D, 6 * D), bf16),
            pltpu.VMEM((2 * NB, NB), bf16), pltpu.VMEM((NB, 2 * NB), bf16),
            pltpu.VMEM((NS, T, D), bf16),
            pltpu.VMEM((NW, NG, 32, D), f32),
            pltpu.VMEM((1, 2 * NB, D), f32),
            pltpu.VMEM((1, T + 32, D), f32),
            pltpu.VMEM((1, HT + 32, D), f32),
            pltpu.VMEM((64, D), f32),
            pltpu.VMEM((1, 2 * T, D), f32),
            pltpu.VMEM((NS, T, D), f32),
            pltpu.VMEM((1, HT + 32, D), f32),
            pltpu.VMEM((1, T, D), f32),
            pltpu.VMEM((2, T, D), f32),
            pltpu.VMEM((4, D), bf16), pltpu.VMEM((D,), bf16), pltpu.VMEM((1, D), bf16),
            dma((5 + 6 + 3 * NC + 3 * NS + NBLK,)), dma((NS,)),
        ],
        compiler_params=pltpu.CompilerParams(vmem_limit_bytes=110 * 1024 * 1024,
                                             dimension_semantics=("arbitrary",)),
    )(A_q, A_k, A_v, A_shift_k.T, A_ssm_k, A_ssm_D, B_W_gate, B_W_up, B_W_down, c, w_mod, fw, iv)
```

```python
import contextlib
import numpy as np
import jax
import jax.numpy as jnp
from jax import lax
from jax.experimental import pallas as pl
from jax.experimental.pallas import tpu as pltpu

S, D, F = 2048, 640, 1536
NB = 128
T = 256
NS = S // T
NBLK = S // NB
FC = 512
NC = F // FC
NQ = FC // 128
NL = D // 128
NG = NB // 8
HT = T // 2
RG = 16
EPS = 1e-5
f32 = jnp.float32
bf16 = jnp.bfloat16
i32 = jnp.int32

CFG = dict(only=None, scopes=False, tree=(2, 5), hpos=(2, 3, 4, 5, 6), sc_lanes=2, lnent=4,
           fhpos=(0, 1, 2, 3, 4))

MPOS = {'sa': 0, 'ca': 1, 'ga': 2, 'sb': 3, 'cb': 4, 'gb': 5}


def _dft_mats():
    f = np.concatenate([np.arange(0, NB, 2), np.arange(1, NB, 2)])
    j = np.arange(NB)
    ang = 2.0 * np.pi * (((2 * f[:, None] + 1) * j[None, :]) % (4 * NB)) / (4 * NB)
    fwd = np.stack([np.cos(ang).reshape(NG, 8, NB), np.sin(ang).reshape(NG, 8, NB)], axis=1).reshape(2 * NB, NB)
    return fwd.astype(np.float32), (fwd.T / NB).astype(np.float32)


def _kvs(s):
    return [('k', s), ('v', s), ('s', 2 * s), ('s', 2 * s + 1)]


GROUPS = [
    ['sh', 'dd', 'c', 'fw', 'iv'] + _kvs(0),
    [('q', 0), ('q', 1)],
    _kvs(1),
    [('wm', 0)], [('wm', 1)], [('wm', 2)], [('wm', 4)], [('wm', 3)],
    [('wgh', 0)],
    [('wgh', 1), ('wuh', 0)],
    [('wuh', 1), ('wd', 0)],
    _kvs(2) + [('wg', 1), ('wu', 1)],
    [('wd', 1), ('wg', 2)],
    [('wu', 2), ('wd', 2), ('wm', 5), ('q', 2)] + _kvs(3),
]
G_STEADY = len(GROUPS)
for _s in range(2, NS - 2):
    GROUPS.append([('q', _s + 1)] + _kvs(_s + 2))
GROUPS.append([('q', NS - 1)])


def _kernel(q_hbm, k_hbm, v_hbm, sh_hbm, ssm_hbm, dd_hbm, wg_hbm, wu_hbm, wd_hbm, c_hbm, wm_hbm,
            fw_hbm, iv_hbm, o_hbm,
            q_v, k_v, v_v, ssm_v, wg_v, wu_v, wd_v, wm_v, fw_v, iv_v, o_v,
            uv, ap, zb, kvb, mv, yb, x1b, hn_v, hf, n1, n2, ab, accb, tp, sh_v, dd_v, c_v,
            sems, osem):
    pid = pl.program_id(0)

    def blk(j, n):
        return pl.ds(j * n, n) if isinstance(j, int) else pl.ds(pl.multiple_of(j * n, n), n)

    small = {'sh': (sh_hbm, sh_v), 'dd': (dd_hbm, dd_v), 'c': (c_hbm, c_v), 'fw': (fw_hbm, fw_v),
             'iv': (iv_hbm, iv_v)}

    def copy(name, gi):
        sem = sems.at[gi]
        if isinstance(name, str):
            return pltpu.make_async_copy(small[name][0], small[name][1], sem)
        kind, j = name
        if kind in ('q', 'k', 'v'):
            src, dst = {'q': (q_hbm, q_v), 'k': (k_hbm, k_v), 'v': (v_hbm, v_v)}[kind]
            return pltpu.make_async_copy(src.at[0, blk(j, T), :], dst.at[j], sem)
        if kind == 's':
            return pltpu.make_async_copy(ssm_hbm.at[:, blk(j, NB)], ssm_v.at[j], sem)
        if kind == 'wm':
            return pltpu.make_async_copy(wm_hbm.at[:, blk(j, D)], wm_v.at[j], sem)
        if kind == 'wd':
            return pltpu.make_async_copy(wd_hbm.at[blk(j, FC), :], wd_v.at[blk(j, FC), :], sem)
        src, dst = (wg_hbm, wg_v) if kind[1] == 'g' else (wu_hbm, wu_v)
        cols = blk(j, FC // 2) if kind.endswith('h') else blk(j, FC)
        return pltpu.make_async_copy(src.at[:, cols], dst.at[:, cols], sem)

    def wait_group(gi):
        for name in GROUPS[gi]:
            copy(name, gi).wait()

    def ocopy(j):
        return pltpu.make_async_copy(o_v.at[j], o_hbm.at[0, blk(j, T), :], osem.at[0])

    def scope(name):
        return jax.named_scope(name) if CFG['scopes'] else contextlib.nullcontext()

    def pack(x):
        return pltpu.bitcast(x.astype(bf16), f32)

    def unpack(x):
        return pltpu.bitcast(x, bf16)

    def rowsum(x, tok=None):
        ps = x[:, 0:128]
        if tok is not None:
            ps = ps + jnp.concatenate([tok] * (x.shape[0] // 8), axis=0)
        for lc in range(1, NL):
            ps = ps + x[:, lc * 128:(lc + 1) * 128]
        return jnp.sum(ps, axis=-1, keepdims=True)

    def normalise(x, tok=None):
        xc = x - rowsum(x) * (1.0 / D)
        var = rowsum(xc * xc, tok) * (1.0 / D) + EPS
        return xc * lax.rsqrt(var)

    def fold(a, p):
        parts = []
        for g in range(NG):
            ar, ai = a[16 * g:16 * g + 8], a[16 * g + 8:16 * g + 16]
            pr, pi = p[16 * g:16 * g + 8], p[16 * g + 8:16 * g + 16]
            parts += [ar + pi, ai - pr] if g < NG // 2 else [ar - pi, ai + pr]
        return jnp.concatenate(parts, axis=0)

    def grp(x):
        return x.reshape(NG, 16, 128)

    row = lax.broadcasted_iota(i32, (8, 128), 0)

    def conv_rows(s, ls, emit, tok_in=None):
        w = [tp[8 * j:8 * j + 8, ls] for j in range(4)]
        if isinstance(s, int) and s == 0:
            pk = jnp.zeros((8, 128), f32)
            pt = jnp.zeros((8, 128), f32)
        else:
            kp = k_v[s - 1, T - 16:T, ls].astype(f32)[8:16]
            pk = pltpu.roll(kp, 1, 0)
            pt = pltpu.roll(w[2] * kp + w[3] * pk, 2, 0)
        for rg in range(T // 16):
            kk = k_v[s, rg * 16:rg * 16 + 16, ls].astype(f32)
            vv = v_v[s, rg * 16:rg * 16 + 16, ls].astype(f32)
            outs = []
            for h in range(2):
                kc = kk[8 * h:8 * h + 8]
                if h == 0 and tok_in is not None and tok_in() is not None:
                    kc = kc + tok_in()
                rk = pltpu.roll(kc, 1, 0)
                sk = jnp.where(row < 1, pk, rk)
                t = w[2] * kc + w[3] * sk
                rt = pltpu.roll(t, 2, 0)
                outs.append(((w[0] * kc + w[1] * sk) + jnp.where(row < 2, pt, rt)) * vv[8 * h:8 * h + 8])
                pk, pt = rk, rt
            emit(rg, pack(jnp.concatenate(outs, axis=0)))

    def dft_x(kv0, kv1, split=False):
        w = unpack(jnp.concatenate([kv0, kv1], axis=1))
        if split:
            xx = jnp.concatenate([jnp.dot(fw_v[h * NB:(h + 1) * NB, :], w, preferred_element_type=f32)
                                  for h in range(2)], axis=0)
        else:
            xx = jnp.dot(fw_v[...], w, preferred_element_type=f32)
        return xx[:, 0:128], xx[:, 128:256]

    def dft_h(s, rows):
        w = jnp.concatenate([ssm_v[2 * s, rows, :], ssm_v[2 * s + 1, rows, :]], axis=0)
        aa = lax.dot_general(fw_v[...], w, (((1,), (1,)), ((), ())), preferred_element_type=f32)
        return aa[:, 0:128], aa[:, 128:256]

    class Reg:
        def __init__(self):
            self.z0 = lax.shift_right_logical(pid, 8)
            self.st = {}

        def sconv(self, s, lanes, lcs=None):
            if lcs is None or lcs[0] == 0:
                self.sc = [None] * lanes
                self.gi = 0
            for lc in (range(NL) if lcs is None else lcs):
                ls = pl.ds(lc * 128, 128)

                def emit(rg, kvp, ls=ls):
                    kvb.at[self.z0][rg * 8:rg * 8 + 8, ls] = kvp
                    self.sc[self.gi % lanes] = kvb[0, HT:HT + 8, ls]
                    self.gi += 1
                conv_rows(s, ls, emit, lambda: self.sc[self.gi % lanes])

        def fwd_x(self, s, lc):
            o = self.z0 + 3 * s
            ls = pl.ds(lc * 128, 128)
            x0, x1 = dft_x(kvb[0, 0:64, ls], kvb[0, 64:128, ls])
            p = 3 * (s - 1)
            u1 = (uv[p + 2, :, 16:32, ls] + uv[p, :, 16:32, ls]) - grp(x0)
            uv[o, :, 16:32, ls] = grp(x0)
            uv[o + 1, :, 16:32, ls] = u1
            uv[o + 2, :, 16:32, ls] = grp(x1 - x0)

        def fwd_h(self, s, lc):
            o = self.z0 + 3 * s
            ls = pl.ds(lc * 128, 128)
            a0, a1 = dft_h(s, ls)
            h0 = fold(a0, ap[0, :, ls])
            h1 = fold(a1, a0)
            uv[o, :, 0:16, ls] = grp(h0 + h1)
            uv[o + 1, :, 0:16, ls] = grp(h1)
            uv[o + 2, :, 0:16, ls] = grp(h0)
            ap[self.z0, :, ls] = a1

        def mac(self, s, tree=()):
            static = isinstance(s, int)
            ng = s + 1 if static else NS - 1
            ub = [3 * (s - g) if static else 3 * jnp.maximum(s - g, 0) for g in range(ng)]
            toks = (None, None)
            for fc in range(NG):
                for lc in range(NL):
                    ls = pl.ds(lc * 128, 128)

                    def chain(j, ar, ai):
                        for g in range(ng):
                            hr = uv[3 * g + j, fc, 0:8, ls]
                            hi = uv[3 * g + j, fc, 8:16, ls]
                            xr = uv[ub[g] + j, fc, 16:24, ls]
                            xi = uv[ub[g] + j, fc, 24:32, ls]
                            if ar is not None and g in tree:
                                ar = ar + (hr * xr - hi * xi)
                                ai = ai + (hr * xi + hi * xr)
                            else:
                                ar = (hr * xr if ar is None else ar + hr * xr) - hi * xi
                                ai = (hr * xi if ai is None else ai + hr * xi) + hi * xr
                        return ar, ai

                    a1 = chain(0, *toks)
                    z0 = chain(1, *a1)
                    zero = pltpu.bitcast(zb[0, T:T + 8, ls], i32)

                    def tk(v):
                        return pltpu.bitcast(pltpu.bitcast(v, i32) & zero, f32)
                    z1 = chain(2, a1[0] + tk(z0[0]), a1[1] + tk(z0[1]))
                    for b, z in enumerate((z0, z1)):
                        zb.at[self.z0][b * HT + fc * 8:b * HT + fc * 8 + 8, ls] = pack(jnp.concatenate(z, axis=0))
                    toks = (tk(z1[0]), tk(z1[1]))

        def inv(self):
            for b in range(2):
                yb[self.z0, b * NB:(b + 1) * NB, :] = jnp.dot(
                    iv_v[...], unpack(zb[0, b * HT:(b + 1) * HT, :]), preferred_element_type=f32)

        def ln(self, s):
            a1 = mv[0:1, :]; a0 = mv[8:9, :]; b1 = mv[16:17, :]; b0 = mv[24:25, :]
            tok = None
            for g in range(T // RG):
                gr = slice(g * RG, (g + 1) * RG)
                x = q_v[s, gr, :].astype(f32)
                x1 = x + (normalise(x) * a1 + a0) * yb[0, gr, :]
                x1b[self.z0 + s, gr, :] = x1
                h2 = normalise(x1, tok) * b1 + b0
                hn_v.at[self.z0][g * (RG // 2):(g + 1) * (RG // 2), :] = pack(h2)
                tok = hn_v[0, HT:HT + 8, 0:128]

        def gcols(self, x, c0, n):
            return jnp.dot(x(), wg_v[:, c0:c0 + n], preferred_element_type=f32)

        def ucols(self, x, c0, n):
            return jnp.dot(x(), wu_v[:, c0:c0 + n], preferred_element_type=f32)

        def g_(self, x, c):
            self.st['g'] = self.gcols(x, c * FC, FC)

        def u_(self, x, c):
            self.st['a'] = (jnp.maximum(self.st.pop('g'), 0.0) * self.ucols(x, c * FC, FC)).astype(bf16)

        def d_(self, c):
            d = jnp.dot(self.st.pop('a'), wd_v[c * FC:(c + 1) * FC, :], preferred_element_type=f32)
            self.st['acc'] = d if c == 0 else self.st['acc'] + d

        def gp(self, x, c, j):
            self.st[('g', j)] = self.gcols(x, c * FC + j * 128, 128)

        def up(self, x, c, j):
            g = self.st.pop(('g', j)) if ('g', j) in self.st else self.st['g'][:, j * 128:(j + 1) * 128]
            self.st[('a', j)] = jnp.maximum(g, 0.0) * self.ucols(x, c * FC + j * 128, 128)
            if j == NQ - 1:
                self.st['a'] = jnp.concatenate([self.st.pop(('a', i)) for i in range(NQ)], axis=1).astype(bf16)

        def dp(self, c, lc, s=None, n=None):
            ls = pl.ds(lc * 128, 128)
            d = jnp.dot(self.st['a'], wd_v[c * FC:(c + 1) * FC, ls], preferred_element_type=f32)
            d = self.st['acc'][:, lc * 128:(lc + 1) * 128] + d
            if c == NC - 1:
                for j in range(n):
                    o_v[s + j, :, ls] = (x1b[s + j, :, ls] + mv[32:33, ls] * d[j * T:(j + 1) * T]).astype(bf16)
            else:
                self.st[('d', lc)] = d
                if lc == NL - 1:
                    self.st['acc'] = jnp.concatenate([self.st.pop(('d', i)) for i in range(NL)], axis=1)

        def tail(self, x, s, n, fs, with_g, hpos, scall):
            c = NC - 1
            k = 0
            hq = 0
            pieces = ([lambda j=j: self.gp(x, c, j) for j in range(NQ)] if with_g else [])
            pieces += [lambda j=j: self.up(x, c, j) for j in range(NQ)]
            for p in pieces:
                p()
                while hq < NL and hpos[hq] == k:
                    self.fwd_h(fs, hq); hq += 1
                k += 1
            for lc in range(NL):
                self.dp(c, lc, s, n)
                while hq < NL and hpos[hq] == k:
                    self.fwd_h(fs, hq); hq += 1
                k += 1
                if not scall:
                    self.sconv(fs, CFG['sc_lanes'], [lc])
                elif lc == 0:
                    self.sconv(fs, CFG['sc_lanes'])
                self.fwd_x(fs, lc)

        def fin(self, s):
            o_v[s] = (x1b[s] + mv[32:33, :] * self.st.pop('acc')).astype(bf16)

    def modvec(p):
        c32 = c_v[...].astype(f32)
        sc8 = jnp.broadcast_to((c32 * jax.nn.sigmoid(c32)).astype(bf16), (8, D))
        return jnp.dot(sc8, wm_v[p], preferred_element_type=f32)

    def first():
        R = Reg()
        for gi, names in enumerate(GROUPS):
            for name in names:
                copy(name, gi).start()
        z = jnp.zeros((8, D), f32)
        kvb[0, HT:HT + 8, :] = z
        hn_v[0, HT:HT + 8, :] = z
        zb[0, T:T + 8, :] = z

        def zero_v(j, _):
            uv[j, :, 0:16, :] = jnp.zeros((NG, 16, D), f32)
            return 0
        lax.fori_loop(12, 3 * (NS - 1), zero_v, 0)

        def cmul(h, x):
            return (h[:, 0:8] * x[:, 0:8] - h[:, 8:16] * x[:, 8:16], h[:, 0:8] * x[:, 8:16] + h[:, 8:16] * x[:, 0:8])

        def conv_pair(s):
            def body(lc, _):
                ls = blk(lc, 128)
                if s == 1:
                    for k in range(7):
                        g = jnp.minimum(lc * 7 + k, 2 * T // RG - 1)
                        gr = blk(g % (T // RG), RG)
                        n1[g // (T // RG), gr, :] = normalise(q_v[g // (T // RG), gr, :].astype(f32))
                rows = []
                conv_rows(s, ls, lambda rg, kvp: rows.append(kvp))
                a0, a1 = dft_h(s, ls)
                x0, x1 = dft_x(jnp.concatenate(rows[0:8], axis=0), jnp.concatenate(rows[8:16], axis=0), True)
                if s == 0:
                    dd = tp[32:40, ls]
                    h0 = jnp.concatenate([a0[8 * g:8 * g + 8] + dd if g % 2 == 0 else a0[8 * g:8 * g + 8]
                                          for g in range(2 * NG)], axis=0)
                    u1 = grp(-x0)
                else:
                    h0 = fold(a0, ap[0, :, ls])
                    u1 = (uv[2, :, 16:32, ls] + uv[0, :, 16:32, ls]) - grp(x0)
                h1 = fold(a1, a0)
                us = [grp(x0), u1, grp(x1 - x0)]
                vs = [grp(h0 + h1), grp(h1), grp(h0)]
                if s == 0:
                    p = [cmul(vs[j], us[j]) for j in range(3)]
                else:
                    p = []
                    for j in range(3):
                        t0 = cmul(uv[j, :, 0:16, ls], us[j])
                        t1 = cmul(vs[j], uv[j, :, 16:32, ls])
                        p.append((t0[0] + t1[0], t0[1] + t1[1]))
                for j in range(3):
                    uv[3 * s + j, :, 16:32, ls] = us[j]
                    uv[3 * s + j, :, 0:16, ls] = vs[j]
                ap[0, :, ls] = a1
                for b in range(2):
                    zz = jnp.concatenate([p[0][0] + p[1 + b][0], p[0][1] + p[1 + b][1]], axis=1)
                    yb[0, (2 * s + b) * NB:(2 * s + b + 1) * NB, ls] = jnp.dot(
                        iv_v[...], zz.reshape(2 * NB, 128).astype(bf16), preferred_element_type=f32)
                return 0
            lax.fori_loop(0, NL, body, 0)

        with scope("p_w0"):
            wait_group(0)
        with scope("p_c0"):
            taps = sh_v[...].astype(f32)
            for j in range(4):
                tp[8 * j:8 * j + 8, :] = jnp.broadcast_to(taps[j:j + 1, :], (8, D))
            tp[32:40, :] = jnp.broadcast_to(dd_v[...].astype(f32).reshape(1, D), (8, D))
            conv_pair(0)
        with scope("p_c1"):
            wait_group(1)
            wait_group(2)
            conv_pair(1)
        with scope("p_mod"):
            for gi in (3, 4, 5):
                wait_group(gi)
            sa, ca, ga = modvec(0), modvec(1), modvec(2)
            mv[0:8, :] = ga * (1.0 + ca)
            mv[8:16, :] = ga * sa
        with scope("p_ln2"):
            def ln2(i, _):
                for g in range(T // RG):
                    gr = slice(g * RG, (g + 1) * RG)
                    x = q_v[i, gr, :].astype(f32)
                    y = yb[0, pl.ds(pl.multiple_of(i * T + g * RG, RG), RG), :]
                    x1 = x + (n1[i, gr, :] * mv[0:1, :] + mv[8:9, :]) * y
                    x1b[i, gr, :] = x1
                    n2[i, gr, :] = normalise(x1)
                return 0
            lax.fori_loop(0, 2, ln2, 0)
        with scope("p_mod2"):
            def mod2(i, _):
                copy(('wm', 4 - i), 6 + i).wait()
                mv[blk(2 + i, 8), :] = modvec(4 - i) + (1 - i).astype(f32)
                return 0
            lax.fori_loop(0, 2, mod2, 0)
            for s in range(2):
                hf.at[R.z0][s * HT:(s + 1) * HT, :] = pack(n2[s] * mv[16:17, :] + mv[24:25, :])
        x = lambda: unpack(hf[0])
        xh = [lambda h=h: unpack(hf[0, h * HT:(h + 1) * HT, :]) for h in range(2)]
        HC = FC // 2
        gbuf = accb.at[R.z0]
        with scope("f_a"):
            wait_group(8)
            for h in range(2):
                gbuf[h * T:(h + 1) * T, 0:HC] = R.gcols(xh[h], 0, HC)
        with scope("f_b"):
            wait_group(9)
            ab.at[R.z0][:, 0:HC] = pack(jnp.maximum(accb[0, :, 0:HC], 0.0) * R.ucols(x, 0, HC))
            gbuf[:, HC:FC] = R.gcols(x, HC, HC)
        with scope("f_c"):
            wait_group(10)
            a2 = (jnp.maximum(accb[0, :, HC:FC], 0.0) * R.ucols(x, HC, HC)).astype(bf16)
            da = jnp.dot(unpack(ab[0, :, 0:HC]), wd_v[0:HC, :], preferred_element_type=f32)
            for h in range(2):
                gbuf[h * T:(h + 1) * T, :] = da[h * T:(h + 1) * T] + jnp.dot(
                    a2[h * T:(h + 1) * T], wd_v[HC:FC, :], preferred_element_type=f32)
        with scope("f_d"):
            wait_group(11)
            R.fwd_h(2, 0)
            for j in range(NQ):
                R.gp(x, 1, j)
                R.fwd_h(2, j + 1)
            for j in range(NQ):
                R.sconv(2, 2, [j])
                R.fwd_x(2, j)
                R.up(x, 1, j)
            R.sconv(2, 2, [NL - 1])
            R.fwd_x(2, NL - 1)
            ab[R.z0] = pltpu.bitcast(R.st.pop('a'), f32)
        with scope("f_e"):
            wait_group(12)
            R.st['a'] = unpack(ab[0])
            R.st['acc'] = accb[0]
            R.mac(2)
            R.d_(1); R.g_(x, 2)
            R.inv()
        with scope("f_f"):
            wait_group(13)
            mv[32:40, :] = modvec(MPOS['gb'])
            R.ln(2)
            R.tail(x, 0, 2, 3, False, CFG['fhpos'], False)
            ocopy(0).start(); ocopy(1).start()

    def steady():
        R = Reg()
        s = pid + 1
        with scope("s_w"):
            for name in [('q', s + 1)] + _kvs(s + 2):
                copy(name, G_STEADY + s - 2).wait()
        with scope("s"):
            xv = unpack(hn_v[0, 0:HT, :])
            x = lambda: xv
            R.mac(s + 1, CFG['tree'])
            R.g_(x, 0); R.u_(x, 0); R.d_(0); R.g_(x, 1); R.u_(x, 1)
            R.inv()
            R.ln(s + 1)
            for lc in range(NL):
                R.dp(1, lc)
            R.tail(x, s, 1, s + 2, True, CFG['hpos'], True)
            ocopy(s).start()

    def last():
        R = Reg()
        s = NS - 2
        with scope("l_w"):
            wait_group(len(GROUPS) - 1)
        with scope("l"):
            xv = unpack(hn_v[0, 0:HT, :])
            x = lambda: xv
            R.mac(s + 1, (2, 5))
            R.g_(x, 0); R.u_(x, 0); R.d_(0); R.g_(x, 1); R.u_(x, 1); R.d_(1)
            R.inv()
            R.ln(s + 1)
            R.g_(x, 2); R.u_(x, 2); R.d_(2)
            R.fin(s)
            ocopy(s).start()
            x = lambda: unpack(hn_v[0, 0:HT, :])
            for c in range(NC):
                R.g_(x, c); R.u_(x, c); R.d_(c)
            R.fin(s + 1)
            ocopy(s + 1).start()
        with scope("e_w"):
            for t in range(NS):
                ocopy(t).wait()

    only = CFG['only']
    if only is None or 0 in only:
        pl.when(pid == 0)(first)
    if only is None or 1 in only:
        pl.when(jnp.logical_and(pid >= 1, pid <= NS - 4))(steady)
    if only is None or 2 in only:
        pl.when(pid == NS - 3)(last)


@jax.jit
def pallas_adaLN_cond__ssm_conv_h3__glu_gated_reglu__prompt_kernel(A_q, A_k, A_v, A_shift_k, A_ssm_k, A_ssm_D, B_x, B_W_gate, B_W_up, B_W_down, c, w_mod):
    fwd, inv = _dft_mats()
    any_spec = pl.BlockSpec(memory_space=pl.ANY)
    vm = pltpu.VMEM
    return pl.pallas_call(
        _kernel,
        grid=(NS - 2,),
        in_specs=[any_spec] * 13,
        out_specs=any_spec,
        out_shape=jax.ShapeDtypeStruct((1, S, D), bf16),
        scratch_shapes=[
            vm((NS, T, D), bf16), vm((NS, T, D), bf16), vm((NS, T, D), bf16),
            vm((NBLK, D, NB), bf16),
            vm((D, F), bf16), vm((D, F), bf16), vm((F, D), bf16),
            vm((6, D, D), bf16),
            vm((2 * NB, NB), bf16), vm((NB, 2 * NB), bf16),
            vm((NS, T, D), bf16),
            vm((3 * NS, NG, 32, D), f32),
            vm((1, 2 * NB, D), f32),
            vm((1, T + 32, D), f32),
            vm((1, HT + 32, D), f32),
            vm((64, D), f32),
            vm((1, 2 * T, D), f32),
            vm((NS, T, D), f32),
            vm((1, HT + 32, D), f32),
            vm((1, T, D), f32),
            vm((2, T, D), f32),
            vm((2, T, D), f32),
            vm((1, T, FC), f32),
            vm((1, 2 * T, D), f32),
            vm((64, D), f32),
            vm((4, D), bf16), vm((D,), bf16), vm((1, D), bf16),
            pltpu.SemaphoreType.DMA((len(GROUPS),)), pltpu.SemaphoreType.DMA((1,)),
        ],
        compiler_params=pltpu.CompilerParams(vmem_limit_bytes=110 * 1024 * 1024,
                                             dimension_semantics=("arbitrary",)),
    )(A_q, A_k, A_v, A_shift_k.T, A_ssm_k, A_ssm_D, B_W_gate, B_W_up, B_W_down, c, w_mod,
      jnp.asarray(fwd, bf16), jnp.asarray(inv, bf16))
```

```python
import contextlib
import numpy as np
import jax
import jax.numpy as jnp
from jax import lax
from jax.experimental import pallas as pl
from jax.experimental.pallas import tpu as pltpu

S, D, F = 2048, 640, 1536
NB = 128
T = 256
NS = S // T
NBLK = S // NB
FC = 512
NC = F // FC
NQ = FC // 128
NL = D // 128
NG = NB // 8
HT = T // 2
RG = 16
EPS = 1e-5
f32 = jnp.float32
bf16 = jnp.bfloat16
i32 = jnp.int32

CFG = dict(only=None, scopes=False, tree=(1, 2, 4, 5), hpos=(2, 3, 4, 5, 6), sc_lanes=2, lnent=3,
           fhpos=(3, 4, 5, 6, 7), premac=True, fent=4, fscall=False, gbpos=1, fdh=(-1, 0, 1, 2, 3), fdx=(3, 4, 5, 6, 7), fdl=1, fdall=True, hp=(0, 2, 4, 6, 8), xp=(10, 12, 13, 15, 17), lastsplit=((0, 128), (128, 128)))

MPOS = {'sa': 0, 'ca': 1, 'ga': 2, 'sb': 3, 'cb': 4, 'gb': 5}


def _dft_mats():
    f = np.concatenate([np.arange(0, NB, 2), np.arange(1, NB, 2)])
    j = np.arange(NB)
    ang = 2.0 * np.pi * (((2 * f[:, None] + 1) * j[None, :]) % (4 * NB)) / (4 * NB)
    fwd = np.stack([np.cos(ang).reshape(NG, 8, NB), np.sin(ang).reshape(NG, 8, NB)], axis=1).reshape(2 * NB, NB)
    return fwd.astype(np.float32), (fwd.T / NB).astype(np.float32)


def _kvs(s):
    return [('k', s), ('v', s), ('s', 2 * s), ('s', 2 * s + 1)]


GROUPS = [
    ['sh', 'dd', 'c', 'fw', 'iv'] + _kvs(0),
    [('q', 0), ('q', 1)],
    _kvs(1),
    [('wm', 0)], [('wm', 1)], [('wm', 2)], [('wm', 4)], [('wm', 3)],
    [('wgh', 0)],
    [('wgh', 1), ('wuh', 0)],
    [('wuh', 1), ('wd', 0)],
    _kvs(2) + [('wg', 1), ('wu', 1)],
    [('wd', 1), ('wg', 2), ('wm', 5)],
    [('wu', 2), ('wd', 2), ('q', 2)] + _kvs(3),
]
G_STEADY = len(GROUPS)
for _s in range(2, NS - 2):
    GROUPS.append([('q', _s + 1)] + _kvs(_s + 2))
GROUPS.append([('q', NS - 1)])


def _kernel(q_hbm, k_hbm, v_hbm, sh_hbm, ssm_hbm, dd_hbm, wg_hbm, wu_hbm, wd_hbm, c_hbm, wm_hbm,
            fw_hbm, iv_hbm, o_hbm,
            q_v, k_v, v_v, ssm_v, wg_v, wu_v, wd_v, wm_v, fw_v, iv_v, o_v,
            uv, ap, zb, kvb, mv, yb, x1b, hn_v, hf, n1, n2, ab, accb, tp, sh_v, dd_v, c_v,
            sems, osem):
    pid = pl.program_id(0)

    def blk(j, n):
        return pl.ds(j * n, n) if isinstance(j, int) else pl.ds(pl.multiple_of(j * n, n), n)

    small = {'sh': (sh_hbm, sh_v), 'dd': (dd_hbm, dd_v), 'c': (c_hbm, c_v), 'fw': (fw_hbm, fw_v),
             'iv': (iv_hbm, iv_v)}

    def copy(name, gi):
        sem = sems.at[gi]
        if isinstance(name, str):
            return pltpu.make_async_copy(small[name][0], small[name][1], sem)
        kind, j = name
        if kind in ('q', 'k', 'v'):
            src, dst = {'q': (q_hbm, q_v), 'k': (k_hbm, k_v), 'v': (v_hbm, v_v)}[kind]
            return pltpu.make_async_copy(src.at[0, blk(j, T), :], dst.at[j], sem)
        if kind == 's':
            return pltpu.make_async_copy(ssm_hbm.at[:, blk(j, NB)], ssm_v.at[j], sem)
        if kind == 'wm':
            return pltpu.make_async_copy(wm_hbm.at[:, blk(j, D)], wm_v.at[j], sem)
        if kind == 'wd':
            return pltpu.make_async_copy(wd_hbm.at[blk(j, FC), :], wd_v.at[blk(j, FC), :], sem)
        src, dst = (wg_hbm, wg_v) if kind[1] == 'g' else (wu_hbm, wu_v)
        cols = blk(j, FC // 2) if kind.endswith('h') else blk(j, FC)
        return pltpu.make_async_copy(src.at[:, cols], dst.at[:, cols], sem)

    def wait_group(gi):
        for name in GROUPS[gi]:
            copy(name, gi).wait()

    def ocopy(j, h=None):
        if h is None:
            return pltpu.make_async_copy(o_v.at[j], o_hbm.at[0, blk(j, T), :], osem.at[0])
        r0, n = h
        return pltpu.make_async_copy(o_v.at[j, pl.ds(r0, n), :], o_hbm.at[0, pl.ds(j * T + r0, n), :], osem.at[0])

    def scope(name):
        return jax.named_scope(name) if CFG['scopes'] else contextlib.nullcontext()

    def pack(x):
        return pltpu.bitcast(x.astype(bf16), f32)

    def unpack(x):
        return pltpu.bitcast(x, bf16)

    def rowsum(x, tok=None):
        ps = x[:, 0:128]
        if tok is not None:
            ps = ps + jnp.concatenate([tok] * (x.shape[0] // 8), axis=0)
        for lc in range(1, NL):
            ps = ps + x[:, lc * 128:(lc + 1) * 128]
        return jnp.sum(ps, axis=-1, keepdims=True)

    def normalise(x, tok=None, ent=4):
        xc = x - rowsum(x, tok if ent == 3 else None) * (1.0 / D)
        var = rowsum(xc * xc, tok if ent == 4 else None) * (1.0 / D) + EPS
        return xc * lax.rsqrt(var)

    def fold(a, p):
        parts = []
        for g in range(NG):
            ar, ai = a[16 * g:16 * g + 8], a[16 * g + 8:16 * g + 16]
            pr, pi = p[16 * g:16 * g + 8], p[16 * g + 8:16 * g + 16]
            parts += [ar + pi, ai - pr] if g < NG // 2 else [ar - pi, ai + pr]
        return jnp.concatenate(parts, axis=0)

    def grp(x):
        return x.reshape(NG, 16, 128)

    row = lax.broadcasted_iota(i32, (8, 128), 0)

    def conv_rows(s, ls, emit, tok_in=None):
        w = [tp[8 * j:8 * j + 8, ls] for j in range(4)]
        if isinstance(s, int) and s == 0:
            pk = jnp.zeros((8, 128), f32)
            pt = jnp.zeros((8, 128), f32)
        else:
            kp = k_v[s - 1, T - 16:T, ls].astype(f32)[8:16]
            pk = pltpu.roll(kp, 1, 0)
            pt = pltpu.roll(w[2] * kp + w[3] * pk, 2, 0)
        for rg in range(T // 16):
            kk = k_v[s, rg * 16:rg * 16 + 16, ls].astype(f32)
            vv = v_v[s, rg * 16:rg * 16 + 16, ls].astype(f32)
            outs = []
            for h in range(2):
                kc = kk[8 * h:8 * h + 8]
                if h == 0 and tok_in is not None and tok_in() is not None:
                    kc = kc + tok_in()
                rk = pltpu.roll(kc, 1, 0)
                sk = jnp.where(row < 1, pk, rk)
                t = w[2] * kc + w[3] * sk
                rt = pltpu.roll(t, 2, 0)
                outs.append(((w[0] * kc + w[1] * sk) + jnp.where(row < 2, pt, rt)) * vv[8 * h:8 * h + 8])
                pk, pt = rk, rt
            emit(rg, pack(jnp.concatenate(outs, axis=0)))

    def dft_x(kv0, kv1, split=False):
        w = unpack(jnp.concatenate([kv0, kv1], axis=1))
        if split:
            xx = jnp.concatenate([jnp.dot(fw_v[h * NB:(h + 1) * NB, :], w, preferred_element_type=f32)
                                  for h in range(2)], axis=0)
        else:
            xx = jnp.dot(fw_v[...], w, preferred_element_type=f32)
        return xx[:, 0:128], xx[:, 128:256]

    def dft_h(s, rows):
        w = jnp.concatenate([ssm_v[2 * s, rows, :], ssm_v[2 * s + 1, rows, :]], axis=0)
        aa = lax.dot_general(fw_v[...], w, (((1,), (1,)), ((), ())), preferred_element_type=f32)
        return aa[:, 0:128], aa[:, 128:256]

    class Reg:
        def __init__(self):
            self.z0 = lax.shift_right_logical(pid, 8)
            self.st = {}

        def sconv(self, s, lanes, lcs=None):
            if lcs is None or lcs[0] == 0:
                self.sc = [None] * lanes
                self.gi = 0
            for lc in (range(NL) if lcs is None else lcs):
                ls = pl.ds(lc * 128, 128)

                def emit(rg, kvp, ls=ls):
                    kvb.at[self.z0][rg * 8:rg * 8 + 8, ls] = kvp
                    self.sc[self.gi % lanes] = kvb[0, HT:HT + 8, ls]
                    self.gi += 1
                conv_rows(s, ls, emit, lambda: self.sc[self.gi % lanes])

        def fwd_x(self, s, lc):
            o = self.z0 + 3 * s
            ls = pl.ds(lc * 128, 128)
            x0, x1 = dft_x(kvb[0, 0:64, ls], kvb[0, 64:128, ls])
            p = 3 * (s - 1)
            u1 = (uv[p + 2, :, 16:32, ls] + uv[p, :, 16:32, ls]) - grp(x0)
            uv[o, :, 16:32, ls] = grp(x0)
            uv[o + 1, :, 16:32, ls] = u1
            uv[o + 2, :, 16:32, ls] = grp(x1 - x0)

        def fwd_h(self, s, lc):
            o = self.z0 + 3 * s
            ls = pl.ds(lc * 128, 128)
            a0, a1 = dft_h(s, ls)
            h0 = fold(a0, ap[0, :, ls])
            h1 = fold(a1, a0)
            uv[o, :, 0:16, ls] = grp(h0 + h1)
            uv[o + 1, :, 0:16, ls] = grp(h1)
            uv[o + 2, :, 0:16, ls] = grp(h0)
            ap[self.z0, :, ls] = a1

        def mac(self, s, tree=(), tok0=None):
            static = isinstance(s, int)
            ng = s + 1 if static else NS - 1
            ub = [3 * (s - g) if static else 3 * jnp.maximum(s - g, 0) for g in range(ng)]
            toks = (tok0, tok0)
            for fc in range(NG):
                for lc in range(NL):
                    ls = pl.ds(lc * 128, 128)

                    def chain(j, ar, ai):
                        for g in range(ng):
                            hr = uv[3 * g + j, fc, 0:8, ls]
                            hi = uv[3 * g + j, fc, 8:16, ls]
                            xr = uv[ub[g] + j, fc, 16:24, ls]
                            xi = uv[ub[g] + j, fc, 24:32, ls]
                            if ar is not None and g in tree:
                                ar = ar + (hr * xr - hi * xi)
                                ai = ai + (hr * xi + hi * xr)
                            else:
                                ar = (hr * xr if ar is None else ar + hr * xr) - hi * xi
                                ai = (hr * xi if ai is None else ai + hr * xi) + hi * xr
                        return ar, ai

                    a1 = chain(0, *toks)
                    z0 = chain(1, *a1)
                    zero = pltpu.bitcast(zb[0, T:T + 8, ls], i32)

                    def tk(v):
                        return pltpu.bitcast(pltpu.bitcast(v, i32) & zero, f32)
                    z1 = chain(2, a1[0] + tk(z0[0]), a1[1] + tk(z0[1]))
                    for b, z in enumerate((z0, z1)):
                        zb.at[self.z0][b * HT + fc * 8:b * HT + fc * 8 + 8, ls] = pack(jnp.concatenate(z, axis=0))
                    toks = (tk(z1[0]), tk(z1[1]))

        def inv(self):
            for b in range(2):
                yb[self.z0, b * NB:(b + 1) * NB, :] = jnp.dot(
                    iv_v[...], unpack(zb[0, b * HT:(b + 1) * HT, :]), preferred_element_type=f32)

        def ln(self, s, ent=4):
            a1 = mv[0:1, :]; a0 = mv[8:9, :]; b1 = mv[16:17, :]; b0 = mv[24:25, :]
            tok = None
            for g in range(T // RG):
                gr = slice(g * RG, (g + 1) * RG)
                x = q_v[s, gr, :].astype(f32)
                x1 = x + (normalise(x) * a1 + a0) * yb[0, gr, :]
                x1b[self.z0 + s, gr, :] = x1
                h2 = normalise(x1, tok, ent) * b1 + b0
                hn_v.at[self.z0][g * (RG // 2):(g + 1) * (RG // 2), :] = pack(h2)
                tok = hn_v[0, HT:HT + 8, 0:128]

        def gcols(self, x, c0, n):
            return jnp.dot(x(), wg_v[:, c0:c0 + n], preferred_element_type=f32)

        def ucols(self, x, c0, n):
            return jnp.dot(x(), wu_v[:, c0:c0 + n], preferred_element_type=f32)

        def g_(self, x, c):
            self.st['g'] = self.gcols(x, c * FC, FC)

        def u_(self, x, c):
            self.st['a'] = (jnp.maximum(self.st.pop('g'), 0.0) * self.ucols(x, c * FC, FC)).astype(bf16)

        def d_(self, c):
            d = jnp.dot(self.st.pop('a'), wd_v[c * FC:(c + 1) * FC, :], preferred_element_type=f32)
            self.st['acc'] = d if c == 0 else self.st['acc'] + d

        def gp(self, x, c, j):
            self.st[('g', j)] = self.gcols(x, c * FC + j * 128, 128)

        def up(self, x, c, j):
            g = self.st.pop(('g', j)) if ('g', j) in self.st else self.st['g'][:, j * 128:(j + 1) * 128]
            self.st[('a', j)] = jnp.maximum(g, 0.0) * self.ucols(x, c * FC + j * 128, 128)
            if j == NQ - 1:
                self.st['a'] = jnp.concatenate([self.st.pop(('a', i)) for i in range(NQ)], axis=1).astype(bf16)

        def dp(self, c, lc, s=None, n=None):
            ls = pl.ds(lc * 128, 128)
            d = jnp.dot(self.st['a'], wd_v[c * FC:(c + 1) * FC, ls], preferred_element_type=f32)
            d = self.st['acc'][:, lc * 128:(lc + 1) * 128] + d
            if c == NC - 1:
                for j in range(n):
                    o_v[s + j, :, ls] = (x1b[s + j, :, ls] + mv[32:33, ls] * d[j * T:(j + 1) * T]).astype(bf16)
            else:
                self.st[('d', lc)] = d
                if lc == NL - 1:
                    self.st['acc'] = jnp.concatenate([self.st.pop(('d', i)) for i in range(NL)], axis=1)

        def tail(self, x, s, n, fs, with_g, hpos, scall):
            c = NC - 1
            k = 0
            hq = 0
            pieces = ([lambda j=j: self.gp(x, c, j) for j in range(NQ)] if with_g else [])
            pieces += [lambda j=j: self.up(x, c, j) for j in range(NQ)]
            for p in pieces:
                p()
                while hq < NL and hpos[hq] == k:
                    self.fwd_h(fs, hq); hq += 1
                k += 1
            for lc in range(NL):
                self.dp(c, lc, s, n)
                while hq < NL and hpos[hq] == k:
                    self.fwd_h(fs, hq); hq += 1
                k += 1
                if not scall:
                    self.sconv(fs, CFG['sc_lanes'], [lc])
                elif lc == 0:
                    self.sconv(fs, CFG['sc_lanes'])
                self.fwd_x(fs, lc)

        def fin(self, s):
            o_v[s] = (x1b[s] + mv[32:33, :] * self.st.pop('acc')).astype(bf16)

    def modvec(p):
        c32 = c_v[...].astype(f32)
        sc8 = jnp.broadcast_to((c32 * jax.nn.sigmoid(c32)).astype(bf16), (8, D))
        return jnp.dot(sc8, wm_v[p], preferred_element_type=f32)

    def first():
        R = Reg()
        for gi, names in enumerate(GROUPS):
            for name in names:
                copy(name, gi).start()
        z = jnp.zeros((8, D), f32)
        kvb[0, HT:HT + 8, :] = z
        hn_v[0, HT:HT + 8, :] = z
        zb[0, T:T + 8, :] = z

        def zero_v(j, _):
            uv[j, :, 0:16, :] = jnp.zeros((NG, 16, D), f32)
            return 0
        lax.fori_loop(12, 3 * (NS - 1), zero_v, 0)

        def cmul(h, x):
            return (h[:, 0:8] * x[:, 0:8] - h[:, 8:16] * x[:, 8:16], h[:, 0:8] * x[:, 8:16] + h[:, 8:16] * x[:, 0:8])

        def conv_pair(s):
            def body(lc, _):
                ls = blk(lc, 128)
                if s == 1:
                    for k in range(7):
                        g = jnp.minimum(lc * 7 + k, 2 * T // RG - 1)
                        gr = blk(g % (T // RG), RG)
                        n1[g // (T // RG), gr, :] = normalise(q_v[g // (T // RG), gr, :].astype(f32))
                rows = []
                conv_rows(s, ls, lambda rg, kvp: rows.append(kvp))
                a0, a1 = dft_h(s, ls)
                x0, x1 = dft_x(jnp.concatenate(rows[0:8], axis=0), jnp.concatenate(rows[8:16], axis=0), True)
                if s == 0:
                    dd = tp[32:40, ls]
                    h0 = jnp.concatenate([a0[8 * g:8 * g + 8] + dd if g % 2 == 0 else a0[8 * g:8 * g + 8]
                                          for g in range(2 * NG)], axis=0)
                    u1 = grp(-x0)
                else:
                    h0 = fold(a0, ap[0, :, ls])
                    u1 = (uv[2, :, 16:32, ls] + uv[0, :, 16:32, ls]) - grp(x0)
                h1 = fold(a1, a0)
                us = [grp(x0), u1, grp(x1 - x0)]
                vs = [grp(h0 + h1), grp(h1), grp(h0)]
                if s == 0:
                    p = [cmul(vs[j], us[j]) for j in range(3)]
                else:
                    p = []
                    for j in range(3):
                        t0 = cmul(uv[j, :, 0:16, ls], us[j])
                        t1 = cmul(vs[j], uv[j, :, 16:32, ls])
                        p.append((t0[0] + t1[0], t0[1] + t1[1]))
                for j in range(3):
                    uv[3 * s + j, :, 16:32, ls] = us[j]
                    uv[3 * s + j, :, 0:16, ls] = vs[j]
                ap[0, :, ls] = a1
                for b in range(2):
                    zz = jnp.concatenate([p[0][0] + p[1 + b][0], p[0][1] + p[1 + b][1]], axis=1)
                    n2[s, b * HT:(b + 1) * HT, ls] = pack(zz.reshape(2 * NB, 128))
                return 0
            lax.fori_loop(0, NL, body, 0)

        with scope("p_w0"):
            wait_group(0)
        with scope("p_c0"):
            taps = sh_v[...].astype(f32)
            for j in range(4):
                tp[8 * j:8 * j + 8, :] = jnp.broadcast_to(taps[j:j + 1, :], (8, D))
            tp[32:40, :] = jnp.broadcast_to(dd_v[...].astype(f32).reshape(1, D), (8, D))
            conv_pair(0)
        with scope("p_c1"):
            wait_group(1)
            wait_group(2)
            conv_pair(1)

            def inv01(i, _):
                for b in range(2):
                    yb[0, pl.ds(pl.multiple_of(i * T + b * NB, NB), NB), :] = jnp.dot(
                        iv_v[...], unpack(n2[i, b * HT:(b + 1) * HT, :]), preferred_element_type=f32)
                return 0
            lax.fori_loop(0, 2, inv01, 0)
        with scope("p_mod"):
            for gi in (3, 4, 5):
                wait_group(gi)
            sa, ca, ga = modvec(0), modvec(1), modvec(2)
            mv[0:8, :] = ga * (1.0 + ca)
            mv[8:16, :] = ga * sa
        with scope("p_ln2"):
            def ln2(i, _):
                for g in range(T // RG):
                    gr = slice(g * RG, (g + 1) * RG)
                    x = q_v[i, gr, :].astype(f32)
                    y = yb[0, pl.ds(pl.multiple_of(i * T + g * RG, RG), RG), :]
                    x1 = x + (n1[i, gr, :] * mv[0:1, :] + mv[8:9, :]) * y
                    x1b[i, gr, :] = x1
                    n2[i, gr, :] = normalise(x1)
                return 0
            lax.fori_loop(0, 2, ln2, 0)
        with scope("p_mod2"):
            def mod2(i, _):
                copy(('wm', 4 - i), 6 + i).wait()
                mv[blk(2 + i, 8), :] = modvec(4 - i) + (1 - i).astype(f32)
                return 0
            lax.fori_loop(0, 2, mod2, 0)
            for s in range(2):
                hf.at[R.z0][s * HT:(s + 1) * HT, :] = pack(n2[s] * mv[16:17, :] + mv[24:25, :])
        x = lambda: unpack(hf[0])
        xh = [lambda h=h: unpack(hf[0, h * HT:(h + 1) * HT, :]) for h in range(2)]
        HC = FC // 2
        gbuf = accb.at[R.z0]
        with scope("f_a"):
            wait_group(8)
            for h in range(2):
                gbuf[h * T:(h + 1) * T, 0:HC] = R.gcols(xh[h], 0, HC)
        with scope("f_b"):
            wait_group(9)
            ab.at[R.z0][:, 0:HC] = pack(jnp.maximum(accb[0, :, 0:HC], 0.0) * R.ucols(x, 0, HC))
            gbuf[:, HC:FC] = R.gcols(x, HC, HC)
        with scope("f_c"):
            wait_group(10)
            a2 = (jnp.maximum(accb[0, :, HC:FC], 0.0) * R.ucols(x, HC, HC)).astype(bf16)
            da = jnp.dot(unpack(ab[0, :, 0:HC]), wd_v[0:HC, :], preferred_element_type=f32)
            for h in range(2):
                gbuf[h * T:(h + 1) * T, :] = da[h * T:(h + 1) * T] + jnp.dot(
                    a2[h * T:(h + 1) * T], wd_v[HC:FC, :], preferred_element_type=f32)
        with scope("f_d"):
            wait_group(11)
            pieces = [lambda: None] + [lambda j=j: R.gp(x, 1, j) for j in range(NQ)]
            pieces += [lambda j=j: R.up(x, 1, j) for j in range(NQ)]
            for k, p in enumerate(pieces):
                p()
                for lc in range(NL):
                    if CFG['fdh'][lc] == k - 1:
                        R.fwd_h(2, lc)
                for lc in range(NL):
                    if CFG['fdx'][lc] == k - 1:
                        if not CFG['fdall']:
                            R.sconv(2, CFG['fdl'], [lc])
                        elif lc == 0:
                            R.sconv(2, CFG['fdl'])
                        R.fwd_x(2, lc)
            ab[R.z0] = pltpu.bitcast(R.st.pop('a'), f32)
        with scope("f_e"):
            wait_group(12)
            R.st['a'] = unpack(ab[0])
            R.st['acc'] = accb[0]
            R.mac(2)
            if CFG['gbpos'] == 0:
                R.d_(1)
            else:
                c32 = c_v[...].astype(f32)
                sc8 = jnp.broadcast_to((c32 * jax.nn.sigmoid(c32)).astype(bf16), (8, D))
                for lc in range(NL):
                    R.dp(1, lc)
                    ls = pl.ds(lc * 128, 128)
                    mv[32:40, ls] = jnp.dot(sc8, wm_v[MPOS['gb'], :, ls], preferred_element_type=f32)
            R.g_(x, 2)
            R.inv()
        with scope("f_f"):
            wait_group(13)
            if CFG['gbpos'] == 0:
                mv[32:40, :] = modvec(MPOS['gb'])
            R.ln(2, CFG['fent'])
            R.tail(x, 0, 2, 3, False, CFG['fhpos'], CFG['fscall'])
            ocopy(0).start(); ocopy(1).start()

    def steady():
        R = Reg()
        s = pid + 1
        with scope("s_w"):
            for name in [('q', s + 1)] + _kvs(s + 2):
                copy(name, G_STEADY + s - 2).wait()
        with scope("s"):
            xv = unpack(hn_v[0, 0:HT, :])
            x = lambda: xv
            if CFG['premac']:
                R.sconv(s + 2, CFG['sc_lanes'])
                R.mac(s + 1, CFG['tree'], kvb[0, HT:HT + 8, 0:128])
                R.g_(x, 0); R.u_(x, 0); R.d_(0); R.g_(x, 1); R.u_(x, 1)
                R.inv()
                R.ln(s + 1, CFG['lnent'])
                pieces = [lambda lc=lc: R.dp(1, lc) for lc in range(NL)]
                pieces += [lambda j=j: R.gp(x, 2, j) for j in range(NQ)]
                pieces += [lambda j=j: R.up(x, 2, j) for j in range(NQ)]
                pieces += [lambda lc=lc: R.dp(2, lc, s, 1) for lc in range(NL)]
                for k, p in enumerate(pieces):
                    p()
                    if k in CFG['hp']:
                        R.fwd_h(s + 2, CFG['hp'].index(k))
                    if k in CFG['xp']:
                        R.fwd_x(s + 2, CFG['xp'].index(k))
            else:
                R.mac(s + 1, CFG['tree'])
                R.g_(x, 0); R.u_(x, 0); R.d_(0); R.g_(x, 1); R.u_(x, 1)
                R.inv()
                R.ln(s + 1, CFG['lnent'])
                for lc in range(NL):
                    R.dp(1, lc)
                R.tail(x, s, 1, s + 2, True, CFG['hpos'], True)
            ocopy(s).start()

    def last():
        R = Reg()
        s = NS - 2
        with scope("l_w"):
            wait_group(len(GROUPS) - 1)
        with scope("l"):
            xv = unpack(hn_v[0, 0:HT, :])
            x = lambda: xv
            R.mac(s + 1, (2, 5))
            R.g_(x, 0); R.u_(x, 0); R.d_(0); R.g_(x, 1); R.u_(x, 1); R.d_(1)
            R.inv()
            R.ln(s + 1)
            R.g_(x, 2); R.u_(x, 2); R.d_(2)
            R.fin(s)
            ocopy(s).start()
            x = lambda: unpack(hn_v[0, 0:HT, :])
            for c in range(NC - 1):
                R.g_(x, c); R.u_(x, c); R.d_(c)
            R.g_(x, NC - 1); R.u_(x, NC - 1)
            a, acc = R.st.pop('a'), R.st.pop('acc')
            for r0, n in CFG['lastsplit']:
                d = acc[r0:r0 + n] + jnp.dot(a[r0:r0 + n], wd_v[F - FC:F, :], preferred_element_type=f32)
                o_v[s + 1, r0:r0 + n, :] = (x1b[s + 1, r0:r0 + n, :] + mv[32:33, :] * d).astype(bf16)
                ocopy(s + 1, (r0, n)).start()
        with scope("e_w"):
            for t in range(NS - 1):
                ocopy(t).wait()
            for h in CFG['lastsplit']:
                ocopy(NS - 1, h).wait()

    only = CFG['only']
    if only is None or 0 in only:
        pl.when(pid == 0)(first)
    if only is None or 1 in only:
        pl.when(jnp.logical_and(pid >= 1, pid <= NS - 4))(steady)
    if only is None or 2 in only:
        pl.when(pid == NS - 3)(last)


@jax.jit
def pallas_adaLN_cond__ssm_conv_h3__glu_gated_reglu__prompt_kernel(A_q, A_k, A_v, A_shift_k, A_ssm_k, A_ssm_D, B_x, B_W_gate, B_W_up, B_W_down, c, w_mod):
    fwd, inv = _dft_mats()
    any_spec = pl.BlockSpec(memory_space=pl.ANY)
    vm = pltpu.VMEM
    return pl.pallas_call(
        _kernel,
        grid=(NS - 2,),
        in_specs=[any_spec] * 13,
        out_specs=any_spec,
        out_shape=jax.ShapeDtypeStruct((1, S, D), bf16),
        scratch_shapes=[
            vm((NS, T, D), bf16), vm((NS, T, D), bf16), vm((NS, T, D), bf16),
            vm((NBLK, D, NB), bf16),
            vm((D, F), bf16), vm((D, F), bf16), vm((F, D), bf16),
            vm((6, D, D), bf16),
            vm((2 * NB, NB), bf16), vm((NB, 2 * NB), bf16),
            vm((NS, T, D), bf16),
            vm((3 * NS, NG, 32, D), f32),
            vm((1, 2 * NB, D), f32),
            vm((1, T + 32, D), f32),
            vm((1, HT + 32, D), f32),
            vm((64, D), f32),
            vm((1, 2 * T, D), f32),
            vm((NS, T, D), f32),
            vm((1, HT + 32, D), f32),
            vm((1, T, D), f32),
            vm((2, T, D), f32),
            vm((2, T, D), f32),
            vm((1, T, FC), f32),
            vm((1, 2 * T, D), f32),
            vm((64, D), f32),
            vm((4, D), bf16), vm((D,), bf16), vm((1, D), bf16),
            pltpu.SemaphoreType.DMA((len(GROUPS),)), pltpu.SemaphoreType.DMA((1,)),
        ],
        compiler_params=pltpu.CompilerParams(vmem_limit_bytes=110 * 1024 * 1024,
                                             dimension_semantics=("arbitrary",)),
    )(A_q, A_k, A_v, A_shift_k.T, A_ssm_k, A_ssm_D, B_W_gate, B_W_up, B_W_down, c, w_mod,
      jnp.asarray(fwd, bf16), jnp.asarray(inv, bf16))
```

```python
import contextlib
import numpy as np
import jax
import jax.numpy as jnp
from jax import lax
from jax.experimental import pallas as pl
from jax.experimental.pallas import tpu as pltpu

S, D, F = 2048, 640, 1536
NB = 128
T = 256
NS = S // T
NBLK = S // NB
FC = 512
NC = F // FC
NQ = FC // 128
NL = D // 128
NG = NB // 8
HT = T // 2
RG = 16
EPS = 1e-5
f32 = jnp.float32
bf16 = jnp.bfloat16
i32 = jnp.int32

CFG = dict(only=None, scopes=False, tree=(1, 2, 3, 4, 5), hpos=(2, 3, 4, 5, 6), sc_lanes=2, lnent=3,
           fhpos=(3, 4, 5, 6, 7), premac=True, learly=False, ltree=(2, 5), fent=4, fscall=False, gbpos=1, fdh=(-1, 0, 1, 2, 3), fdx=(3, 4, 5, 6, 7), fdl=1, fdall=True, hp=(0, 2, 4, 6, 8), xp=(10, 12, 13, 15, 17), lastsplit=((0, 128), (128, 64), (192, 32), (224, 32)))

MPOS = {'sa': 0, 'ca': 1, 'ga': 2, 'sb': 3, 'cb': 4, 'gb': 5}


def _dft_mats():
    f = np.concatenate([np.arange(0, NB, 2), np.arange(1, NB, 2)])
    j = np.arange(NB)
    ang = 2.0 * np.pi * (((2 * f[:, None] + 1) * j[None, :]) % (4 * NB)) / (4 * NB)
    fwd = np.stack([np.cos(ang).reshape(NG, 8, NB), np.sin(ang).reshape(NG, 8, NB)], axis=1).reshape(2 * NB, NB)
    return fwd.astype(np.float32), (fwd.T / NB).astype(np.float32)


def _kvs(s):
    return [('k', s), ('v', s), ('s', 2 * s), ('s', 2 * s + 1)]


GROUPS = [
    ['sh', 'dd', 'c', 'fw', 'iv'] + _kvs(0),
    [('q', 0), ('q', 1)],
    _kvs(1),
    [('wm', 0)], [('wm', 1)], [('wm', 2)], [('wm', 4)], [('wm', 3)],
    [('wgh', 0)],
    [('wgh', 1), ('wuh', 0)],
    [('wuh', 1), ('wd', 0)],
    _kvs(2) + [('wg', 1), ('wu', 1)],
    [('wd', 1), ('wg', 2), ('wm', 5)],
    [('wu', 2), ('wd', 2), ('q', 2)] + _kvs(3),
]
G_STEADY = len(GROUPS)
for _s in range(2, NS - 2):
    GROUPS.append([('q', _s + 1)] + _kvs(_s + 2))
GROUPS.append([('q', NS - 1)])


def _kernel(q_hbm, k_hbm, v_hbm, sh_hbm, ssm_hbm, dd_hbm, wg_hbm, wu_hbm, wd_hbm, c_hbm, wm_hbm,
            fw_hbm, iv_hbm, o_hbm,
            q_v, k_v, v_v, ssm_v, wg_v, wu_v, wd_v, wm_v, fw_v, iv_v, o_v,
            uv, ap, zb, kvb, mv, yb, x1b, hn_v, hf, n1, n2, ab, accb, tp, sh_v, dd_v, c_v,
            sems, osem):
    pid = pl.program_id(0)

    def blk(j, n):
        return pl.ds(j * n, n) if isinstance(j, int) else pl.ds(pl.multiple_of(j * n, n), n)

    small = {'sh': (sh_hbm, sh_v), 'dd': (dd_hbm, dd_v), 'c': (c_hbm, c_v), 'fw': (fw_hbm, fw_v),
             'iv': (iv_hbm, iv_v)}

    def copy(name, gi):
        sem = sems.at[gi]
        if isinstance(name, str):
            return pltpu.make_async_copy(small[name][0], small[name][1], sem)
        kind, j = name
        if kind in ('q', 'k', 'v'):
            src, dst = {'q': (q_hbm, q_v), 'k': (k_hbm, k_v), 'v': (v_hbm, v_v)}[kind]
            return pltpu.make_async_copy(src.at[0, blk(j, T), :], dst.at[j], sem)
        if kind == 's':
            return pltpu.make_async_copy(ssm_hbm.at[:, blk(j, NB)], ssm_v.at[j], sem)
        if kind == 'wm':
            return pltpu.make_async_copy(wm_hbm.at[:, blk(j, D)], wm_v.at[j], sem)
        if kind == 'wd':
            return pltpu.make_async_copy(wd_hbm.at[blk(j, FC), :], wd_v.at[blk(j, FC), :], sem)
        src, dst = (wg_hbm, wg_v) if kind[1] == 'g' else (wu_hbm, wu_v)
        cols = blk(j, FC // 2) if kind.endswith('h') else blk(j, FC)
        return pltpu.make_async_copy(src.at[:, cols], dst.at[:, cols], sem)

    def wait_group(gi):
        for name in GROUPS[gi]:
            copy(name, gi).wait()

    def ocopy(j, h=None):
        if h is None:
            return pltpu.make_async_copy(o_v.at[j], o_hbm.at[0, blk(j, T), :], osem.at[0])
        r0, n = h
        return pltpu.make_async_copy(o_v.at[j, pl.ds(r0, n), :], o_hbm.at[0, pl.ds(j * T + r0, n), :], osem.at[0])

    def scope(name):
        return jax.named_scope(name) if CFG['scopes'] else contextlib.nullcontext()

    def pack(x):
        return pltpu.bitcast(x.astype(bf16), f32)

    def unpack(x):
        return pltpu.bitcast(x, bf16)

    def rowsum(x, tok=None):
        ps = x[:, 0:128]
        if tok is not None:
            ps = ps + jnp.concatenate([tok] * (x.shape[0] // 8), axis=0)
        for lc in range(1, NL):
            ps = ps + x[:, lc * 128:(lc + 1) * 128]
        return jnp.sum(ps, axis=-1, keepdims=True)

    def normalise(x, tok=None, ent=4):
        xc = x - rowsum(x, tok if ent == 3 else None) * (1.0 / D)
        var = rowsum(xc * xc, tok if ent == 4 else None) * (1.0 / D) + EPS
        return xc * lax.rsqrt(var)

    def fold(a, p):
        parts = []
        for g in range(NG):
            ar, ai = a[16 * g:16 * g + 8], a[16 * g + 8:16 * g + 16]
            pr, pi = p[16 * g:16 * g + 8], p[16 * g + 8:16 * g + 16]
            parts += [ar + pi, ai - pr] if g < NG // 2 else [ar - pi, ai + pr]
        return jnp.concatenate(parts, axis=0)

    def grp(x):
        return x.reshape(NG, 16, 128)

    row = lax.broadcasted_iota(i32, (8, 128), 0)

    def conv_rows(s, ls, emit, tok_in=None):
        w = [tp[8 * j:8 * j + 8, ls] for j in range(4)]
        if isinstance(s, int) and s == 0:
            pk = jnp.zeros((8, 128), f32)
            pt = jnp.zeros((8, 128), f32)
        else:
            kp = k_v[s - 1, T - 16:T, ls].astype(f32)[8:16]
            pk = pltpu.roll(kp, 1, 0)
            pt = pltpu.roll(w[2] * kp + w[3] * pk, 2, 0)
        for rg in range(T // 16):
            kk = k_v[s, rg * 16:rg * 16 + 16, ls].astype(f32)
            vv = v_v[s, rg * 16:rg * 16 + 16, ls].astype(f32)
            outs = []
            for h in range(2):
                kc = kk[8 * h:8 * h + 8]
                if h == 0 and tok_in is not None and tok_in() is not None:
                    kc = kc + tok_in()
                rk = pltpu.roll(kc, 1, 0)
                sk = jnp.where(row < 1, pk, rk)
                t = w[2] * kc + w[3] * sk
                rt = pltpu.roll(t, 2, 0)
                outs.append(((w[0] * kc + w[1] * sk) + jnp.where(row < 2, pt, rt)) * vv[8 * h:8 * h + 8])
                pk, pt = rk, rt
            emit(rg, pack(jnp.concatenate(outs, axis=0)))

    def dft_x(kv0, kv1, split=False):
        w = unpack(jnp.concatenate([kv0, kv1], axis=1))
        if split:
            xx = jnp.concatenate([jnp.dot(fw_v[h * NB:(h + 1) * NB, :], w, preferred_element_type=f32)
                                  for h in range(2)], axis=0)
        else:
            xx = jnp.dot(fw_v[...], w, preferred_element_type=f32)
        return xx[:, 0:128], xx[:, 128:256]

    def dft_h(s, rows):
        w = jnp.concatenate([ssm_v[2 * s, rows, :], ssm_v[2 * s + 1, rows, :]], axis=0)
        aa = lax.dot_general(fw_v[...], w, (((1,), (1,)), ((), ())), preferred_element_type=f32)
        return aa[:, 0:128], aa[:, 128:256]

    class Reg:
        def __init__(self):
            self.z0 = lax.shift_right_logical(pid, 8)
            self.st = {}

        def sconv(self, s, lanes, lcs=None):
            if lcs is None or lcs[0] == 0:
                self.sc = [None] * lanes
                self.gi = 0
            for lc in (range(NL) if lcs is None else lcs):
                ls = pl.ds(lc * 128, 128)

                def emit(rg, kvp, ls=ls):
                    kvb.at[self.z0][rg * 8:rg * 8 + 8, ls] = kvp
                    self.sc[self.gi % lanes] = kvb[0, HT:HT + 8, ls]
                    self.gi += 1
                conv_rows(s, ls, emit, lambda: self.sc[self.gi % lanes])

        def fwd_x(self, s, lc):
            o = self.z0 + 3 * s
            ls = pl.ds(lc * 128, 128)
            x0, x1 = dft_x(kvb[0, 0:64, ls], kvb[0, 64:128, ls])
            p = 3 * (s - 1)
            u1 = (uv[p + 2, :, 16:32, ls] + uv[p, :, 16:32, ls]) - grp(x0)
            uv[o, :, 16:32, ls] = grp(x0)
            uv[o + 1, :, 16:32, ls] = u1
            uv[o + 2, :, 16:32, ls] = grp(x1 - x0)

        def fwd_h(self, s, lc):
            o = self.z0 + 3 * s
            ls = pl.ds(lc * 128, 128)
            a0, a1 = dft_h(s, ls)
            h0 = fold(a0, ap[0, :, ls])
            h1 = fold(a1, a0)
            uv[o, :, 0:16, ls] = grp(h0 + h1)
            uv[o + 1, :, 0:16, ls] = grp(h1)
            uv[o + 2, :, 0:16, ls] = grp(h0)
            ap[self.z0, :, ls] = a1

        def mac(self, s, tree=(), tok0=None):
            static = isinstance(s, int)
            ng = s + 1 if static else NS - 1
            ub = [3 * (s - g) if static else 3 * jnp.maximum(s - g, 0) for g in range(ng)]
            toks = (tok0, tok0)
            for fc in range(NG):
                for lc in range(NL):
                    ls = pl.ds(lc * 128, 128)

                    def chain(j, ar, ai):
                        for g in range(ng):
                            hr = uv[3 * g + j, fc, 0:8, ls]
                            hi = uv[3 * g + j, fc, 8:16, ls]
                            xr = uv[ub[g] + j, fc, 16:24, ls]
                            xi = uv[ub[g] + j, fc, 24:32, ls]
                            if ar is not None and g in tree:
                                ar = ar + (hr * xr - hi * xi)
                                ai = ai + (hr * xi + hi * xr)
                            else:
                                ar = (hr * xr if ar is None else ar + hr * xr) - hi * xi
                                ai = (hr * xi if ai is None else ai + hr * xi) + hi * xr
                        return ar, ai

                    a1 = chain(0, *toks)
                    z0 = chain(1, *a1)
                    zero = pltpu.bitcast(zb[0, T:T + 8, ls], i32)

                    def tk(v):
                        return pltpu.bitcast(pltpu.bitcast(v, i32) & zero, f32)
                    z1 = chain(2, a1[0] + tk(z0[0]), a1[1] + tk(z0[1]))
                    for b, z in enumerate((z0, z1)):
                        zb.at[self.z0][b * HT + fc * 8:b * HT + fc * 8 + 8, ls] = pack(jnp.concatenate(z, axis=0))
                    toks = (tk(z1[0]), tk(z1[1]))

        def inv(self):
            for b in range(2):
                yb[self.z0, b * NB:(b + 1) * NB, :] = jnp.dot(
                    iv_v[...], unpack(zb[0, b * HT:(b + 1) * HT, :]), preferred_element_type=f32)

        def ln(self, s, ent=4):
            a1 = mv[0:1, :]; a0 = mv[8:9, :]; b1 = mv[16:17, :]; b0 = mv[24:25, :]
            tok = None
            for g in range(T // RG):
                gr = slice(g * RG, (g + 1) * RG)
                x = q_v[s, gr, :].astype(f32)
                x1 = x + (normalise(x) * a1 + a0) * yb[0, gr, :]
                x1b[self.z0 + s, gr, :] = x1
                h2 = normalise(x1, tok, ent) * b1 + b0
                hn_v.at[self.z0][g * (RG // 2):(g + 1) * (RG // 2), :] = pack(h2)
                tok = hn_v[0, HT:HT + 8, 0:128]

        def gcols(self, x, c0, n):
            return jnp.dot(x(), wg_v[:, c0:c0 + n], preferred_element_type=f32)

        def ucols(self, x, c0, n):
            return jnp.dot(x(), wu_v[:, c0:c0 + n], preferred_element_type=f32)

        def g_(self, x, c):
            self.st['g'] = self.gcols(x, c * FC, FC)

        def u_(self, x, c):
            self.st['a'] = (jnp.maximum(self.st.pop('g'), 0.0) * self.ucols(x, c * FC, FC)).astype(bf16)

        def d_(self, c):
            d = jnp.dot(self.st.pop('a'), wd_v[c * FC:(c + 1) * FC, :], preferred_element_type=f32)
            self.st['acc'] = d if c == 0 else self.st['acc'] + d

        def gp(self, x, c, j):
            self.st[('g', j)] = self.gcols(x, c * FC + j * 128, 128)

        def up(self, x, c, j):
            g = self.st.pop(('g', j)) if ('g', j) in self.st else self.st['g'][:, j * 128:(j + 1) * 128]
            self.st[('a', j)] = jnp.maximum(g, 0.0) * self.ucols(x, c * FC + j * 128, 128)
            if j == NQ - 1:
                self.st['a'] = jnp.concatenate([self.st.pop(('a', i)) for i in range(NQ)], axis=1).astype(bf16)

        def dp(self, c, lc, s=None, n=None):
            ls = pl.ds(lc * 128, 128)
            d = jnp.dot(self.st['a'], wd_v[c * FC:(c + 1) * FC, ls], preferred_element_type=f32)
            d = self.st['acc'][:, lc * 128:(lc + 1) * 128] + d
            if c == NC - 1:
                for j in range(n):
                    o_v[s + j, :, ls] = (x1b[s + j, :, ls] + mv[32:33, ls] * d[j * T:(j + 1) * T]).astype(bf16)
            else:
                self.st[('d', lc)] = d
                if lc == NL - 1:
                    self.st['acc'] = jnp.concatenate([self.st.pop(('d', i)) for i in range(NL)], axis=1)

        def tail(self, x, s, n, fs, with_g, hpos, scall):
            c = NC - 1
            k = 0
            hq = 0
            pieces = ([lambda j=j: self.gp(x, c, j) for j in range(NQ)] if with_g else [])
            pieces += [lambda j=j: self.up(x, c, j) for j in range(NQ)]
            for p in pieces:
                p()
                while hq < NL and hpos[hq] == k:
                    self.fwd_h(fs, hq); hq += 1
                k += 1
            for lc in range(NL):
                self.dp(c, lc, s, n)
                while hq < NL and hpos[hq] == k:
                    self.fwd_h(fs, hq); hq += 1
                k += 1
                if not scall:
                    self.sconv(fs, CFG['sc_lanes'], [lc])
                elif lc == 0:
                    self.sconv(fs, CFG['sc_lanes'])
                self.fwd_x(fs, lc)

        def fin(self, s):
            o_v[s] = (x1b[s] + mv[32:33, :] * self.st.pop('acc')).astype(bf16)

    def modvec(p):
        c32 = c_v[...].astype(f32)
        sc8 = jnp.broadcast_to((c32 * jax.nn.sigmoid(c32)).astype(bf16), (8, D))
        return jnp.dot(sc8, wm_v[p], preferred_element_type=f32)

    def first():
        R = Reg()
        for gi, names in enumerate(GROUPS):
            for name in names:
                copy(name, gi).start()
        z = jnp.zeros((8, D), f32)
        kvb[0, HT:HT + 8, :] = z
        hn_v[0, HT:HT + 8, :] = z
        zb[0, T:T + 8, :] = z

        def zero_v(j, _):
            uv[j, :, 0:16, :] = jnp.zeros((NG, 16, D), f32)
            return 0
        lax.fori_loop(12, 3 * (NS - 1), zero_v, 0)

        def cmul(h, x):
            return (h[:, 0:8] * x[:, 0:8] - h[:, 8:16] * x[:, 8:16], h[:, 0:8] * x[:, 8:16] + h[:, 8:16] * x[:, 0:8])

        def conv_pair(s):
            def body(lc, _):
                ls = blk(lc, 128)
                if s == 1:
                    for k in range(7):
                        g = jnp.minimum(lc * 7 + k, 2 * T // RG - 1)
                        gr = blk(g % (T // RG), RG)
                        n1[g // (T // RG), gr, :] = normalise(q_v[g // (T // RG), gr, :].astype(f32))
                rows = []
                conv_rows(s, ls, lambda rg, kvp: rows.append(kvp))
                a0, a1 = dft_h(s, ls)
                x0, x1 = dft_x(jnp.concatenate(rows[0:8], axis=0), jnp.concatenate(rows[8:16], axis=0), True)
                if s == 0:
                    dd = tp[32:40, ls]
                    h0 = jnp.concatenate([a0[8 * g:8 * g + 8] + dd if g % 2 == 0 else a0[8 * g:8 * g + 8]
                                          for g in range(2 * NG)], axis=0)
                    u1 = grp(-x0)
                else:
                    h0 = fold(a0, ap[0, :, ls])
                    u1 = (uv[2, :, 16:32, ls] + uv[0, :, 16:32, ls]) - grp(x0)
                h1 = fold(a1, a0)
                us = [grp(x0), u1, grp(x1 - x0)]
                vs = [grp(h0 + h1), grp(h1), grp(h0)]
                if s == 0:
                    p = [cmul(vs[j], us[j]) for j in range(3)]
                else:
                    p = []
                    for j in range(3):
                        t0 = cmul(uv[j, :, 0:16, ls], us[j])
                        t1 = cmul(vs[j], uv[j, :, 16:32, ls])
                        p.append((t0[0] + t1[0], t0[1] + t1[1]))
                for j in range(3):
                    uv[3 * s + j, :, 16:32, ls] = us[j]
                    uv[3 * s + j, :, 0:16, ls] = vs[j]
                ap[0, :, ls] = a1
                for b in range(2):
                    zz = jnp.concatenate([p[0][0] + p[1 + b][0], p[0][1] + p[1 + b][1]], axis=1)
                    n2[s, b * HT:(b + 1) * HT, ls] = pack(zz.reshape(2 * NB, 128))
                return 0
            lax.fori_loop(0, NL, body, 0)

        with scope("p_w0"):
            wait_group(0)
        with scope("p_c0"):
            taps = sh_v[...].astype(f32)
            for j in range(4):
                tp[8 * j:8 * j + 8, :] = jnp.broadcast_to(taps[j:j + 1, :], (8, D))
            tp[32:40, :] = jnp.broadcast_to(dd_v[...].astype(f32).reshape(1, D), (8, D))
            conv_pair(0)
        with scope("p_c1"):
            wait_group(1)
            wait_group(2)
            conv_pair(1)

            def inv01(i, _):
                for b in range(2):
                    yb[0, pl.ds(pl.multiple_of(i * T + b * NB, NB), NB), :] = jnp.dot(
                        iv_v[...], unpack(n2[i, b * HT:(b + 1) * HT, :]), preferred_element_type=f32)
                return 0
            lax.fori_loop(0, 2, inv01, 0)
        with scope("p_mod"):
            for gi in (3, 4, 5):
                wait_group(gi)
            sa, ca, ga = modvec(0), modvec(1), modvec(2)
            mv[0:8, :] = ga * (1.0 + ca)
            mv[8:16, :] = ga * sa
        with scope("p_ln2"):
            def ln2(i, _):
                for g in range(T // RG):
                    gr = slice(g * RG, (g + 1) * RG)
                    x = q_v[i, gr, :].astype(f32)
                    y = yb[0, pl.ds(pl.multiple_of(i * T + g * RG, RG), RG), :]
                    x1 = x + (n1[i, gr, :] * mv[0:1, :] + mv[8:9, :]) * y
                    x1b[i, gr, :] = x1
                    n2[i, gr, :] = normalise(x1)
                return 0
            lax.fori_loop(0, 2, ln2, 0)
        with scope("p_mod2"):
            def mod2(i, _):
                copy(('wm', 4 - i), 6 + i).wait()
                mv[blk(2 + i, 8), :] = modvec(4 - i) + (1 - i).astype(f32)
                return 0
            lax.fori_loop(0, 2, mod2, 0)
            for s in range(2):
                hf.at[R.z0][s * HT:(s + 1) * HT, :] = pack(n2[s] * mv[16:17, :] + mv[24:25, :])
        x = lambda: unpack(hf[0])
        xh = [lambda h=h: unpack(hf[0, h * HT:(h + 1) * HT, :]) for h in range(2)]
        HC = FC // 2
        gbuf = accb.at[R.z0]
        with scope("f_a"):
            wait_group(8)
            for h in range(2):
                gbuf[h * T:(h + 1) * T, 0:HC] = R.gcols(xh[h], 0, HC)
        with scope("f_b"):
            wait_group(9)
            ab.at[R.z0][:, 0:HC] = pack(jnp.maximum(accb[0, :, 0:HC], 0.0) * R.ucols(x, 0, HC))
            gbuf[:, HC:FC] = R.gcols(x, HC, HC)
        with scope("f_c"):
            wait_group(10)
            a2 = (jnp.maximum(accb[0, :, HC:FC], 0.0) * R.ucols(x, HC, HC)).astype(bf16)
            da = jnp.dot(unpack(ab[0, :, 0:HC]), wd_v[0:HC, :], preferred_element_type=f32)
            for h in range(2):
                gbuf[h * T:(h + 1) * T, :] = da[h * T:(h + 1) * T] + jnp.dot(
                    a2[h * T:(h + 1) * T], wd_v[HC:FC, :], preferred_element_type=f32)
        with scope("f_d"):
            wait_group(11)
            pieces = [lambda: None] + [lambda j=j: R.gp(x, 1, j) for j in range(NQ)]
            pieces += [lambda j=j: R.up(x, 1, j) for j in range(NQ)]
            for k, p in enumerate(pieces):
                p()
                for lc in range(NL):
                    if CFG['fdh'][lc] == k - 1:
                        R.fwd_h(2, lc)
                for lc in range(NL):
                    if CFG['fdx'][lc] == k - 1:
                        if not CFG['fdall']:
                            R.sconv(2, CFG['fdl'], [lc])
                        elif lc == 0:
                            R.sconv(2, CFG['fdl'])
                        R.fwd_x(2, lc)
            ab[R.z0] = pltpu.bitcast(R.st.pop('a'), f32)
        with scope("f_e"):
            wait_group(12)
            R.st['a'] = unpack(ab[0])
            R.st['acc'] = accb[0]
            R.mac(2)
            if CFG['gbpos'] == 0:
                R.d_(1)
            else:
                c32 = c_v[...].astype(f32)
                sc8 = jnp.broadcast_to((c32 * jax.nn.sigmoid(c32)).astype(bf16), (8, D))
                for lc in range(NL):
                    R.dp(1, lc)
                    ls = pl.ds(lc * 128, 128)
                    mv[32:40, ls] = jnp.dot(sc8, wm_v[MPOS['gb'], :, ls], preferred_element_type=f32)
            R.g_(x, 2)
            R.inv()
        with scope("f_f"):
            wait_group(13)
            if CFG['gbpos'] == 0:
                mv[32:40, :] = modvec(MPOS['gb'])
            R.ln(2, CFG['fent'])
            R.tail(x, 0, 2, 3, False, CFG['fhpos'], CFG['fscall'])
            ocopy(0).start(); ocopy(1).start()

    def steady():
        R = Reg()
        s = pid + 1
        with scope("s_w"):
            for name in [('q', s + 1)] + _kvs(s + 2):
                copy(name, G_STEADY + s - 2).wait()
        with scope("s"):
            xv = unpack(hn_v[0, 0:HT, :])
            x = lambda: xv
            if CFG['premac']:
                R.sconv(s + 2, CFG['sc_lanes'])
                R.mac(s + 1, CFG['tree'], kvb[0, HT:HT + 8, 0:128])
                R.g_(x, 0); R.u_(x, 0); R.d_(0); R.g_(x, 1); R.u_(x, 1)
                R.inv()
                R.ln(s + 1, CFG['lnent'])
                pieces = [lambda lc=lc: R.dp(1, lc) for lc in range(NL)]
                pieces += [lambda j=j: R.gp(x, 2, j) for j in range(NQ)]
                pieces += [lambda j=j: R.up(x, 2, j) for j in range(NQ)]
                pieces += [lambda lc=lc: R.dp(2, lc, s, 1) for lc in range(NL)]
                for k, p in enumerate(pieces):
                    p()
                    if k in CFG['hp']:
                        R.fwd_h(s + 2, CFG['hp'].index(k))
                    if k in CFG['xp']:
                        R.fwd_x(s + 2, CFG['xp'].index(k))
            else:
                R.mac(s + 1, CFG['tree'])
                R.g_(x, 0); R.u_(x, 0); R.d_(0); R.g_(x, 1); R.u_(x, 1)
                R.inv()
                R.ln(s + 1, CFG['lnent'])
                for lc in range(NL):
                    R.dp(1, lc)
                R.tail(x, s, 1, s + 2, True, CFG['hpos'], True)
            ocopy(s).start()

    def last():
        R = Reg()
        s = NS - 2
        with scope("l_w"):
            wait_group(len(GROUPS) - 1)
        with scope("l"):
            xv = unpack(hn_v[0, 0:HT, :])
            x = lambda: xv
            R.mac(s + 1, CFG['ltree'])
            R.g_(x, 0); R.u_(x, 0); R.d_(0); R.g_(x, 1); R.u_(x, 1)
            if CFG['learly']:
                R.inv()
                R.ln(s + 1, 3)
                for lc in range(NL):
                    R.dp(1, lc)
            else:
                R.d_(1)
                R.inv()
                R.ln(s + 1)
            R.g_(x, 2); R.u_(x, 2); R.d_(2)
            R.fin(s)
            ocopy(s).start()
            x = lambda: unpack(hn_v[0, 0:HT, :])
            for c in range(NC - 1):
                R.g_(x, c); R.u_(x, c); R.d_(c)
            R.g_(x, NC - 1); R.u_(x, NC - 1)
            a, acc = R.st.pop('a'), R.st.pop('acc')
            for r0, n in CFG['lastsplit']:
                d = acc[r0:r0 + n] + jnp.dot(a[r0:r0 + n], wd_v[F - FC:F, :], preferred_element_type=f32)
                o_v[s + 1, r0:r0 + n, :] = (x1b[s + 1, r0:r0 + n, :] + mv[32:33, :] * d).astype(bf16)
                ocopy(s + 1, (r0, n)).start()
        with scope("e_w"):
            for t in range(NS - 1):
                ocopy(t).wait()
            for h in CFG['lastsplit']:
                ocopy(NS - 1, h).wait()

    only = CFG['only']
    if only is None or 0 in only:
        pl.when(pid == 0)(first)
    if only is None or 1 in only:
        pl.when(jnp.logical_and(pid >= 1, pid <= NS - 4))(steady)
    if only is None or 2 in only:
        pl.when(pid == NS - 3)(last)


@jax.jit
def pallas_adaLN_cond__ssm_conv_h3__glu_gated_reglu__prompt_kernel(A_q, A_k, A_v, A_shift_k, A_ssm_k, A_ssm_D, B_x, B_W_gate, B_W_up, B_W_down, c, w_mod):
    fwd, inv = _dft_mats()
    any_spec = pl.BlockSpec(memory_space=pl.ANY)
    vm = pltpu.VMEM
    return pl.pallas_call(
        _kernel,
        grid=(NS - 2,),
        in_specs=[any_spec] * 13,
        out_specs=any_spec,
        out_shape=jax.ShapeDtypeStruct((1, S, D), bf16),
        scratch_shapes=[
            vm((NS, T, D), bf16), vm((NS, T, D), bf16), vm((NS, T, D), bf16),
            vm((NBLK, D, NB), bf16),
            vm((D, F), bf16), vm((D, F), bf16), vm((F, D), bf16),
            vm((6, D, D), bf16),
            vm((2 * NB, NB), bf16), vm((NB, 2 * NB), bf16),
            vm((NS, T, D), bf16),
            vm((3 * NS, NG, 32, D), f32),
            vm((1, 2 * NB, D), f32),
            vm((1, T + 32, D), f32),
            vm((1, HT + 32, D), f32),
            vm((64, D), f32),
            vm((1, 2 * T, D), f32),
            vm((NS, T, D), f32),
            vm((1, HT + 32, D), f32),
            vm((1, T, D), f32),
            vm((2, T, D), f32),
            vm((2, T, D), f32),
            vm((1, T, FC), f32),
            vm((1, 2 * T, D), f32),
            vm((64, D), f32),
            vm((4, D), bf16), vm((D,), bf16), vm((1, D), bf16),
            pltpu.SemaphoreType.DMA((len(GROUPS),)), pltpu.SemaphoreType.DMA((1,)),
        ],
        compiler_params=pltpu.CompilerParams(vmem_limit_bytes=110 * 1024 * 1024,
                                             dimension_semantics=("arbitrary",)),
    )(A_q, A_k, A_v, A_shift_k.T, A_ssm_k, A_ssm_D, B_W_gate, B_W_up, B_W_down, c, w_mod,
      jnp.asarray(fwd, bf16), jnp.asarray(inv, bf16))
```

```python
import contextlib
import numpy as np
import jax
import jax.numpy as jnp
from jax import lax
from jax.experimental import pallas as pl
from jax.experimental.pallas import tpu as pltpu

S, D, F = 2048, 640, 1536
NB = 128
T = 256
NS = S // T
NBLK = S // NB
FC = 512
NC = F // FC
NQ = FC // 128
NL = D // 128
NG = NB // 8
HT = T // 2
RG = 16
EPS = 1e-5
f32 = jnp.float32
bf16 = jnp.bfloat16
i32 = jnp.int32

CFG = dict(only=None, scopes=False, tree=(1, 2, 3, 4, 5), hpos=(2, 3, 4, 5, 6), sc_lanes=2, lnent=3,
           fhpos=(3, 4, 5, 6, 7), premac=True, learly=False, ltree=(2, 5), fent=4, fscall=False, gbpos=1, fch=4, split=True, gbp=(0, 1, 2, 3, 4), fdx=(3, 4, 5, 6, 7), fford=0, fhp=(7, 9, 11, 13, 15), fxp=(10, 12, 14, 16, 17), ffl=2, fdl=2, hp=(0, 2, 4, 6, 8), xp=(10, 12, 13, 15, 17), lastsplit=((0, 128), (128, 64), (192, 32), (224, 32)))

MPOS = {'sa': 0, 'ca': 1, 'ga': 2, 'sb': 3, 'cb': 4, 'gb': 5}


def _dft_mats():
    f = np.concatenate([np.arange(0, NB, 2), np.arange(1, NB, 2)])
    j = np.arange(NB)
    ang = 2.0 * np.pi * (((2 * f[:, None] + 1) * j[None, :]) % (4 * NB)) / (4 * NB)
    fwd = np.stack([np.cos(ang).reshape(NG, 8, NB), np.sin(ang).reshape(NG, 8, NB)], axis=1).reshape(2 * NB, NB)
    return fwd.astype(np.float32), (fwd.T / NB).astype(np.float32)


def _kvs(s):
    return [('k', s), ('v', s), ('s', 2 * s), ('s', 2 * s + 1)]


GROUPS = [
    ['sh', 'dd', 'c', 'fw', 'iv'] + _kvs(0),
    [('q', 0), ('q', 1)],
    _kvs(1),
    [('wm', 0), ('wm', 1)],
    [('wm', 2)],
    [('cb', 0), ('sb', 0)],
]
G_K = len(GROUPS)
for _k in range(NL):
    GROUPS.append(([('cb', _k + 1), ('sb', _k + 1)] if _k + 1 < NL else []) + [('wgk', _k), ('wuk', _k)])
G_F = len(GROUPS)
GROUPS += [
    [('s', 4), ('s', 5), ('wd', 0)],
    [('k', 2), ('v', 2), ('wg', 1)],
    [('wu', 1), ('wd', 1), ('wg', 2)],
    [('wu', 2), ('wd', 2), ('wm', 5), ('q', 2)] + _kvs(3),
]
G_STEADY = len(GROUPS)
for _s in range(2, NS - 2):
    GROUPS.append([('q', _s + 1)] + _kvs(_s + 2))
GROUPS.append([('q', NS - 1)])


def _kernel(q_hbm, k_hbm, v_hbm, sh_hbm, ssm_hbm, dd_hbm, wg_hbm, wu_hbm, wd_hbm, c_hbm, wm_hbm,
            fw_hbm, iv_hbm, o_hbm,
            q_v, k_v, v_v, ssm_v, wg_v, wu_v, wd_v, wm_v, fw_v, iv_v, o_v,
            uv, ap, zb, kvb, mv, yb, x1b, hn_v, hf, n1, n2, gu, accb, tp, sh_v, dd_v, c_v,
            sems, osem):
    pid = pl.program_id(0)

    def blk(j, n):
        return pl.ds(j * n, n) if isinstance(j, int) else pl.ds(pl.multiple_of(j * n, n), n)

    small = {'sh': (sh_hbm, sh_v), 'dd': (dd_hbm, dd_v), 'c': (c_hbm, c_v), 'fw': (fw_hbm, fw_v),
             'iv': (iv_hbm, iv_v)}

    def copy(name, gi):
        sem = sems.at[gi]
        if isinstance(name, str):
            return pltpu.make_async_copy(small[name][0], small[name][1], sem)
        kind, j = name
        if kind in ('q', 'k', 'v'):
            src, dst = {'q': (q_hbm, q_v), 'k': (k_hbm, k_v), 'v': (v_hbm, v_v)}[kind]
            return pltpu.make_async_copy(src.at[0, blk(j, T), :], dst.at[j], sem)
        if kind == 's':
            return pltpu.make_async_copy(ssm_hbm.at[:, blk(j, NB)], ssm_v.at[j], sem)
        if kind == 'wm':
            return pltpu.make_async_copy(wm_hbm.at[:, blk(j, D)], wm_v.at[j], sem)
        if kind in ('cb', 'sb'):
            p = MPOS[kind]
            c0 = p * D + j * 128 if isinstance(j, int) else pl.multiple_of(p * D + j * 128, 128)
            return pltpu.make_async_copy(wm_hbm.at[:, pl.ds(c0, 128)], wm_v.at[p, :, blk(j, 128)], sem)
        if kind in ('wgk', 'wuk'):
            src, dst = (wg_hbm, wg_v) if kind == 'wgk' else (wu_hbm, wu_v)
            return pltpu.make_async_copy(src.at[blk(j, 128), 0:FC], dst.at[blk(j, 128), 0:FC], sem)
        if kind == 'wd':
            return pltpu.make_async_copy(wd_hbm.at[blk(j, FC), :], wd_v.at[blk(j, FC), :], sem)
        src, dst = (wg_hbm, wg_v) if kind[1] == 'g' else (wu_hbm, wu_v)
        return pltpu.make_async_copy(src.at[:, blk(j, FC)], dst.at[:, blk(j, FC)], sem)

    def wait_group(gi):
        for name in GROUPS[gi]:
            copy(name, gi).wait()

    def ocopy(j, h=None):
        if h is None:
            return pltpu.make_async_copy(o_v.at[j], o_hbm.at[0, blk(j, T), :], osem.at[0])
        r0, n = h
        return pltpu.make_async_copy(o_v.at[j, pl.ds(r0, n), :], o_hbm.at[0, pl.ds(j * T + r0, n), :], osem.at[0])

    def scope(name):
        return jax.named_scope(name) if CFG['scopes'] else contextlib.nullcontext()

    def pack(x):
        return pltpu.bitcast(x.astype(bf16), f32)

    def unpack(x):
        return pltpu.bitcast(x, bf16)

    def rowsum(x, tok=None):
        ps = x[:, 0:128]
        if tok is not None:
            ps = ps + jnp.concatenate([tok] * (x.shape[0] // 8), axis=0)
        for lc in range(1, NL):
            ps = ps + x[:, lc * 128:(lc + 1) * 128]
        return jnp.sum(ps, axis=-1, keepdims=True)

    def normalise(x, tok=None, ent=4):
        xc = x - rowsum(x, tok if ent == 3 else None) * (1.0 / D)
        var = rowsum(xc * xc, tok if ent == 4 else None) * (1.0 / D) + EPS
        return xc * lax.rsqrt(var)

    def fold(a, p):
        parts = []
        for g in range(NG):
            ar, ai = a[16 * g:16 * g + 8], a[16 * g + 8:16 * g + 16]
            pr, pi = p[16 * g:16 * g + 8], p[16 * g + 8:16 * g + 16]
            parts += [ar + pi, ai - pr] if g < NG // 2 else [ar - pi, ai + pr]
        return jnp.concatenate(parts, axis=0)

    def grp(x):
        return x.reshape(NG, 16, 128)

    row = lax.broadcasted_iota(i32, (8, 128), 0)

    def conv_rows(s, ls, emit, tok_in=None):
        w = [tp[8 * j:8 * j + 8, ls] for j in range(4)]
        if isinstance(s, int) and s == 0:
            pk = jnp.zeros((8, 128), f32)
            pt = jnp.zeros((8, 128), f32)
        else:
            kp = k_v[s - 1, T - 16:T, ls].astype(f32)[8:16]
            pk = pltpu.roll(kp, 1, 0)
            pt = pltpu.roll(w[2] * kp + w[3] * pk, 2, 0)
        for rg in range(T // 16):
            kk = k_v[s, rg * 16:rg * 16 + 16, ls].astype(f32)
            vv = v_v[s, rg * 16:rg * 16 + 16, ls].astype(f32)
            outs = []
            for h in range(2):
                kc = kk[8 * h:8 * h + 8]
                if h == 0 and tok_in is not None and tok_in() is not None:
                    kc = kc + tok_in()
                rk = pltpu.roll(kc, 1, 0)
                sk = jnp.where(row < 1, pk, rk)
                t = w[2] * kc + w[3] * sk
                rt = pltpu.roll(t, 2, 0)
                outs.append(((w[0] * kc + w[1] * sk) + jnp.where(row < 2, pt, rt)) * vv[8 * h:8 * h + 8])
                pk, pt = rk, rt
            emit(rg, pack(jnp.concatenate(outs, axis=0)))

    def dft_x(kv0, kv1, split=False):
        w = unpack(jnp.concatenate([kv0, kv1], axis=1))
        if split:
            xx = jnp.concatenate([jnp.dot(fw_v[h * NB:(h + 1) * NB, :], w, preferred_element_type=f32)
                                  for h in range(2)], axis=0)
        else:
            xx = jnp.dot(fw_v[...], w, preferred_element_type=f32)
        return xx[:, 0:128], xx[:, 128:256]

    def dft_h(s, rows):
        w = jnp.concatenate([ssm_v[2 * s, rows, :], ssm_v[2 * s + 1, rows, :]], axis=0)
        aa = lax.dot_general(fw_v[...], w, (((1,), (1,)), ((), ())), preferred_element_type=f32)
        return aa[:, 0:128], aa[:, 128:256]

    def silu_c():
        return unpack(tp[40:48, :])

    def modvec(p):
        return jnp.dot(silu_c(), wm_v[p], preferred_element_type=f32)[0:8]

    def mm(lhs, w):
        if lhs.shape[0] <= T or not CFG['split']:
            return jnp.dot(lhs, w(), preferred_element_type=f32)
        return jnp.concatenate([jnp.dot(lhs[r:r + T], w(), preferred_element_type=f32)
                                for r in range(0, lhs.shape[0], T)], axis=0)

    class Reg:
        def __init__(self):
            self.z0 = lax.shift_right_logical(pid, 8)
            self.st = {}

        def sconv(self, s, lanes, lcs=None):
            if lcs is None or lcs[0] == 0:
                self.sc = [None] * lanes
                self.gi = 0
            for lc in (range(NL) if lcs is None else lcs):
                ls = pl.ds(lc * 128, 128)

                def emit(rg, kvp, ls=ls):
                    kvb.at[self.z0][rg * 8:rg * 8 + 8, ls] = kvp
                    self.sc[self.gi % lanes] = kvb[0, HT:HT + 8, ls]
                    self.gi += 1
                conv_rows(s, ls, emit, lambda: self.sc[self.gi % lanes])

        def fwd_x(self, s, lc):
            o = self.z0 + 3 * s
            ls = pl.ds(lc * 128, 128)
            x0, x1 = dft_x(kvb[0, 0:64, ls], kvb[0, 64:128, ls])
            p = 3 * (s - 1)
            u1 = (uv[p + 2, :, 16:32, ls] + uv[p, :, 16:32, ls]) - grp(x0)
            uv[o, :, 16:32, ls] = grp(x0)
            uv[o + 1, :, 16:32, ls] = u1
            uv[o + 2, :, 16:32, ls] = grp(x1 - x0)

        def fwd_h(self, s, lc):
            o = self.z0 + 3 * s
            ls = pl.ds(lc * 128, 128)
            a0, a1 = dft_h(s, ls)
            h0 = fold(a0, ap[0, :, ls])
            h1 = fold(a1, a0)
            uv[o, :, 0:16, ls] = grp(h0 + h1)
            uv[o + 1, :, 0:16, ls] = grp(h1)
            uv[o + 2, :, 0:16, ls] = grp(h0)
            ap[self.z0, :, ls] = a1

        def mac(self, s, tree=(), tok0=None):
            static = isinstance(s, int)
            ng = s + 1 if static else NS - 1
            ub = [3 * (s - g) if static else 3 * jnp.maximum(s - g, 0) for g in range(ng)]
            toks = (tok0, tok0)
            for fc in range(NG):
                for lc in range(NL):
                    ls = pl.ds(lc * 128, 128)

                    def chain(j, ar, ai):
                        for g in range(ng):
                            hr = uv[3 * g + j, fc, 0:8, ls]
                            hi = uv[3 * g + j, fc, 8:16, ls]
                            xr = uv[ub[g] + j, fc, 16:24, ls]
                            xi = uv[ub[g] + j, fc, 24:32, ls]
                            if ar is not None and g in tree:
                                ar = ar + (hr * xr - hi * xi)
                                ai = ai + (hr * xi + hi * xr)
                            else:
                                ar = (hr * xr if ar is None else ar + hr * xr) - hi * xi
                                ai = (hr * xi if ai is None else ai + hr * xi) + hi * xr
                        return ar, ai

                    a1 = chain(0, *toks)
                    z0 = chain(1, *a1)
                    zero = pltpu.bitcast(zb[0, T:T + 8, ls], i32)

                    def tk(v):
                        return pltpu.bitcast(pltpu.bitcast(v, i32) & zero, f32)
                    z1 = chain(2, a1[0] + tk(z0[0]), a1[1] + tk(z0[1]))
                    for b, z in enumerate((z0, z1)):
                        zb.at[self.z0][b * HT + fc * 8:b * HT + fc * 8 + 8, ls] = pack(jnp.concatenate(z, axis=0))
                    toks = (tk(z1[0]), tk(z1[1]))

        def inv(self):
            for b in range(2):
                yb[self.z0, b * NB:(b + 1) * NB, :] = jnp.dot(
                    iv_v[...], unpack(zb[0, b * HT:(b + 1) * HT, :]), preferred_element_type=f32)

        def ln(self, s, ent=4):
            a1 = mv[0:1, :]; a0 = mv[8:9, :]; b1 = mv[16:17, :]; b0 = mv[24:25, :]
            tok = None
            for g in range(T // RG):
                gr = slice(g * RG, (g + 1) * RG)
                x = q_v[s, gr, :].astype(f32)
                x1 = x + (normalise(x) * a1 + a0) * yb[0, gr, :]
                x1b[self.z0 + s, gr, :] = x1
                h2 = normalise(x1, tok, ent) * b1 + b0
                hn_v.at[self.z0][g * (RG // 2):(g + 1) * (RG // 2), :] = pack(h2)
                tok = hn_v[0, HT:HT + 8, 0:128]

        def gcols(self, x, c0, n):
            return mm(x(), lambda: wg_v[:, c0:c0 + n])

        def ucols(self, x, c0, n):
            return mm(x(), lambda: wu_v[:, c0:c0 + n])

        def g_(self, x, c):
            self.st['g'] = self.gcols(x, c * FC, FC)

        def u_(self, x, c):
            self.st['a'] = (jnp.maximum(self.st.pop('g'), 0.0) * self.ucols(x, c * FC, FC)).astype(bf16)

        def d_(self, c):
            d = mm(self.st.pop('a'), lambda: wd_v[c * FC:(c + 1) * FC, :])
            self.st['acc'] = d if c == 0 else self.st['acc'] + d

        def gp(self, x, c, j):
            self.st[('g', j)] = self.gcols(x, c * FC + j * 128, 128)

        def up(self, x, c, j):
            g = self.st.pop(('g', j)) if ('g', j) in self.st else self.st['g'][:, j * 128:(j + 1) * 128]
            self.st[('a', j)] = jnp.maximum(g, 0.0) * self.ucols(x, c * FC + j * 128, 128)
            if j == NQ - 1:
                self.st['a'] = jnp.concatenate([self.st.pop(('a', i)) for i in range(NQ)], axis=1).astype(bf16)

        def dp(self, c, lc, s=None, n=None):
            ls = pl.ds(lc * 128, 128)
            d = mm(self.st['a'], lambda: wd_v[c * FC:(c + 1) * FC, ls])
            d = self.st['acc'][:, lc * 128:(lc + 1) * 128] + d
            if c == NC - 1:
                for j in range(n):
                    o_v[s + j, :, ls] = (x1b[s + j, :, ls] + mv[32:33, ls] * d[j * T:(j + 1) * T]).astype(bf16)
            else:
                self.st[('d', lc)] = d
                if lc == NL - 1:
                    self.st['acc'] = jnp.concatenate([self.st.pop(('d', i)) for i in range(NL)], axis=1)

        def tail(self, x, s, n, fs, with_g, hpos, scall, gb=False):
            c = NC - 1
            k = 0
            hq = 0
            pieces = ([lambda j=j: self.gp(x, c, j) for j in range(NQ)] if with_g else [])
            pieces += [lambda j=j: self.up(x, c, j) for j in range(NQ)]
            for p in pieces:
                p()
                if gb:
                    for lc in [i for i in range(NL) if CFG['gbp'][i] == k]:
                        ls = pl.ds(lc * 128, 128)
                        mv[32:40, ls] = jnp.dot(silu_c(), wm_v[MPOS['gb'], :, ls], preferred_element_type=f32)[0:8]
                while hq < NL and hpos[hq] == k:
                    self.fwd_h(fs, hq); hq += 1
                k += 1
            for lc in range(NL):
                self.dp(c, lc, s, n)
                while hq < NL and hpos[hq] == k:
                    self.fwd_h(fs, hq); hq += 1
                k += 1
                if not scall:
                    self.sconv(fs, CFG['sc_lanes'], [lc])
                elif lc == 0:
                    self.sconv(fs, CFG['sc_lanes'])
                self.fwd_x(fs, lc)

        def fin(self, s):
            o_v[s] = (x1b[s] + mv[32:33, :] * self.st.pop('acc')).astype(bf16)


    def first():
        R = Reg()
        for gi, names in enumerate(GROUPS):
            for name in names:
                copy(name, gi).start()
        z = jnp.zeros((8, D), f32)
        kvb[0, HT:HT + 8, :] = z
        hn_v[0, HT:HT + 8, :] = z
        zb[0, T:T + 8, :] = z

        def zero_v(j, _):
            uv[j, :, 0:16, :] = jnp.zeros((NG, 16, D), f32)
            return 0
        lax.fori_loop(12, 3 * (NS - 1), zero_v, 0)

        def zero_gu(j, _):
            gu[blk(j, 64), :] = jnp.zeros((64, 2 * FC), f32)
            return 0
        lax.fori_loop(0, 2 * T // 64, zero_gu, 0)

        def cmul(h, x):
            return (h[:, 0:8] * x[:, 0:8] - h[:, 8:16] * x[:, 8:16], h[:, 0:8] * x[:, 8:16] + h[:, 8:16] * x[:, 0:8])

        def conv_pair(s):
            def body(lc, _):
                ls = blk(lc, 128)
                if s == 1:
                    for k in range(7):
                        g = jnp.minimum(lc * 7 + k, 2 * T // RG - 1)
                        gr = blk(g % (T // RG), RG)
                        n1[g // (T // RG), gr, :] = normalise(q_v[g // (T // RG), gr, :].astype(f32))
                    for b in range(2):
                        yb[0, b * NB:(b + 1) * NB, ls] = jnp.dot(
                            iv_v[...], unpack(n2[0, b * HT:(b + 1) * HT, ls]), preferred_element_type=f32)
                rows = []
                conv_rows(s, ls, lambda rg, kvp: rows.append(kvp))
                a0, a1 = dft_h(s, ls)
                x0, x1 = dft_x(jnp.concatenate(rows[0:8], axis=0), jnp.concatenate(rows[8:16], axis=0), True)
                if s == 0:
                    dd = tp[32:40, ls]
                    h0 = jnp.concatenate([a0[8 * g:8 * g + 8] + dd if g % 2 == 0 else a0[8 * g:8 * g + 8]
                                          for g in range(2 * NG)], axis=0)
                    u1 = grp(-x0)
                else:
                    h0 = fold(a0, ap[0, :, ls])
                    u1 = (uv[2, :, 16:32, ls] + uv[0, :, 16:32, ls]) - grp(x0)
                h1 = fold(a1, a0)
                us = [grp(x0), u1, grp(x1 - x0)]
                vs = [grp(h0 + h1), grp(h1), grp(h0)]
                if s == 0:
                    p = [cmul(vs[j], us[j]) for j in range(3)]
                else:
                    p = []
                    for j in range(3):
                        t0 = cmul(uv[j, :, 0:16, ls], us[j])
                        t1 = cmul(vs[j], uv[j, :, 16:32, ls])
                        p.append((t0[0] + t1[0], t0[1] + t1[1]))
                for j in range(3):
                    uv[3 * s + j, :, 16:32, ls] = us[j]
                    uv[3 * s + j, :, 0:16, ls] = vs[j]
                ap[0, :, ls] = a1
                for b in range(2):
                    zz = jnp.concatenate([p[0][0] + p[1 + b][0], p[0][1] + p[1 + b][1]], axis=1)
                    n2[s, b * HT:(b + 1) * HT, ls] = pack(zz.reshape(2 * NB, 128))
                return 0
            lax.fori_loop(0, NL, body, 0)

        with scope("p_w0"):
            wait_group(0)
        with scope("p_c0"):
            taps = sh_v[...].astype(f32)
            for j in range(4):
                tp[8 * j:8 * j + 8, :] = jnp.broadcast_to(taps[j:j + 1, :], (8, D))
            tp[32:40, :] = jnp.broadcast_to(dd_v[...].astype(f32).reshape(1, D), (8, D))
            c32 = c_v[...].astype(f32)
            tp[40:48, :] = pack(jnp.broadcast_to(c32 * jax.nn.sigmoid(c32), (16, D)))
            conv_pair(0)
        with scope("p_c1"):
            wait_group(1)
            wait_group(2)
            conv_pair(1)

            wait_group(3)
            for b in range(2):
                yb[0, T + b * NB:T + (b + 1) * NB, :] = jnp.dot(
                    iv_v[...], unpack(n2[1, b * HT:(b + 1) * HT, :]), preferred_element_type=f32)
            mv[40:48, :] = modvec(0)
            mv[48:56, :] = modvec(1)
        with scope("p_mod"):
            wait_group(4)
            ga = modvec(2)
            mv[0:8, :] = ga * (1.0 + mv[48:56, :])
            mv[8:16, :] = ga * mv[40:48, :]
        with scope("p_ln2"):
            def ln2(i, _):
                for g in range(T // RG):
                    gr = slice(g * RG, (g + 1) * RG)
                    x = q_v[i, gr, :].astype(f32)
                    y = yb[0, pl.ds(pl.multiple_of(i * T + g * RG, RG), RG), :]
                    x1 = x + (n1[i, gr, :] * mv[0:1, :] + mv[8:9, :]) * y
                    x1b[i, gr, :] = x1
                    n2[i, gr, :] = normalise(x1)
                return 0
            lax.fori_loop(0, 2, ln2, 0)

        def h2_tile(k):
            ls = blk(k, 128)
            b1 = 1.0 + jnp.dot(silu_c(), wm_v[MPOS['cb'], :, ls], preferred_element_type=f32)[0:8]
            b0 = jnp.dot(silu_c(), wm_v[MPOS['sb'], :, ls], preferred_element_type=f32)[0:8]
            mv[16:24, ls] = b1
            mv[24:32, ls] = b0
            t = jnp.concatenate([pack(n2[i, :, ls] * b1[0:1] + b0[0:1]) for i in range(2)], axis=0)
            hf[0, :, ls] = t
            return t

        with scope("f_k"):
            wait_group(G_K - 1)

            def kstep(k, lhs):
                @pl.when(k + 1 < NL)
                def _():
                    copy(('cb', k + 1), G_K + k).wait()
                    copy(('sb', k + 1), G_K + k).wait()
                copy(('wgk', k), G_K + k).wait()
                copy(('wuk', k), G_K + k).wait()
                xk = unpack(lhs)
                gu[:, 0:FC] += jnp.dot(xk, wg_v[blk(k, 128), 0:FC], preferred_element_type=f32)
                nxt = h2_tile(jnp.minimum(k + 1, NL - 1))
                gu[:, FC:2 * FC] += jnp.dot(xk, wu_v[blk(k, 128), 0:FC], preferred_element_type=f32)
                return nxt
            lax.fori_loop(0, NL, kstep, h2_tile(0))
        x = lambda: unpack(hf[0])
        xh = [lambda h=h: unpack(hf[0, h * HT:(h + 1) * HT, :]) for h in range(2)]
        with scope("f_c"):
            wait_group(G_F)
            R.st['a'] = (jnp.maximum(gu[:, 0:FC], 0.0) * gu[:, FC:2 * FC]).astype(bf16)
            for lc in range(NL):
                ls = pl.ds(lc * 128, 128)
                if lc < CFG['fch']:
                    R.fwd_h(2, lc)
                accb.at[R.z0][:, ls] = mm(R.st['a'], lambda: wd_v[0:FC, ls])
        with scope("f_d"):
            wait_group(G_F + 1)
            for lc in range(CFG['fch'], NL):
                R.fwd_h(2, lc)
            for k in range(2 * NQ):
                j, h = k // 2, k % 2
                gu.at[blk(R.z0, 2 * T)][h * T:(h + 1) * T, j * 128:(j + 1) * 128] = R.gcols(xh[h], FC + j * 128, 128)
                if k in CFG['fdx']:
                    lc = CFG['fdx'].index(k)
                    if lc == 0:
                        R.sconv(2, CFG['fdl'])
                    R.fwd_x(2, lc)
        with scope("f_e"):
            wait_group(G_F + 2)
            R.st['g'] = gu[:, 0:FC]
            R.st['acc'] = accb[0]
            R.mac(2)
            R.u_(x, 1); R.d_(1); R.g_(x, 2)
            R.inv()
        with scope("f_f"):
            wait_group(G_F + 3)
            R.ln(2, CFG['fent'])
            g, acc = R.st.pop('g'), R.st.pop('acc')
            act = {}

            def upiece(j, h):
                u = R.ucols(xh[h], F - FC + j * 128, 128)
                act[(h, j)] = jnp.maximum(g[h * T:(h + 1) * T, j * 128:(j + 1) * 128], 0.0) * u
                if j == NQ - 1:
                    act[h] = jnp.concatenate([act.pop((h, i)) for i in range(NQ)], axis=1).astype(bf16)

            def dpiece(lc, h):
                ls = pl.ds(lc * 128, 128)
                d = acc[h * T:(h + 1) * T, lc * 128:(lc + 1) * 128] + jnp.dot(
                    act[h], wd_v[F - FC:F, ls], preferred_element_type=f32)
                o_v[h, :, ls] = (x1b[h, :, ls] + mv[32:33, ls] * d).astype(bf16)

            if CFG['fford'] == 0:
                pieces = [(upiece, j, h) for j in range(NQ) for h in range(2)]
                pieces += [(dpiece, lc, h) for lc in range(NL) for h in range(2)]
            else:
                pieces = [(upiece, j, h) for h in range(2) for j in range(NQ)]
                pieces += [(dpiece, lc, h) for h in range(2) for lc in range(NL)]
            for k, (fn, i, h) in enumerate(pieces):
                fn(i, h)
                if k in CFG['gbp']:
                    ls = pl.ds(CFG['gbp'].index(k) * 128, 128)
                    mv[32:40, ls] = jnp.dot(silu_c(), wm_v[MPOS['gb'], :, ls], preferred_element_type=f32)[0:8]
                if k in CFG['fhp']:
                    R.fwd_h(3, CFG['fhp'].index(k))
                if k in CFG['fxp']:
                    lc = CFG['fxp'].index(k)
                    if not CFG['fscall']:
                        R.sconv(3, CFG['ffl'], [lc])
                    elif lc == 0:
                        R.sconv(3, CFG['ffl'])
                    R.fwd_x(3, lc)
            ocopy(0).start(); ocopy(1).start()

    def steady():
        R = Reg()
        s = pid + 1
        with scope("s_w"):
            for name in [('q', s + 1)] + _kvs(s + 2):
                copy(name, G_STEADY + s - 2).wait()
        with scope("s"):
            xv = unpack(hn_v[0, 0:HT, :])
            x = lambda: xv
            if CFG['premac']:
                R.sconv(s + 2, CFG['sc_lanes'])
                R.mac(s + 1, CFG['tree'], kvb[0, HT:HT + 8, 0:128])
                R.g_(x, 0); R.u_(x, 0); R.d_(0); R.g_(x, 1); R.u_(x, 1)
                R.inv()
                R.ln(s + 1, CFG['lnent'])
                pieces = [lambda lc=lc: R.dp(1, lc) for lc in range(NL)]
                pieces += [lambda j=j: R.gp(x, 2, j) for j in range(NQ)]
                pieces += [lambda j=j: R.up(x, 2, j) for j in range(NQ)]
                pieces += [lambda lc=lc: R.dp(2, lc, s, 1) for lc in range(NL)]
                for k, p in enumerate(pieces):
                    p()
                    if k in CFG['hp']:
                        R.fwd_h(s + 2, CFG['hp'].index(k))
                    if k in CFG['xp']:
                        R.fwd_x(s + 2, CFG['xp'].index(k))
            else:
                R.mac(s + 1, CFG['tree'])
                R.g_(x, 0); R.u_(x, 0); R.d_(0); R.g_(x, 1); R.u_(x, 1)
                R.inv()
                R.ln(s + 1, CFG['lnent'])
                for lc in range(NL):
                    R.dp(1, lc)
                R.tail(x, s, 1, s + 2, True, CFG['hpos'], True)
            ocopy(s).start()

    def last():
        R = Reg()
        s = NS - 2
        with scope("l_w"):
            wait_group(len(GROUPS) - 1)
        with scope("l"):
            xv = unpack(hn_v[0, 0:HT, :])
            x = lambda: xv
            R.mac(s + 1, CFG['ltree'])
            R.g_(x, 0); R.u_(x, 0); R.d_(0); R.g_(x, 1); R.u_(x, 1)
            if CFG['learly']:
                R.inv()
                R.ln(s + 1, 3)
                for lc in range(NL):
                    R.dp(1, lc)
            else:
                R.d_(1)
                R.inv()
                R.ln(s + 1)
            R.g_(x, 2); R.u_(x, 2); R.d_(2)
            R.fin(s)
            ocopy(s).start()
            x = lambda: unpack(hn_v[0, 0:HT, :])
            for c in range(NC - 1):
                R.g_(x, c); R.u_(x, c); R.d_(c)
            R.g_(x, NC - 1); R.u_(x, NC - 1)
            a, acc = R.st.pop('a'), R.st.pop('acc')
            for r0, n in CFG['lastsplit']:
                d = acc[r0:r0 + n] + jnp.dot(a[r0:r0 + n], wd_v[F - FC:F, :], preferred_element_type=f32)
                o_v[s + 1, r0:r0 + n, :] = (x1b[s + 1, r0:r0 + n, :] + mv[32:33, :] * d).astype(bf16)
                ocopy(s + 1, (r0, n)).start()
        with scope("e_w"):
            for t in range(NS - 1):
                ocopy(t).wait()
            for h in CFG['lastsplit']:
                ocopy(NS - 1, h).wait()

    only = CFG['only']
    if only is None or 0 in only:
        pl.when(pid == 0)(first)
    if only is None or 1 in only:
        pl.when(jnp.logical_and(pid >= 1, pid <= NS - 4))(steady)
    if only is None or 2 in only:
        pl.when(pid == NS - 3)(last)


@jax.jit
def pallas_adaLN_cond__ssm_conv_h3__glu_gated_reglu__prompt_kernel(A_q, A_k, A_v, A_shift_k, A_ssm_k, A_ssm_D, B_x, B_W_gate, B_W_up, B_W_down, c, w_mod):
    fwd, inv = _dft_mats()
    any_spec = pl.BlockSpec(memory_space=pl.ANY)
    vm = pltpu.VMEM
    return pl.pallas_call(
        _kernel,
        grid=(NS - 2,),
        in_specs=[any_spec] * 13,
        out_specs=any_spec,
        out_shape=jax.ShapeDtypeStruct((1, S, D), bf16),
        scratch_shapes=[
            vm((NS, T, D), bf16), vm((NS, T, D), bf16), vm((NS, T, D), bf16),
            vm((NBLK, D, NB), bf16),
            vm((D, F), bf16), vm((D, F), bf16), vm((F, D), bf16),
            vm((6, D, D), bf16),
            vm((2 * NB, NB), bf16), vm((NB, 2 * NB), bf16),
            vm((NS, T, D), bf16),
            vm((3 * NS, NG, 32, D), f32),
            vm((1, 2 * NB, D), f32),
            vm((1, T + 32, D), f32),
            vm((1, HT + 32, D), f32),
            vm((64, D), f32),
            vm((1, 2 * T, D), f32),
            vm((NS, T, D), f32),
            vm((1, HT + 32, D), f32),
            vm((1, T, D), f32),
            vm((2, T, D), f32),
            vm((2, T, D), f32),
            vm((2 * T, 2 * FC), f32),
            vm((1, 2 * T, D), f32),
            vm((64, D), f32),
            vm((4, D), bf16), vm((D,), bf16), vm((1, D), bf16),
            pltpu.SemaphoreType.DMA((len(GROUPS),)), pltpu.SemaphoreType.DMA((1,)),
        ],
        compiler_params=pltpu.CompilerParams(vmem_limit_bytes=110 * 1024 * 1024,
                                             dimension_semantics=("arbitrary",)),
    )(A_q, A_k, A_v, A_shift_k.T, A_ssm_k, A_ssm_D, B_W_gate, B_W_up, B_W_down, c, w_mod,
      jnp.asarray(fwd, bf16), jnp.asarray(inv, bf16))
```

```python
import contextlib
import numpy as np
import jax
import jax.numpy as jnp
from jax import lax
from jax.experimental import pallas as pl
from jax.experimental.pallas import tpu as pltpu

S, D, F = 2048, 640, 1536
NB = 128
T = 256
NS = S // T
NBLK = S // NB
FC = 512
NC = F // FC
NQ = FC // 128
NL = D // 128
NG = NB // 8
HT = T // 2
RG = 16
EPS = 1e-5
f32 = jnp.float32
bf16 = jnp.bfloat16
i32 = jnp.int32

CFG = dict(
    only=None, scopes=False,
    tree=(1, 2, 3, 4, 5), ltree=(2, 5),
    hp=(0, 2, 4, 6, 8), xp=(10, 12, 13, 15, 17),
    fch=4, fdx=(3, 4, 5, 6, 7),
    gbp=(0, 1, 2, 3, 4), fhp=(7, 9, 11, 13, 15), fxp=(10, 12, 14, 16, 17),
    lastsplit=((0, 128), (128, 64), (192, 32), (224, 32)),
)

MPOS = {'sa': 0, 'ca': 1, 'ga': 2, 'sb': 3, 'cb': 4, 'gb': 5}


def _dft_mats():
    f = np.concatenate([np.arange(0, NB, 2), np.arange(1, NB, 2)])
    j = np.arange(NB)
    ang = 2.0 * np.pi * (((2 * f[:, None] + 1) * j[None, :]) % (4 * NB)) / (4 * NB)
    fwd = np.stack([np.cos(ang).reshape(NG, 8, NB), np.sin(ang).reshape(NG, 8, NB)], axis=1).reshape(2 * NB, NB)
    return fwd.astype(np.float32), (fwd.T / NB).astype(np.float32)


def _kvs(s):
    return [('k', s), ('v', s), ('s', 2 * s), ('s', 2 * s + 1)]


GROUPS = [
    ['sh', 'dd', 'c', 'fw', 'iv'] + _kvs(0),
    [('q', 0), ('q', 1)],
    _kvs(1),
    [('wm', 0), ('wm', 1)],
    [('wm', 2)],
    [('cb', 0), ('sb', 0)],
]
G_K = len(GROUPS)
for _k in range(NL):
    GROUPS.append(([('cb', _k + 1), ('sb', _k + 1)] if _k + 1 < NL else []) + [('wgk', _k), ('wuk', _k)])
G_F = len(GROUPS)
GROUPS += [
    [('s', 4), ('s', 5), ('wd', 0)],
    [('k', 2), ('v', 2), ('wg', 1)],
    [('wu', 1), ('wd', 1), ('wg', 2)],
    [('wu', 2), ('wd', 2), ('wm', 5), ('q', 2)] + _kvs(3),
]
G_STEADY = len(GROUPS)
for _s in range(2, NS - 2):
    GROUPS.append([('q', _s + 1)] + _kvs(_s + 2))
GROUPS.append([('q', NS - 1)])


def _kernel(q_hbm, k_hbm, v_hbm, sh_hbm, ssm_hbm, dd_hbm, wg_hbm, wu_hbm, wd_hbm, c_hbm, wm_hbm,
            fw_hbm, iv_hbm, o_hbm,
            q_v, k_v, v_v, ssm_v, wg_v, wu_v, wd_v, wm_v, fw_v, iv_v, o_v,
            uv, ap, zb, kvb, mv, yb, x1b, hn_v, hf, n1, n2, gu, accb, tp, sh_v, dd_v, c_v,
            sems, osem):
    pid = pl.program_id(0)

    def blk(j, n):
        return pl.ds(j * n, n) if isinstance(j, int) else pl.ds(pl.multiple_of(j * n, n), n)

    small = {'sh': (sh_hbm, sh_v), 'dd': (dd_hbm, dd_v), 'c': (c_hbm, c_v), 'fw': (fw_hbm, fw_v),
             'iv': (iv_hbm, iv_v)}

    def copy(name, gi):
        sem = sems.at[gi]
        if isinstance(name, str):
            return pltpu.make_async_copy(small[name][0], small[name][1], sem)
        kind, j = name
        if kind in ('q', 'k', 'v'):
            src, dst = {'q': (q_hbm, q_v), 'k': (k_hbm, k_v), 'v': (v_hbm, v_v)}[kind]
            return pltpu.make_async_copy(src.at[0, blk(j, T), :], dst.at[j], sem)
        if kind == 's':
            return pltpu.make_async_copy(ssm_hbm.at[:, blk(j, NB)], ssm_v.at[j], sem)
        if kind == 'wm':
            return pltpu.make_async_copy(wm_hbm.at[:, blk(j, D)], wm_v.at[j], sem)
        if kind in ('cb', 'sb'):
            p = MPOS[kind]
            c0 = p * D + j * 128 if isinstance(j, int) else pl.multiple_of(p * D + j * 128, 128)
            return pltpu.make_async_copy(wm_hbm.at[:, pl.ds(c0, 128)], wm_v.at[p, :, blk(j, 128)], sem)
        if kind in ('wgk', 'wuk'):
            src, dst = (wg_hbm, wg_v) if kind == 'wgk' else (wu_hbm, wu_v)
            return pltpu.make_async_copy(src.at[blk(j, 128), 0:FC], dst.at[blk(j, 128), 0:FC], sem)
        if kind == 'wd':
            return pltpu.make_async_copy(wd_hbm.at[blk(j, FC), :], wd_v.at[blk(j, FC), :], sem)
        src, dst = (wg_hbm, wg_v) if kind[1] == 'g' else (wu_hbm, wu_v)
        return pltpu.make_async_copy(src.at[:, blk(j, FC)], dst.at[:, blk(j, FC)], sem)

    def wait_group(gi):
        for name in GROUPS[gi]:
            copy(name, gi).wait()

    def ocopy(j, h=None):
        if h is None:
            return pltpu.make_async_copy(o_v.at[j], o_hbm.at[0, blk(j, T), :], osem.at[0])
        r0, n = h
        return pltpu.make_async_copy(o_v.at[j, pl.ds(r0, n), :], o_hbm.at[0, pl.ds(j * T + r0, n), :], osem.at[0])

    def scope(name):
        return jax.named_scope(name) if CFG['scopes'] else contextlib.nullcontext()

    def pack(x):
        return pltpu.bitcast(x.astype(bf16), f32)

    def unpack(x):
        return pltpu.bitcast(x, bf16)

    def rowsum(x, tok=None):
        ps = x[:, 0:128]
        if tok is not None:
            ps = ps + jnp.concatenate([tok] * (x.shape[0] // 8), axis=0)
        for lc in range(1, NL):
            ps = ps + x[:, lc * 128:(lc + 1) * 128]
        return jnp.sum(ps, axis=-1, keepdims=True)

    def normalise(x, tok=None, ent=4):
        xc = x - rowsum(x, tok if ent == 3 else None) * (1.0 / D)
        var = rowsum(xc * xc, tok if ent == 4 else None) * (1.0 / D) + EPS
        return xc * lax.rsqrt(var)

    def fold(a, p):
        parts = []
        for g in range(NG):
            ar, ai = a[16 * g:16 * g + 8], a[16 * g + 8:16 * g + 16]
            pr, pi = p[16 * g:16 * g + 8], p[16 * g + 8:16 * g + 16]
            parts += [ar + pi, ai - pr] if g < NG // 2 else [ar - pi, ai + pr]
        return jnp.concatenate(parts, axis=0)

    def grp(x):
        return x.reshape(NG, 16, 128)

    row = lax.broadcasted_iota(i32, (8, 128), 0)

    def conv_rows(s, ls, emit, tok_in=None):
        w = [tp[8 * j:8 * j + 8, ls] for j in range(4)]
        if isinstance(s, int) and s == 0:
            pk = jnp.zeros((8, 128), f32)
            pt = jnp.zeros((8, 128), f32)
        else:
            kp = k_v[s - 1, T - 16:T, ls].astype(f32)[8:16]
            pk = pltpu.roll(kp, 1, 0)
            pt = pltpu.roll(w[2] * kp + w[3] * pk, 2, 0)
        for rg in range(T // 16):
            kk = k_v[s, rg * 16:rg * 16 + 16, ls].astype(f32)
            vv = v_v[s, rg * 16:rg * 16 + 16, ls].astype(f32)
            outs = []
            for h in range(2):
                kc = kk[8 * h:8 * h + 8]
                if h == 0 and tok_in is not None and tok_in() is not None:
                    kc = kc + tok_in()
                rk = pltpu.roll(kc, 1, 0)
                sk = jnp.where(row < 1, pk, rk)
                t = w[2] * kc + w[3] * sk
                rt = pltpu.roll(t, 2, 0)
                outs.append(((w[0] * kc + w[1] * sk) + jnp.where(row < 2, pt, rt)) * vv[8 * h:8 * h + 8])
                pk, pt = rk, rt
            emit(rg, pack(jnp.concatenate(outs, axis=0)))

    def dft_x(kv0, kv1, split=False):
        w = unpack(jnp.concatenate([kv0, kv1], axis=1))
        if split:
            xx = jnp.concatenate([jnp.dot(fw_v[h * NB:(h + 1) * NB, :], w, preferred_element_type=f32)
                                  for h in range(2)], axis=0)
        else:
            xx = jnp.dot(fw_v[...], w, preferred_element_type=f32)
        return xx[:, 0:128], xx[:, 128:256]

    def dft_h(s, rows):
        w = jnp.concatenate([ssm_v[2 * s, rows, :], ssm_v[2 * s + 1, rows, :]], axis=0)
        aa = lax.dot_general(fw_v[...], w, (((1,), (1,)), ((), ())), preferred_element_type=f32)
        return aa[:, 0:128], aa[:, 128:256]

    def silu_c():
        return unpack(tp[40:48, :])

    def modvec(p):
        return jnp.dot(silu_c(), wm_v[p], preferred_element_type=f32)[0:8]

    def mm(lhs, w):
        if lhs.shape[0] <= T:
            return jnp.dot(lhs, w(), preferred_element_type=f32)
        return jnp.concatenate([jnp.dot(lhs[r:r + T], w(), preferred_element_type=f32)
                                for r in range(0, lhs.shape[0], T)], axis=0)

    class Reg:
        def __init__(self):
            self.z0 = lax.shift_right_logical(pid, 8)
            self.st = {}

        def sconv(self, s, lanes, lcs=None):
            if lcs is None or lcs[0] == 0:
                self.sc = [None] * lanes
                self.gi = 0
            for lc in (range(NL) if lcs is None else lcs):
                ls = pl.ds(lc * 128, 128)

                def emit(rg, kvp, ls=ls):
                    kvb.at[self.z0][rg * 8:rg * 8 + 8, ls] = kvp
                    self.sc[self.gi % lanes] = kvb[0, HT:HT + 8, ls]
                    self.gi += 1
                conv_rows(s, ls, emit, lambda: self.sc[self.gi % lanes])

        def fwd_x(self, s, lc):
            o = self.z0 + 3 * s
            ls = pl.ds(lc * 128, 128)
            x0, x1 = dft_x(kvb[0, 0:64, ls], kvb[0, 64:128, ls])
            p = 3 * (s - 1)
            u1 = (uv[p + 2, :, 16:32, ls] + uv[p, :, 16:32, ls]) - grp(x0)
            uv[o, :, 16:32, ls] = grp(x0)
            uv[o + 1, :, 16:32, ls] = u1
            uv[o + 2, :, 16:32, ls] = grp(x1 - x0)

        def fwd_h(self, s, lc):
            o = self.z0 + 3 * s
            ls = pl.ds(lc * 128, 128)
            a0, a1 = dft_h(s, ls)
            h0 = fold(a0, ap[0, :, ls])
            h1 = fold(a1, a0)
            uv[o, :, 0:16, ls] = grp(h0 + h1)
            uv[o + 1, :, 0:16, ls] = grp(h1)
            uv[o + 2, :, 0:16, ls] = grp(h0)
            ap[self.z0, :, ls] = a1

        def mac(self, s, tree=(), tok0=None):
            static = isinstance(s, int)
            ng = s + 1 if static else NS - 1
            ub = [3 * (s - g) if static else 3 * jnp.maximum(s - g, 0) for g in range(ng)]
            toks = (tok0, tok0)
            for fc in range(NG):
                for lc in range(NL):
                    ls = pl.ds(lc * 128, 128)

                    def chain(j, ar, ai):
                        for g in range(ng):
                            hr = uv[3 * g + j, fc, 0:8, ls]
                            hi = uv[3 * g + j, fc, 8:16, ls]
                            xr = uv[ub[g] + j, fc, 16:24, ls]
                            xi = uv[ub[g] + j, fc, 24:32, ls]
                            if ar is not None and g in tree:
                                ar = ar + (hr * xr - hi * xi)
                                ai = ai + (hr * xi + hi * xr)
                            else:
                                ar = (hr * xr if ar is None else ar + hr * xr) - hi * xi
                                ai = (hr * xi if ai is None else ai + hr * xi) + hi * xr
                        return ar, ai

                    a1 = chain(0, *toks)
                    z0 = chain(1, *a1)
                    zero = pltpu.bitcast(zb[0, T:T + 8, ls], i32)

                    def tk(v):
                        return pltpu.bitcast(pltpu.bitcast(v, i32) & zero, f32)
                    z1 = chain(2, a1[0] + tk(z0[0]), a1[1] + tk(z0[1]))
                    for b, z in enumerate((z0, z1)):
                        zb.at[self.z0][b * HT + fc * 8:b * HT + fc * 8 + 8, ls] = pack(jnp.concatenate(z, axis=0))
                    toks = (tk(z1[0]), tk(z1[1]))

        def inv(self):
            for b in range(2):
                yb[self.z0, b * NB:(b + 1) * NB, :] = jnp.dot(
                    iv_v[...], unpack(zb[0, b * HT:(b + 1) * HT, :]), preferred_element_type=f32)

        def ln(self, s, ent=4):
            a1 = mv[0:1, :]; a0 = mv[8:9, :]; b1 = mv[16:17, :]; b0 = mv[24:25, :]
            tok = None
            for g in range(T // RG):
                gr = slice(g * RG, (g + 1) * RG)
                x = q_v[s, gr, :].astype(f32)
                x1 = x + (normalise(x) * a1 + a0) * yb[0, gr, :]
                x1b[self.z0 + s, gr, :] = x1
                h2 = normalise(x1, tok, ent) * b1 + b0
                hn_v.at[self.z0][g * (RG // 2):(g + 1) * (RG // 2), :] = pack(h2)
                tok = hn_v[0, HT:HT + 8, 0:128]

        def gcols(self, x, c0, n):
            return mm(x(), lambda: wg_v[:, c0:c0 + n])

        def ucols(self, x, c0, n):
            return mm(x(), lambda: wu_v[:, c0:c0 + n])

        def g_(self, x, c):
            self.st['g'] = self.gcols(x, c * FC, FC)

        def u_(self, x, c):
            self.st['a'] = (jnp.maximum(self.st.pop('g'), 0.0) * self.ucols(x, c * FC, FC)).astype(bf16)

        def d_(self, c):
            d = mm(self.st.pop('a'), lambda: wd_v[c * FC:(c + 1) * FC, :])
            self.st['acc'] = d if c == 0 else self.st['acc'] + d

        def gp(self, x, c, j):
            self.st[('g', j)] = self.gcols(x, c * FC + j * 128, 128)

        def up(self, x, c, j):
            self.st[('a', j)] = jnp.maximum(self.st.pop(('g', j)), 0.0) * self.ucols(x, c * FC + j * 128, 128)
            if j == NQ - 1:
                self.st['a'] = jnp.concatenate([self.st.pop(('a', i)) for i in range(NQ)], axis=1).astype(bf16)

        def dp(self, c, lc, s=None):
            ls = pl.ds(lc * 128, 128)
            d = mm(self.st['a'], lambda: wd_v[c * FC:(c + 1) * FC, ls])
            d = self.st['acc'][:, lc * 128:(lc + 1) * 128] + d
            if c == NC - 1:
                o_v[s, :, ls] = (x1b[s, :, ls] + mv[32:33, ls] * d).astype(bf16)
            else:
                self.st[('d', lc)] = d
                if lc == NL - 1:
                    self.st['acc'] = jnp.concatenate([self.st.pop(('d', i)) for i in range(NL)], axis=1)

        def fin(self, s):
            o_v[s] = (x1b[s] + mv[32:33, :] * self.st.pop('acc')).astype(bf16)

    def first():
        R = Reg()
        for gi, names in enumerate(GROUPS):
            for name in names:
                copy(name, gi).start()
        z = jnp.zeros((8, D), f32)
        kvb[0, HT:HT + 8, :] = z
        hn_v[0, HT:HT + 8, :] = z
        zb[0, T:T + 8, :] = z

        def zero_v(j, _):
            uv[j, :, 0:16, :] = jnp.zeros((NG, 16, D), f32)
            return 0
        lax.fori_loop(12, 3 * (NS - 1), zero_v, 0)

        def zero_gu(j, _):
            gu[blk(j, 64), :] = jnp.zeros((64, 2 * FC), f32)
            return 0
        lax.fori_loop(0, 2 * T // 64, zero_gu, 0)

        def cmul(h, x):
            return (h[:, 0:8] * x[:, 0:8] - h[:, 8:16] * x[:, 8:16], h[:, 0:8] * x[:, 8:16] + h[:, 8:16] * x[:, 0:8])

        def conv_pair(s):
            def body(lc, _):
                ls = blk(lc, 128)
                if s == 1:
                    for k in range(7):
                        g = jnp.minimum(lc * 7 + k, 2 * T // RG - 1)
                        gr = blk(g % (T // RG), RG)
                        n1[g // (T // RG), gr, :] = normalise(q_v[g // (T // RG), gr, :].astype(f32))
                    for b in range(2):
                        yb[0, b * NB:(b + 1) * NB, ls] = jnp.dot(
                            iv_v[...], unpack(n2[0, b * HT:(b + 1) * HT, ls]), preferred_element_type=f32)
                rows = []
                conv_rows(s, ls, lambda rg, kvp: rows.append(kvp))
                a0, a1 = dft_h(s, ls)
                x0, x1 = dft_x(jnp.concatenate(rows[0:8], axis=0), jnp.concatenate(rows[8:16], axis=0), True)
                if s == 0:
                    dd = tp[32:40, ls]
                    h0 = jnp.concatenate([a0[8 * g:8 * g + 8] + dd if g % 2 == 0 else a0[8 * g:8 * g + 8]
                                          for g in range(2 * NG)], axis=0)
                    u1 = grp(-x0)
                else:
                    h0 = fold(a0, ap[0, :, ls])
                    u1 = (uv[2, :, 16:32, ls] + uv[0, :, 16:32, ls]) - grp(x0)
                h1 = fold(a1, a0)
                us = [grp(x0), u1, grp(x1 - x0)]
                vs = [grp(h0 + h1), grp(h1), grp(h0)]
                if s == 0:
                    p = [cmul(vs[j], us[j]) for j in range(3)]
                else:
                    p = []
                    for j in range(3):
                        t0 = cmul(uv[j, :, 0:16, ls], us[j])
                        t1 = cmul(vs[j], uv[j, :, 16:32, ls])
                        p.append((t0[0] + t1[0], t0[1] + t1[1]))
                for j in range(3):
                    uv[3 * s + j, :, 16:32, ls] = us[j]
                    uv[3 * s + j, :, 0:16, ls] = vs[j]
                ap[0, :, ls] = a1
                for b in range(2):
                    zz = jnp.concatenate([p[0][0] + p[1 + b][0], p[0][1] + p[1 + b][1]], axis=1)
                    n2[s, b * HT:(b + 1) * HT, ls] = pack(zz.reshape(2 * NB, 128))
                return 0
            lax.fori_loop(0, NL, body, 0)

        with scope("p_w0"):
            wait_group(0)
        with scope("p_c0"):
            taps = sh_v[...].astype(f32)
            for j in range(4):
                tp[8 * j:8 * j + 8, :] = jnp.broadcast_to(taps[j:j + 1, :], (8, D))
            tp[32:40, :] = jnp.broadcast_to(dd_v[...].astype(f32).reshape(1, D), (8, D))
            c32 = c_v[...].astype(f32)
            tp[40:48, :] = pack(jnp.broadcast_to(c32 * jax.nn.sigmoid(c32), (16, D)))
            conv_pair(0)
        with scope("p_c1"):
            wait_group(1)
            wait_group(2)
            conv_pair(1)

            wait_group(3)
            for b in range(2):
                yb[0, T + b * NB:T + (b + 1) * NB, :] = jnp.dot(
                    iv_v[...], unpack(n2[1, b * HT:(b + 1) * HT, :]), preferred_element_type=f32)
            sa, ca1 = modvec(MPOS['sa']), 1.0 + modvec(MPOS['ca'])
            mv[40:48, :] = sa
            mv[48:56, :] = ca1

            def pre(i, _):
                r = blk(i, 64)
                for h in range(2):
                    y = yb[0, pl.ds(pl.multiple_of(h * T + i * 64, 64), 64), :]
                    n1[h, r, :] = (n1[h, r, :] * mv[48:49, :] + mv[40:41, :]) * y
                return 0
            lax.fori_loop(0, T // 64, pre, 0)
        with scope("p_ln2"):
            wait_group(4)
            ga = modvec(MPOS['ga'])
            mv[0:8, :] = ga * mv[48:56, :]
            mv[8:16, :] = ga * mv[40:48, :]
            for i in range(2):
                for g in range(T // RG):
                    gr = slice(g * RG, (g + 1) * RG)
                    x1 = q_v[i, gr, :].astype(f32) + ga[0:1] * n1[i, gr, :]
                    x1b[i, gr, :] = x1
                    n2[R.z0 + i, gr, :] = normalise(x1)

        def h2_tile(k):
            ls = blk(k, 128)
            b1 = 1.0 + jnp.dot(silu_c(), wm_v[MPOS['cb'], :, ls], preferred_element_type=f32)[0:8]
            b0 = jnp.dot(silu_c(), wm_v[MPOS['sb'], :, ls], preferred_element_type=f32)[0:8]
            mv[16:24, ls] = b1
            mv[24:32, ls] = b0
            t = jnp.concatenate([pack(n2[i, :, ls] * b1[0:1] + b0[0:1]) for i in range(2)], axis=0)
            hf[0, :, ls] = t
            return t

        with scope("f_k"):
            wait_group(G_K - 1)

            def kstep(k, lhs):
                @pl.when(k + 1 < NL)
                def _():
                    copy(('cb', k + 1), G_K + k).wait()
                    copy(('sb', k + 1), G_K + k).wait()
                copy(('wgk', k), G_K + k).wait()
                copy(('wuk', k), G_K + k).wait()
                xk = unpack(lhs)
                gu[:, 0:FC] += jnp.dot(xk, wg_v[blk(k, 128), 0:FC], preferred_element_type=f32)
                nxt = h2_tile(jnp.minimum(k + 1, NL - 1))
                gu[:, FC:2 * FC] += jnp.dot(xk, wu_v[blk(k, 128), 0:FC], preferred_element_type=f32)
                return nxt
            lax.fori_loop(0, NL, kstep, h2_tile(0))
        x = lambda: unpack(hf[0])
        xh = [lambda h=h: unpack(hf[0, h * HT:(h + 1) * HT, :]) for h in range(2)]
        with scope("f_c"):
            wait_group(G_F)
            R.st['a'] = (jnp.maximum(gu[:, 0:FC], 0.0) * gu[:, FC:2 * FC]).astype(bf16)
            for lc in range(NL):
                ls = pl.ds(lc * 128, 128)
                if lc < CFG['fch']:
                    R.fwd_h(2, lc)
                accb.at[R.z0][:, ls] = mm(R.st['a'], lambda: wd_v[0:FC, ls])
        with scope("f_d"):
            wait_group(G_F + 1)
            for lc in range(CFG['fch'], NL):
                R.fwd_h(2, lc)
            for k in range(2 * NQ):
                j, h = k // 2, k % 2
                gu.at[blk(R.z0, 2 * T)][h * T:(h + 1) * T, j * 128:(j + 1) * 128] = R.gcols(xh[h], FC + j * 128, 128)
                if k in CFG['fdx']:
                    lc = CFG['fdx'].index(k)
                    if lc == 0:
                        R.sconv(2, 2)
                    R.fwd_x(2, lc)
        with scope("f_e"):
            wait_group(G_F + 2)
            R.st['g'] = gu[:, 0:FC]
            R.st['acc'] = accb[0]
            R.mac(2)
            R.u_(x, 1); R.d_(1); R.g_(x, 2)
            R.inv()
        with scope("f_f"):
            wait_group(G_F + 3)
            R.ln(2, 4)
            g, acc = R.st.pop('g'), R.st.pop('acc')
            act = {}

            def upiece(j, h):
                u = R.ucols(xh[h], F - FC + j * 128, 128)
                act[(h, j)] = jnp.maximum(g[h * T:(h + 1) * T, j * 128:(j + 1) * 128], 0.0) * u
                if j == NQ - 1:
                    act[h] = jnp.concatenate([act.pop((h, i)) for i in range(NQ)], axis=1).astype(bf16)

            def dpiece(lc, h):
                ls = pl.ds(lc * 128, 128)
                d = acc[h * T:(h + 1) * T, lc * 128:(lc + 1) * 128] + jnp.dot(
                    act[h], wd_v[F - FC:F, ls], preferred_element_type=f32)
                o_v[h, :, ls] = (x1b[h, :, ls] + mv[32:33, ls] * d).astype(bf16)

            pieces = [(upiece, j, h) for j in range(NQ) for h in range(2)]
            pieces += [(dpiece, lc, h) for lc in range(NL) for h in range(2)]
            for k, (fn, i, h) in enumerate(pieces):
                fn(i, h)
                if k in CFG['gbp']:
                    ls = pl.ds(CFG['gbp'].index(k) * 128, 128)
                    mv[32:40, ls] = jnp.dot(silu_c(), wm_v[MPOS['gb'], :, ls], preferred_element_type=f32)[0:8]
                if k in CFG['fhp']:
                    R.fwd_h(3, CFG['fhp'].index(k))
                if k in CFG['fxp']:
                    lc = CFG['fxp'].index(k)
                    R.sconv(3, 2, [lc])
                    R.fwd_x(3, lc)
            ocopy(0).start(); ocopy(1).start()

    def steady():
        R = Reg()
        s = pid + 1
        with scope("s_w"):
            for name in [('q', s + 1)] + _kvs(s + 2):
                copy(name, G_STEADY + s - 2).wait()
        with scope("s"):
            xv = unpack(hn_v[0, 0:HT, :])
            x = lambda: xv
            R.sconv(s + 2, 2)
            R.mac(s + 1, CFG['tree'], kvb[0, HT:HT + 8, 0:128])
            R.g_(x, 0); R.u_(x, 0); R.d_(0); R.g_(x, 1); R.u_(x, 1)
            R.inv()
            R.ln(s + 1, 3)
            pieces = [lambda lc=lc: R.dp(1, lc) for lc in range(NL)]
            pieces += [lambda j=j: R.gp(x, 2, j) for j in range(NQ)]
            pieces += [lambda j=j: R.up(x, 2, j) for j in range(NQ)]
            pieces += [lambda lc=lc: R.dp(2, lc, s) for lc in range(NL)]
            for k, p in enumerate(pieces):
                p()
                if k in CFG['hp']:
                    R.fwd_h(s + 2, CFG['hp'].index(k))
                if k in CFG['xp']:
                    R.fwd_x(s + 2, CFG['xp'].index(k))
            ocopy(s).start()

    def last():
        R = Reg()
        s = NS - 2
        with scope("l_w"):
            wait_group(len(GROUPS) - 1)
        with scope("l"):
            xv = unpack(hn_v[0, 0:HT, :])
            x = lambda: xv
            R.mac(s + 1, CFG['ltree'])
            R.g_(x, 0); R.u_(x, 0); R.d_(0); R.g_(x, 1); R.u_(x, 1); R.d_(1)
            R.inv()
            R.ln(s + 1, 4)
            R.g_(x, 2); R.u_(x, 2); R.d_(2)
            R.fin(s)
            ocopy(s).start()
            x = lambda: unpack(hn_v[0, 0:HT, :])
            for c in range(NC - 1):
                R.g_(x, c); R.u_(x, c); R.d_(c)
            R.g_(x, NC - 1); R.u_(x, NC - 1)
            a, acc = R.st.pop('a'), R.st.pop('acc')
            for r0, n in CFG['lastsplit']:
                d = acc[r0:r0 + n] + jnp.dot(a[r0:r0 + n], wd_v[F - FC:F, :], preferred_element_type=f32)
                o_v[s + 1, r0:r0 + n, :] = (x1b[s + 1, r0:r0 + n, :] + mv[32:33, :] * d).astype(bf16)
                ocopy(s + 1, (r0, n)).start()
        with scope("e_w"):
            for t in range(NS - 1):
                ocopy(t).wait()
            for h in CFG['lastsplit']:
                ocopy(NS - 1, h).wait()

    only = CFG['only']
    if only is None or 0 in only:
        pl.when(pid == 0)(first)
    if only is None or 1 in only:
        pl.when(jnp.logical_and(pid >= 1, pid <= NS - 4))(steady)
    if only is None or 2 in only:
        pl.when(pid == NS - 3)(last)


@jax.jit
def pallas_adaLN_cond__ssm_conv_h3__glu_gated_reglu__prompt_kernel(A_q, A_k, A_v, A_shift_k, A_ssm_k, A_ssm_D, B_x, B_W_gate, B_W_up, B_W_down, c, w_mod):
    fwd, inv = _dft_mats()
    any_spec = pl.BlockSpec(memory_space=pl.ANY)
    vm = pltpu.VMEM
    return pl.pallas_call(
        _kernel,
        grid=(NS - 2,),
        in_specs=[any_spec] * 13,
        out_specs=any_spec,
        out_shape=jax.ShapeDtypeStruct((1, S, D), bf16),
        scratch_shapes=[
            vm((NS, T, D), bf16), vm((NS, T, D), bf16), vm((NS, T, D), bf16),
            vm((NBLK, D, NB), bf16),
            vm((D, F), bf16), vm((D, F), bf16), vm((F, D), bf16),
            vm((6, D, D), bf16),
            vm((2 * NB, NB), bf16), vm((NB, 2 * NB), bf16),
            vm((NS, T, D), bf16),
            vm((3 * NS, NG, 32, D), f32),
            vm((1, 2 * NB, D), f32),
            vm((1, T + 32, D), f32),
            vm((1, HT + 32, D), f32),
            vm((64, D), f32),
            vm((1, 2 * T, D), f32),
            vm((NS, T, D), f32),
            vm((1, HT + 32, D), f32),
            vm((1, T, D), f32),
            vm((2, T, D), f32),
            vm((2, T, D), f32),
            vm((2 * T, 2 * FC), f32),
            vm((1, 2 * T, D), f32),
            vm((64, D), f32),
            vm((4, D), bf16), vm((D,), bf16), vm((1, D), bf16),
            pltpu.SemaphoreType.DMA((len(GROUPS),)), pltpu.SemaphoreType.DMA((1,)),
        ],
        compiler_params=pltpu.CompilerParams(vmem_limit_bytes=110 * 1024 * 1024,
                                             dimension_semantics=("arbitrary",)),
    )(A_q, A_k, A_v, A_shift_k.T, A_ssm_k, A_ssm_D, B_W_gate, B_W_up, B_W_down, c, w_mod,
      jnp.asarray(fwd, bf16), jnp.asarray(inv, bf16))
```

```python
import contextlib
import numpy as np
import jax
import jax.numpy as jnp
from jax import lax
from jax.experimental import pallas as pl
from jax.experimental.pallas import tpu as pltpu

S, D, F = 2048, 640, 1536
NB = 128
T = 256
NS = S // T
NBLK = S // NB
FC = 512
NC = F // FC
NQ = FC // 128
NL = D // 128
NG = NB // 8
HT = T // 2
RG = 16
EPS = 1e-5
f32 = jnp.float32
bf16 = jnp.bfloat16
i32 = jnp.int32

CFG = dict(
    only=None, scopes=False,
    tree=(1, 2, 3, 4, 5), ltree=(2, 5),
    hp=(0, 2, 4, 6, 8), xp=(10, 12, 13, 15, 17),
    ftree=(1, 2), finv=0, fent=3, fscall=True,
    fch=4, fdx=(3, 4, 5, 6, 7),
    gbp=(1, 3, 5, 6, 7), fhp=(0, 2, 4, 6, 8), fxp=(10, 12, 13, 15, 17),
    lastsplit=((0, 128), (128, 64), (192, 32), (224, 32)),
)

MPOS = {'sa': 0, 'ca': 1, 'ga': 2, 'sb': 3, 'cb': 4, 'gb': 5}


def _dft_mats():
    f = np.concatenate([np.arange(0, NB, 2), np.arange(1, NB, 2)])
    j = np.arange(NB)
    ang = 2.0 * np.pi * (((2 * f[:, None] + 1) * j[None, :]) % (4 * NB)) / (4 * NB)
    fwd = np.stack([np.cos(ang).reshape(NG, 8, NB), np.sin(ang).reshape(NG, 8, NB)], axis=1).reshape(2 * NB, NB)
    return fwd.astype(np.float32), (fwd.T / NB).astype(np.float32)


def _kvs(s):
    return [('k', s), ('v', s), ('s', 2 * s), ('s', 2 * s + 1)]


GROUPS = [
    ['sh', 'dd', 'c', 'fw', 'iv'] + _kvs(0),
    [('q', 0), ('q', 1)],
    _kvs(1),
    [('wm', 0), ('wm', 1)],
    [('wm', 2)],
    [('cb', 0), ('sb', 0)],
]
G_K = len(GROUPS)
for _k in range(NL):
    GROUPS.append(([('cb', _k + 1), ('sb', _k + 1)] if _k + 1 < NL else []) + [('wgk', _k), ('wuk', _k)])
G_F = len(GROUPS)
GROUPS += [
    [('s', 4), ('s', 5), ('wd', 0)],
    [('k', 2), ('v', 2), ('wg', 1)],
    [('wu', 1), ('wd', 1), ('wg', 2), ('q', 2)],
    [('wu', 2), ('wd', 2), ('wm', 5)] + _kvs(3),
]
G_STEADY = len(GROUPS)
for _s in range(2, NS - 2):
    GROUPS.append([('q', _s + 1)] + _kvs(_s + 2))
GROUPS.append([('q', NS - 1)])


def _kernel(q_hbm, k_hbm, v_hbm, sh_hbm, ssm_hbm, dd_hbm, wg_hbm, wu_hbm, wd_hbm, c_hbm, wm_hbm,
            fw_hbm, iv_hbm, o_hbm,
            q_v, k_v, v_v, ssm_v, wg_v, wu_v, wd_v, wm_v, fw_v, iv_v, o_v,
            uv, ap, zb, kvb, mv, yb, x1b, hn_v, hf, n1, n2, gu, accb, tp, sh_v, dd_v, c_v,
            sems, osem):
    pid = pl.program_id(0)

    def blk(j, n):
        return pl.ds(j * n, n) if isinstance(j, int) else pl.ds(pl.multiple_of(j * n, n), n)

    small = {'sh': (sh_hbm, sh_v), 'dd': (dd_hbm, dd_v), 'c': (c_hbm, c_v), 'fw': (fw_hbm, fw_v),
             'iv': (iv_hbm, iv_v)}

    def copy(name, gi):
        sem = sems.at[gi]
        if isinstance(name, str):
            return pltpu.make_async_copy(small[name][0], small[name][1], sem)
        kind, j = name
        if kind in ('q', 'k', 'v'):
            src, dst = {'q': (q_hbm, q_v), 'k': (k_hbm, k_v), 'v': (v_hbm, v_v)}[kind]
            return pltpu.make_async_copy(src.at[0, blk(j, T), :], dst.at[j], sem)
        if kind == 's':
            return pltpu.make_async_copy(ssm_hbm.at[:, blk(j, NB)], ssm_v.at[j], sem)
        if kind == 'wm':
            return pltpu.make_async_copy(wm_hbm.at[:, blk(j, D)], wm_v.at[j], sem)
        if kind in ('cb', 'sb'):
            p = MPOS[kind]
            c0 = p * D + j * 128 if isinstance(j, int) else pl.multiple_of(p * D + j * 128, 128)
            return pltpu.make_async_copy(wm_hbm.at[:, pl.ds(c0, 128)], wm_v.at[p, :, blk(j, 128)], sem)
        if kind in ('wgk', 'wuk'):
            src, dst = (wg_hbm, wg_v) if kind == 'wgk' else (wu_hbm, wu_v)
            return pltpu.make_async_copy(src.at[blk(j, 128), 0:FC], dst.at[blk(j, 128), 0:FC], sem)
        if kind == 'wd':
            return pltpu.make_async_copy(wd_hbm.at[blk(j, FC), :], wd_v.at[blk(j, FC), :], sem)
        src, dst = (wg_hbm, wg_v) if kind[1] == 'g' else (wu_hbm, wu_v)
        return pltpu.make_async_copy(src.at[:, blk(j, FC)], dst.at[:, blk(j, FC)], sem)

    def wait_group(gi):
        for name in GROUPS[gi]:
            copy(name, gi).wait()

    def ocopy(j, h=None):
        if h is None:
            return pltpu.make_async_copy(o_v.at[j], o_hbm.at[0, blk(j, T), :], osem.at[0])
        r0, n = h
        return pltpu.make_async_copy(o_v.at[j, pl.ds(r0, n), :], o_hbm.at[0, pl.ds(j * T + r0, n), :], osem.at[0])

    def scope(name):
        return jax.named_scope(name) if CFG['scopes'] else contextlib.nullcontext()

    def pack(x):
        return pltpu.bitcast(x.astype(bf16), f32)

    def unpack(x):
        return pltpu.bitcast(x, bf16)

    def rowsum(x, tok=None):
        ps = x[:, 0:128]
        if tok is not None:
            ps = ps + jnp.concatenate([tok] * (x.shape[0] // 8), axis=0)
        for lc in range(1, NL):
            ps = ps + x[:, lc * 128:(lc + 1) * 128]
        return jnp.sum(ps, axis=-1, keepdims=True)

    def normalise(x, tok=None, ent=4):
        xc = x - rowsum(x, tok if ent == 3 else None) * (1.0 / D)
        var = rowsum(xc * xc, tok if ent == 4 else None) * (1.0 / D) + EPS
        return xc * lax.rsqrt(var)

    def fold(a, p):
        parts = []
        for g in range(NG):
            ar, ai = a[16 * g:16 * g + 8], a[16 * g + 8:16 * g + 16]
            pr, pi = p[16 * g:16 * g + 8], p[16 * g + 8:16 * g + 16]
            parts += [ar + pi, ai - pr] if g < NG // 2 else [ar - pi, ai + pr]
        return jnp.concatenate(parts, axis=0)

    def grp(x):
        return x.reshape(NG, 16, 128)

    row = lax.broadcasted_iota(i32, (8, 128), 0)

    def conv_rows(s, ls, emit, tok_in=None):
        w = [tp[8 * j:8 * j + 8, ls] for j in range(4)]
        if isinstance(s, int) and s == 0:
            pk = jnp.zeros((8, 128), f32)
            pt = jnp.zeros((8, 128), f32)
        else:
            kp = k_v[s - 1, T - 16:T, ls].astype(f32)[8:16]
            pk = pltpu.roll(kp, 1, 0)
            pt = pltpu.roll(w[2] * kp + w[3] * pk, 2, 0)
        for rg in range(T // 16):
            kk = k_v[s, rg * 16:rg * 16 + 16, ls].astype(f32)
            vv = v_v[s, rg * 16:rg * 16 + 16, ls].astype(f32)
            outs = []
            for h in range(2):
                kc = kk[8 * h:8 * h + 8]
                if h == 0 and tok_in is not None and tok_in() is not None:
                    kc = kc + tok_in()
                rk = pltpu.roll(kc, 1, 0)
                sk = jnp.where(row < 1, pk, rk)
                t = w[2] * kc + w[3] * sk
                rt = pltpu.roll(t, 2, 0)
                outs.append(((w[0] * kc + w[1] * sk) + jnp.where(row < 2, pt, rt)) * vv[8 * h:8 * h + 8])
                pk, pt = rk, rt
            emit(rg, pack(jnp.concatenate(outs, axis=0)))

    def dft_x(kv0, kv1, split=False):
        w = unpack(jnp.concatenate([kv0, kv1], axis=1))
        if split:
            xx = jnp.concatenate([jnp.dot(fw_v[h * NB:(h + 1) * NB, :], w, preferred_element_type=f32)
                                  for h in range(2)], axis=0)
        else:
            xx = jnp.dot(fw_v[...], w, preferred_element_type=f32)
        return xx[:, 0:128], xx[:, 128:256]

    def dft_h(s, rows):
        w = jnp.concatenate([ssm_v[2 * s, rows, :], ssm_v[2 * s + 1, rows, :]], axis=0)
        aa = lax.dot_general(fw_v[...], w, (((1,), (1,)), ((), ())), preferred_element_type=f32)
        return aa[:, 0:128], aa[:, 128:256]

    def silu_c():
        return unpack(tp[40:48, :])

    def modvec(p):
        return jnp.dot(silu_c(), wm_v[p], preferred_element_type=f32)[0:8]

    def mm(lhs, w):
        if lhs.shape[0] <= T:
            return jnp.dot(lhs, w(), preferred_element_type=f32)
        return jnp.concatenate([jnp.dot(lhs[r:r + T], w(), preferred_element_type=f32)
                                for r in range(0, lhs.shape[0], T)], axis=0)

    class Reg:
        def __init__(self):
            self.z0 = lax.shift_right_logical(pid, 8)
            self.st = {}

        def sconv(self, s, lanes, lcs=None):
            if lcs is None or lcs[0] == 0:
                self.sc = [None] * lanes
                self.gi = 0
            for lc in (range(NL) if lcs is None else lcs):
                ls = pl.ds(lc * 128, 128)

                def emit(rg, kvp, ls=ls):
                    kvb.at[self.z0][rg * 8:rg * 8 + 8, ls] = kvp
                    self.sc[self.gi % lanes] = kvb[0, HT:HT + 8, ls]
                    self.gi += 1
                conv_rows(s, ls, emit, lambda: self.sc[self.gi % lanes])

        def fwd_x(self, s, lc):
            o = self.z0 + 3 * s
            ls = pl.ds(lc * 128, 128)
            x0, x1 = dft_x(kvb[0, 0:64, ls], kvb[0, 64:128, ls])
            p = 3 * (s - 1)
            u1 = (uv[p + 2, :, 16:32, ls] + uv[p, :, 16:32, ls]) - grp(x0)
            uv[o, :, 16:32, ls] = grp(x0)
            uv[o + 1, :, 16:32, ls] = u1
            uv[o + 2, :, 16:32, ls] = grp(x1 - x0)

        def fwd_h(self, s, lc):
            o = self.z0 + 3 * s
            ls = pl.ds(lc * 128, 128)
            a0, a1 = dft_h(s, ls)
            h0 = fold(a0, ap[0, :, ls])
            h1 = fold(a1, a0)
            uv[o, :, 0:16, ls] = grp(h0 + h1)
            uv[o + 1, :, 0:16, ls] = grp(h1)
            uv[o + 2, :, 0:16, ls] = grp(h0)
            ap[self.z0, :, ls] = a1

        def mac(self, s, tree=(), tok0=None):
            static = isinstance(s, int)
            ng = s + 1 if static else NS - 1
            ub = [3 * (s - g) if static else 3 * jnp.maximum(s - g, 0) for g in range(ng)]
            toks = (tok0, tok0)
            for fc in range(NG):
                for lc in range(NL):
                    ls = pl.ds(lc * 128, 128)

                    def chain(j, ar, ai):
                        for g in range(ng):
                            hr = uv[3 * g + j, fc, 0:8, ls]
                            hi = uv[3 * g + j, fc, 8:16, ls]
                            xr = uv[ub[g] + j, fc, 16:24, ls]
                            xi = uv[ub[g] + j, fc, 24:32, ls]
                            if ar is not None and g in tree:
                                ar = ar + (hr * xr - hi * xi)
                                ai = ai + (hr * xi + hi * xr)
                            else:
                                ar = (hr * xr if ar is None else ar + hr * xr) - hi * xi
                                ai = (hr * xi if ai is None else ai + hr * xi) + hi * xr
                        return ar, ai

                    a1 = chain(0, *toks)
                    z0 = chain(1, *a1)
                    zero = pltpu.bitcast(zb[0, T:T + 8, ls], i32)

                    def tk(v):
                        return pltpu.bitcast(pltpu.bitcast(v, i32) & zero, f32)
                    z1 = chain(2, a1[0] + tk(z0[0]), a1[1] + tk(z0[1]))
                    for b, z in enumerate((z0, z1)):
                        zb.at[self.z0][b * HT + fc * 8:b * HT + fc * 8 + 8, ls] = pack(jnp.concatenate(z, axis=0))
                    toks = (tk(z1[0]), tk(z1[1]))

        def inv(self):
            for b in range(2):
                yb[self.z0, b * NB:(b + 1) * NB, :] = jnp.dot(
                    iv_v[...], unpack(zb[0, b * HT:(b + 1) * HT, :]), preferred_element_type=f32)

        def ln(self, s, ent=4):
            a1 = mv[0:1, :]; a0 = mv[8:9, :]; b1 = mv[16:17, :]; b0 = mv[24:25, :]
            tok = None
            for g in range(T // RG):
                gr = slice(g * RG, (g + 1) * RG)
                x = q_v[s, gr, :].astype(f32)
                x1 = x + (normalise(x) * a1 + a0) * yb[0, gr, :]
                x1b[self.z0 + s, gr, :] = x1
                h2 = normalise(x1, tok, ent) * b1 + b0
                hn_v.at[self.z0][g * (RG // 2):(g + 1) * (RG // 2), :] = pack(h2)
                tok = hn_v[0, HT:HT + 8, 0:128]

        def gcols(self, x, c0, n):
            return mm(x(), lambda: wg_v[:, c0:c0 + n])

        def ucols(self, x, c0, n):
            return mm(x(), lambda: wu_v[:, c0:c0 + n])

        def g_(self, x, c):
            self.st['g'] = self.gcols(x, c * FC, FC)

        def u_(self, x, c):
            self.st['a'] = (jnp.maximum(self.st.pop('g'), 0.0) * self.ucols(x, c * FC, FC)).astype(bf16)

        def d_(self, c):
            d = mm(self.st.pop('a'), lambda: wd_v[c * FC:(c + 1) * FC, :])
            self.st['acc'] = d if c == 0 else self.st['acc'] + d

        def gp(self, x, c, j):
            self.st[('g', j)] = self.gcols(x, c * FC + j * 128, 128)

        def up(self, x, c, j):
            self.st[('a', j)] = jnp.maximum(self.st.pop(('g', j)), 0.0) * self.ucols(x, c * FC + j * 128, 128)
            if j == NQ - 1:
                self.st['a'] = jnp.concatenate([self.st.pop(('a', i)) for i in range(NQ)], axis=1).astype(bf16)

        def dp(self, c, lc, s=None):
            ls = pl.ds(lc * 128, 128)
            d = mm(self.st['a'], lambda: wd_v[c * FC:(c + 1) * FC, ls])
            d = self.st['acc'][:, lc * 128:(lc + 1) * 128] + d
            if c == NC - 1:
                o_v[s, :, ls] = (x1b[s, :, ls] + mv[32:33, ls] * d).astype(bf16)
            else:
                self.st[('d', lc)] = d
                if lc == NL - 1:
                    self.st['acc'] = jnp.concatenate([self.st.pop(('d', i)) for i in range(NL)], axis=1)

        def fin(self, s):
            o_v[s] = (x1b[s] + mv[32:33, :] * self.st.pop('acc')).astype(bf16)

    def first():
        R = Reg()
        for gi, names in enumerate(GROUPS):
            for name in names:
                copy(name, gi).start()
        z = jnp.zeros((8, D), f32)
        kvb[0, HT:HT + 8, :] = z
        hn_v[0, HT:HT + 8, :] = z
        zb[0, T:T + 8, :] = z

        def zero_v(j, _):
            uv[j, :, 0:16, :] = jnp.zeros((NG, 16, D), f32)
            return 0
        lax.fori_loop(12, 3 * (NS - 1), zero_v, 0)

        def zero_gu(j, _):
            gu[blk(j, 64), :] = jnp.zeros((64, 2 * FC), f32)
            return 0
        lax.fori_loop(0, 2 * T // 64, zero_gu, 0)

        def cmul(h, x):
            return (h[:, 0:8] * x[:, 0:8] - h[:, 8:16] * x[:, 8:16], h[:, 0:8] * x[:, 8:16] + h[:, 8:16] * x[:, 0:8])

        def conv_pair(s):
            def body(lc, _):
                ls = blk(lc, 128)
                if s == 1:
                    for k in range(7):
                        g = jnp.minimum(lc * 7 + k, 2 * T // RG - 1)
                        gr = blk(g % (T // RG), RG)
                        n1[g // (T // RG), gr, :] = normalise(q_v[g // (T // RG), gr, :].astype(f32))
                    for b in range(2):
                        yb[0, b * NB:(b + 1) * NB, ls] = jnp.dot(
                            iv_v[...], unpack(n2[0, b * HT:(b + 1) * HT, ls]), preferred_element_type=f32)
                rows = []
                conv_rows(s, ls, lambda rg, kvp: rows.append(kvp))
                a0, a1 = dft_h(s, ls)
                x0, x1 = dft_x(jnp.concatenate(rows[0:8], axis=0), jnp.concatenate(rows[8:16], axis=0), True)
                if s == 0:
                    dd = tp[32:40, ls]
                    h0 = jnp.concatenate([a0[8 * g:8 * g + 8] + dd if g % 2 == 0 else a0[8 * g:8 * g + 8]
                                          for g in range(2 * NG)], axis=0)
                    u1 = grp(-x0)
                else:
                    h0 = fold(a0, ap[0, :, ls])
                    u1 = (uv[2, :, 16:32, ls] + uv[0, :, 16:32, ls]) - grp(x0)
                h1 = fold(a1, a0)
                us = [grp(x0), u1, grp(x1 - x0)]
                vs = [grp(h0 + h1), grp(h1), grp(h0)]
                if s == 0:
                    p = [cmul(vs[j], us[j]) for j in range(3)]
                else:
                    p = []
                    for j in range(3):
                        t0 = cmul(uv[j, :, 0:16, ls], us[j])
                        t1 = cmul(vs[j], uv[j, :, 16:32, ls])
                        p.append((t0[0] + t1[0], t0[1] + t1[1]))
                for j in range(3):
                    uv[3 * s + j, :, 16:32, ls] = us[j]
                    uv[3 * s + j, :, 0:16, ls] = vs[j]
                ap[0, :, ls] = a1
                for b in range(2):
                    zz = jnp.concatenate([p[0][0] + p[1 + b][0], p[0][1] + p[1 + b][1]], axis=1)
                    n2[s, b * HT:(b + 1) * HT, ls] = pack(zz.reshape(2 * NB, 128))
                return 0
            lax.fori_loop(0, NL, body, 0)

        with scope("p_w0"):
            wait_group(0)
        with scope("p_c0"):
            taps = sh_v[...].astype(f32)
            for j in range(4):
                tp[8 * j:8 * j + 8, :] = jnp.broadcast_to(taps[j:j + 1, :], (8, D))
            tp[32:40, :] = jnp.broadcast_to(dd_v[...].astype(f32).reshape(1, D), (8, D))
            c32 = c_v[...].astype(f32)
            tp[40:48, :] = pack(jnp.broadcast_to(c32 * jax.nn.sigmoid(c32), (16, D)))
            conv_pair(0)
        with scope("p_c1"):
            wait_group(1)
            wait_group(2)
            conv_pair(1)

            wait_group(3)
            for b in range(2):
                yb[0, T + b * NB:T + (b + 1) * NB, :] = jnp.dot(
                    iv_v[...], unpack(n2[1, b * HT:(b + 1) * HT, :]), preferred_element_type=f32)
            sa, ca1 = modvec(MPOS['sa']), 1.0 + modvec(MPOS['ca'])
            mv[40:48, :] = sa
            mv[48:56, :] = ca1

            def pre(i, _):
                r = blk(i, 64)
                for h in range(2):
                    y = yb[0, pl.ds(pl.multiple_of(h * T + i * 64, 64), 64), :]
                    n1[h, r, :] = (n1[h, r, :] * mv[48:49, :] + mv[40:41, :]) * y
                return 0
            lax.fori_loop(0, T // 64, pre, 0)
        with scope("p_ln2"):
            wait_group(4)
            ga = modvec(MPOS['ga'])
            mv[0:8, :] = ga * mv[48:56, :]
            mv[8:16, :] = ga * mv[40:48, :]
            for i in range(2):
                for g in range(T // RG):
                    gr = slice(g * RG, (g + 1) * RG)
                    x1 = q_v[i, gr, :].astype(f32) + ga[0:1] * n1[i, gr, :]
                    x1b[i, gr, :] = x1
                    n2[R.z0 + i, gr, :] = normalise(x1)

        def h2_tile(k):
            ls = blk(k, 128)
            b1 = 1.0 + jnp.dot(silu_c(), wm_v[MPOS['cb'], :, ls], preferred_element_type=f32)[0:8]
            b0 = jnp.dot(silu_c(), wm_v[MPOS['sb'], :, ls], preferred_element_type=f32)[0:8]
            mv[16:24, ls] = b1
            mv[24:32, ls] = b0
            t = jnp.concatenate([pack(n2[i, :, ls] * b1[0:1] + b0[0:1]) for i in range(2)], axis=0)
            hf[0, :, ls] = t
            return t

        with scope("f_k"):
            wait_group(G_K - 1)

            def kstep(k, lhs):
                @pl.when(k + 1 < NL)
                def _():
                    copy(('cb', k + 1), G_K + k).wait()
                    copy(('sb', k + 1), G_K + k).wait()
                copy(('wgk', k), G_K + k).wait()
                copy(('wuk', k), G_K + k).wait()
                xk = unpack(lhs)
                gu[:, 0:FC] += jnp.dot(xk, wg_v[blk(k, 128), 0:FC], preferred_element_type=f32)
                nxt = h2_tile(jnp.minimum(k + 1, NL - 1))
                gu[:, FC:2 * FC] += jnp.dot(xk, wu_v[blk(k, 128), 0:FC], preferred_element_type=f32)
                return nxt
            lax.fori_loop(0, NL, kstep, h2_tile(0))
        x = lambda: unpack(hf[0])
        xh = [lambda h=h: unpack(hf[0, h * HT:(h + 1) * HT, :]) for h in range(2)]
        with scope("f_c"):
            wait_group(G_F)
            R.st['a'] = (jnp.maximum(gu[:, 0:FC], 0.0) * gu[:, FC:2 * FC]).astype(bf16)
            for lc in range(NL):
                ls = pl.ds(lc * 128, 128)
                if lc < CFG['fch']:
                    R.fwd_h(2, lc)
                accb.at[R.z0][:, ls] = mm(R.st['a'], lambda: wd_v[0:FC, ls])
        with scope("f_d"):
            wait_group(G_F + 1)
            for lc in range(CFG['fch'], NL):
                R.fwd_h(2, lc)
            for k in range(2 * NQ):
                j, h = k // 2, k % 2
                gu.at[blk(R.z0, 2 * T)][h * T:(h + 1) * T, j * 128:(j + 1) * 128] = R.gcols(xh[h], FC + j * 128, 128)
                if k in CFG['fdx']:
                    lc = CFG['fdx'].index(k)
                    if lc == 0:
                        R.sconv(2, 2)
                    R.fwd_x(2, lc)
        with scope("f_e"):
            wait_group(G_F + 2)
            R.st['g'] = gu[:, 0:FC]
            R.st['acc'] = accb[0]
            R.mac(2, CFG['ftree'])
            R.u_(x, 1)
            for lc in range(NL):
                if lc == CFG['finv']:
                    R.inv()
                    R.ln(2, CFG['fent'])
                R.dp(1, lc)
            R.g_(x, 2)
        with scope("f_f"):
            wait_group(G_F + 3)
            g, acc = R.st.pop('g'), R.st.pop('acc')
            act = {}

            def upiece(j, h):
                u = R.ucols(xh[h], F - FC + j * 128, 128)
                act[(h, j)] = jnp.maximum(g[h * T:(h + 1) * T, j * 128:(j + 1) * 128], 0.0) * u
                if j == NQ - 1:
                    act[h] = jnp.concatenate([act.pop((h, i)) for i in range(NQ)], axis=1).astype(bf16)

            def dpiece(lc, h):
                ls = pl.ds(lc * 128, 128)
                d = acc[h * T:(h + 1) * T, lc * 128:(lc + 1) * 128] + jnp.dot(
                    act[h], wd_v[F - FC:F, ls], preferred_element_type=f32)
                o_v[h, :, ls] = (x1b[h, :, ls] + mv[32:33, ls] * d).astype(bf16)

            pieces = [(upiece, j, h) for j in range(NQ) for h in range(2)]
            pieces += [(dpiece, lc, h) for lc in range(NL) for h in range(2)]
            for k, (fn, i, h) in enumerate(pieces):
                fn(i, h)
                if k in CFG['gbp']:
                    ls = pl.ds(CFG['gbp'].index(k) * 128, 128)
                    mv[32:40, ls] = jnp.dot(silu_c(), wm_v[MPOS['gb'], :, ls], preferred_element_type=f32)[0:8]
                if k in CFG['fhp']:
                    R.fwd_h(3, CFG['fhp'].index(k))
                if k in CFG['fxp']:
                    lc = CFG['fxp'].index(k)
                    if not CFG['fscall']:
                        R.sconv(3, 2, [lc])
                    elif lc == 0:
                        R.sconv(3, 2)
                    R.fwd_x(3, lc)
            ocopy(0).start(); ocopy(1).start()

    def steady():
        R = Reg()
        s = pid + 1
        with scope("s_w"):
            for name in [('q', s + 1)] + _kvs(s + 2):
                copy(name, G_STEADY + s - 2).wait()
        with scope("s"):
            xv = unpack(hn_v[0, 0:HT, :])
            x = lambda: xv
            R.sconv(s + 2, 2)
            R.mac(s + 1, CFG['tree'], kvb[0, HT:HT + 8, 0:128])
            R.g_(x, 0); R.u_(x, 0); R.d_(0); R.g_(x, 1); R.u_(x, 1)
            R.inv()
            R.ln(s + 1, 3)
            pieces = [lambda lc=lc: R.dp(1, lc) for lc in range(NL)]
            pieces += [lambda j=j: R.gp(x, 2, j) for j in range(NQ)]
            pieces += [lambda j=j: R.up(x, 2, j) for j in range(NQ)]
            pieces += [lambda lc=lc: R.dp(2, lc, s) for lc in range(NL)]
            for k, p in enumerate(pieces):
                p()
                if k in CFG['hp']:
                    R.fwd_h(s + 2, CFG['hp'].index(k))
                if k in CFG['xp']:
                    R.fwd_x(s + 2, CFG['xp'].index(k))
            ocopy(s).start()

    def last():
        R = Reg()
        s = NS - 2
        with scope("l_w"):
            wait_group(len(GROUPS) - 1)
        with scope("l"):
            xv = unpack(hn_v[0, 0:HT, :])
            x = lambda: xv
            R.mac(s + 1, CFG['ltree'])
            R.g_(x, 0); R.u_(x, 0); R.d_(0); R.g_(x, 1); R.u_(x, 1); R.d_(1)
            R.inv()
            R.ln(s + 1, 4)
            R.g_(x, 2); R.u_(x, 2); R.d_(2)
            R.fin(s)
            ocopy(s).start()
            x = lambda: unpack(hn_v[0, 0:HT, :])
            for c in range(NC - 1):
                R.g_(x, c); R.u_(x, c); R.d_(c)
            R.g_(x, NC - 1); R.u_(x, NC - 1)
            a, acc = R.st.pop('a'), R.st.pop('acc')
            for r0, n in CFG['lastsplit']:
                d = acc[r0:r0 + n] + jnp.dot(a[r0:r0 + n], wd_v[F - FC:F, :], preferred_element_type=f32)
                o_v[s + 1, r0:r0 + n, :] = (x1b[s + 1, r0:r0 + n, :] + mv[32:33, :] * d).astype(bf16)
                ocopy(s + 1, (r0, n)).start()
        with scope("e_w"):
            for t in range(NS - 1):
                ocopy(t).wait()
            for h in CFG['lastsplit']:
                ocopy(NS - 1, h).wait()

    only = CFG['only']
    if only is None or 0 in only:
        pl.when(pid == 0)(first)
    if only is None or 1 in only:
        pl.when(jnp.logical_and(pid >= 1, pid <= NS - 4))(steady)
    if only is None or 2 in only:
        pl.when(pid == NS - 3)(last)


@jax.jit
def pallas_adaLN_cond__ssm_conv_h3__glu_gated_reglu__prompt_kernel(A_q, A_k, A_v, A_shift_k, A_ssm_k, A_ssm_D, B_x, B_W_gate, B_W_up, B_W_down, c, w_mod):
    fwd, inv = _dft_mats()
    any_spec = pl.BlockSpec(memory_space=pl.ANY)
    vm = pltpu.VMEM
    return pl.pallas_call(
        _kernel,
        grid=(NS - 2,),
        in_specs=[any_spec] * 13,
        out_specs=any_spec,
        out_shape=jax.ShapeDtypeStruct((1, S, D), bf16),
        scratch_shapes=[
            vm((NS, T, D), bf16), vm((NS, T, D), bf16), vm((NS, T, D), bf16),
            vm((NBLK, D, NB), bf16),
            vm((D, F), bf16), vm((D, F), bf16), vm((F, D), bf16),
            vm((6, D, D), bf16),
            vm((2 * NB, NB), bf16), vm((NB, 2 * NB), bf16),
            vm((NS, T, D), bf16),
            vm((3 * NS, NG, 32, D), f32),
            vm((1, 2 * NB, D), f32),
            vm((1, T + 32, D), f32),
            vm((1, HT + 32, D), f32),
            vm((64, D), f32),
            vm((1, 2 * T, D), f32),
            vm((NS, T, D), f32),
            vm((1, HT + 32, D), f32),
            vm((1, T, D), f32),
            vm((2, T, D), f32),
            vm((2, T, D), f32),
            vm((2 * T, 2 * FC), f32),
            vm((1, 2 * T, D), f32),
            vm((64, D), f32),
            vm((4, D), bf16), vm((D,), bf16), vm((1, D), bf16),
            pltpu.SemaphoreType.DMA((len(GROUPS),)), pltpu.SemaphoreType.DMA((1,)),
        ],
        compiler_params=pltpu.CompilerParams(vmem_limit_bytes=110 * 1024 * 1024,
                                             dimension_semantics=("arbitrary",)),
    )(A_q, A_k, A_v, A_shift_k.T, A_ssm_k, A_ssm_D, B_W_gate, B_W_up, B_W_down, c, w_mod,
      jnp.asarray(fwd, bf16), jnp.asarray(inv, bf16))
```
